```python
import os as _os
_os.environ.setdefault("JAX_PLATFORMS", "cpu")
import jax
import jax.numpy as jnp

def _softmax(x, axis=-1):
    return jax.nn.softmax(x, axis=axis)
def _gelu(x):
    return jax.nn.gelu(x, approximate=True)
def _silu(x):
    return jax.nn.silu(x)
def _sigmoid(x):
    return jax.nn.sigmoid(x)
def _layernorm(x, axis=-1, eps=1e-5):
    m = jnp.mean(x, axis=axis, keepdims=True)
    v = jnp.var(x, axis=axis, keepdims=True)
    return (x - m) / jnp.sqrt(v + eps)
def _scatter_add(tgt, idx, src, axis=0):
    return tgt.at[idx].add(src)
def _segment_sum(src, seg, n):
    return jax.ops.segment_sum(src, seg, n)
class _Rng:
    def __init__(self, key):
        self._k = key
    def _next(self):
        self._k, sub = jax.random.split(self._k)
        return sub
    def normal(self, shape):
        return jax.random.normal(self._next(), shape, dtype=jnp.bfloat16)
    def randint(self, lo, hi, shape):
        return jax.random.randint(self._next(), shape, lo, hi, dtype=jnp.int32)
    def uniform(self, shape, lo=0.0, hi=1.0):
        return jax.random.uniform(self._next(), shape, jnp.bfloat16, lo, hi)
    def permutation(self, n):
        return jax.random.permutation(self._next(), n)


kernel_name = 'recurrent_scan__ssm_conv_s5__geglu_ffn__prompt'

def setup_inputs():
    _rng = _Rng(jax.random.key(int.from_bytes(__import__("os").urandom(4), "little")))
    _w = (lambda a: (lambda t: t.astype(jnp.bfloat16) if jnp.issubdtype(t.dtype, jnp.floating) else t)(jnp.asarray(a)))
    def _A_setup():
        B, S, D = 1, 2048, 640
        P = D
        Lambda_re = -0.5 * jnp.exp((lambda *s: _rng.normal(s) * 0.4)(P))
        Lambda_im = (lambda *s: _rng.normal(s) * 0.4)(P) * 1.0
        B_re = (lambda *s: _rng.normal(s) * 0.4)(P, D) * (D ** -0.5)
        B_im = (lambda *s: _rng.normal(s) * 0.4)(P, D) * (D ** -0.5)
        C_re = (lambda *s: _rng.normal(s) * 0.4)(D, P) * (P ** -0.5)
        C_im = (lambda *s: _rng.normal(s) * 0.4)(D, P) * (P ** -0.5)
        log_dt = (lambda *s: _rng.normal(s) * 0.4)(P) * 0.3 - 2.0
        Dskip = (lambda *s: _rng.normal(s) * 0.4)(D)
        return {
            "x": _w((lambda *s: _rng.normal(s) * 0.05)(B, S, D)),
            "Lambda_re": _w(Lambda_re),
            "Lambda_im": _w(Lambda_im),
            "B_re": _w(B_re),
            "B_im": _w(B_im),
            "C_re": _w(C_re),
            "C_im": _w(C_im),
            "log_dt": _w(log_dt),
            "Dskip": _w(Dskip),
        }
    _A_in = _A_setup()

    def _B_setup():
        B, S, D, F = 1, 2048, 640, 1728
        return {
            "x": _w((lambda *s: _rng.normal(s) * 0.05)(B, S, D)),
            "w_gate": _w((lambda *s: _rng.normal(s) * 0.05)(D, F)),
            "w_up": _w((lambda *s: _rng.normal(s) * 0.05)(D, F)),
            "w_down": _w((lambda *s: _rng.normal(s) * 0.05)(F, D)),
        }
    _B_in = _B_setup()

    return {
        "A_x": _A_in["x"],
        "A_Lambda_re": _A_in["Lambda_re"],
        "A_Lambda_im": _A_in["Lambda_im"],
        "A_B_re": _A_in["B_re"],
        "A_B_im": _A_in["B_im"],
        "A_C_re": _A_in["C_re"],
        "A_C_im": _A_in["C_im"],
        "A_log_dt": _A_in["log_dt"],
        "A_Dskip": _A_in["Dskip"],
        "B_x": _B_in["x"],
        "B_w_gate": _B_in["w_gate"],
        "B_w_up": _B_in["w_up"],
        "B_w_down": _B_in["w_down"],
    }

def reference(A_x, A_Lambda_re, A_Lambda_im, A_B_re, A_B_im, A_C_re, A_C_im, A_log_dt, A_Dskip, B_x, B_w_gate, B_w_up, B_w_down):
    def _A_ref(x, Lambda_re, Lambda_im, B_re, B_im, C_re, C_im, log_dt, Dskip):
        Bsz, L, H = x.shape
        Lam = Lambda_re + 1j * Lambda_im
        Bmat = B_re + 1j * B_im
        Cmat = C_re + 1j * C_im
        dt = jnp.exp(log_dt)
        Lam_bar = jnp.exp(dt * Lam)
        B_bar = ((Lam_bar - 1.0) / Lam)[:, None] * Bmat
        Bu = jnp.einsum("bld,pd->blp", x + 0j, B_bar)
        h = jnp.zeros_like(Bu[:, 0, :])
        hs = []
        for t in range(L):
            h = Lam_bar[None, :] * h + Bu[:, t, :]
            hs.append(h)
        hseq = jnp.stack(hs, 1)
        y = 2.0 * jnp.einsum("blp,dp->bld", hseq, Cmat).real + x * Dskip[None, None, :]
        return y

    def _B_ref(x, w_gate, w_up, w_down):
        return (_gelu(x @ w_gate) * (x @ w_up)) @ w_down

    x = A_x
    xn = _layernorm(x, axis=-1)
    s = _A_ref(xn, A_Lambda_re, A_Lambda_im, A_B_re, A_B_im, A_C_re, A_C_im, A_log_dt, A_Dskip)
    g = _silu(_B_ref(xn, B_w_gate, B_w_up, B_w_down))
    return x + s * g
```

```python
import functools

import numpy as np
import jax
import jax.numpy as jnp
from jax import lax
import jax.experimental.pallas as pl
import jax.experimental.pallas.tpu as pltpu

F32 = jnp.float32
BF16 = jnp.bfloat16
U32 = jnp.uint32
LANE = 128
NT = (((1,), (1,)), ((), ()))
NN = (((1,), (0,)), ((), ()))


def _acc(d, k, c):
    d[k] = d.get(k, 0) + c
    if d[k] == 0:
        del d[k]


class _HK:
    def __init__(self, methods, via):
        self.names, self.lhs, self.out = [], {}, {}
        n = len(methods)
        self.idx = [self._index(str(i), {i: 1}, {i: 1}, m) for i, m in enumerate(methods)]
        self.y, virt = {}, {}
        for i in range(n):
            self.y[i, i] = {self.idx[i][4]: 1, self.idx[i][5]: -1}
        for i in range(n):
            for j in range(n):
                if (methods[i] + 1) % 3 == methods[j]:
                    self.y[i, j], self.y[j, i], v = self._pair(self.idx[i], self.idx[j])
                    virt[i, j] = (v, 1)
                    virt[j, i] = (v, -1)
        for (i, j), l in via:
            v, sg = virt[j, l]
            if (methods[i] + 1) % 3 == v[3]:
                yiv, yvi, _ = self._pair(self.idx[i], v)
            else:
                yvi, yiv, _ = self._pair(v, self.idx[i])
            d = dict(yiv)
            for k, c in self.y[i, l].items():
                _acc(d, k, -c)
            self.y[i, j] = d
            d = {k: sg * c for k, c in yvi.items()}
            for k, c in self.y[l, i].items():
                _acc(d, k, c)
            self.y[j, i] = d
        assert len(self.y) == n * n

    def _prod(self, name, lhs, out):
        self.names.append(name)
        self.lhs[name], self.out[name] = lhs, out

    def _index(self, name, a, c, m):
        m1, m2 = (m + 1) % 3, (m + 2) % 3
        d1, d2 = name + ".1", name + ".2"
        self._prod(d1, {(i, m1): v for i, v in a.items()}, {(j, m2): v for j, v in c.items()})
        self._prod(d2, {(i, m2): v for i, v in a.items()}, {(j, m1): v for j, v in c.items()})
        return (name, a, c, m, d1, d2)

    def _pair(self, I, J):
        s = I[3]
        s1 = (s + 1) % 3
        assert s1 == J[3]
        a, c, lhs, out = dict(I[1]), dict(I[2]), {}, {}
        for k, v in J[1].items():
            _acc(a, k, -v)
        for k, v in J[2].items():
            _acc(c, k, v)
        V = self._index("(%s-%s)" % (I[0], J[0]), a, c, (s + 2) % 3)
        for k, v in I[1].items():
            _acc(lhs, (k, s1), v)
        for k, v in J[1].items():
            _acc(lhs, (k, s), v)
        for k, v in I[2].items():
            _acc(out, (k, s1), v)
        for k, v in J[2].items():
            _acc(out, (k, s), -v)
        sn = "S(%s,%s)" % (I[0], J[0])
        self._prod(sn, lhs, out)
        return ({sn: 1, V[4]: 1, I[5]: 1, J[5]: -1}, {sn: 1, V[5]: 1, I[4]: 1, J[4]: -1}, V)

    def weights(self, entries):
        w = {}
        for ij in entries:
            for p, c in self.y[ij].items():
                _acc(w.setdefault(p, {}), ij, c)
        return {p: d for p, d in w.items() if d}


def _slp(targets):
    ts = [dict(t) for t in targets]
    ops = []
    while any(len(t) > 1 for t in ts):
        cnt = {}
        for t in ts:
            ks = sorted(t, key=repr)
            for x in range(len(ks)):
                for y in range(x + 1, len(ks)):
                    key = (ks[x], ks[y], t[ks[x]] * t[ks[y]])
                    cnt[key] = cnt.get(key, 0) + 1
        a, b, sg = max(cnt, key=lambda k: cnt[k])
        new = ("t", len(ops))
        ops.append((new, a, b, sg))
        for t in ts:
            if a in t and b in t and t[a] * t[b] == sg:
                t[new] = t.pop(a)
                del t[b]
    return ops, [next(iter(t.items()))[::-1] for t in ts]


def _run_slp(slp, env, positive=False):
    ops, results = slp
    env = dict(env)
    inner = {v for _, a, b, _ in ops for v in (a, b)}
    want = {v: s for s, v in results if positive and v not in inner}
    for new, a, b, sg in ops:
        (sp, vp), (sq, vq) = env[a], env[b]
        sq = sq * sg
        if sp == sq:
            env[new] = sp, lax.add(vp, vq)
        else:
            s = want.get(new, 1)
            env[new] = s, (lax.sub(vp, vq) if sp == s else lax.sub(vq, vp))
    return [(s * env[v][0], env[v][1]) for s, v in results]


def _slp_signs(slp, env_signs):
    ops, results = slp
    env = dict(env_signs)
    for new, a, b, sg in ops:
        sp, sq = env[a], sg * env[b]
        env[new] = sp if sp == sq else 1
    return [s * env[v] for s, v in results]


class _Sum:
    def __init__(self, sign, value):
        self.terms = [(sign, value)]

    def get(self, sign):
        if len(self.terms) == 2:
            (sp, vp), (sq, vq) = self.terms
            if sp == sq:
                return sp, lax.add(vp, vq)
            return sign, (lax.sub(vp, vq) if sp == sign else lax.sub(vq, vp))
        return self.terms[0]

    def add(self, sign, value):
        self.terms = [self.get(-sign), (sign, value)]


class _Transposed:
    def __init__(self, slp, dry=False):
        ops, self.results = slp
        self.dry, self.adj = dry, {}
        self.split = {new: (a, b, sg) for new, a, b, sg in ops}
        self.pending = {}
        for v in [v for _, v in self.results] + [v for _, a, b, _ in ops for v in (a, b)]:
            self.pending[v] = self.pending.get(v, 0) + 1

    def put(self, v, sign, val):
        if v not in self.adj:
            self.adj[v] = _Sum(sign, val)
        elif not self.dry:
            self.adj[v].add(sign, val)
        self.pending[v] -= 1
        if self.pending[v] == 0 and v in self.split:
            a, b, sg = self.split[v]
            s, val = self.adj.pop(v).get(1)
            self.put(a, s, val)
            self.put(b, s * sg, val)

    def feed(self, t, val, sign=1):
        s, v = self.results[t]
        self.put(v, s * sign, val)


def _feed_order(slp):
    order, rest = [], list(range(len(slp[1])))

    def live(seq):
        tr = _Transposed(slp, dry=True)
        for t in seq:
            tr.feed(t, None)
        done = [j for j in range(5) if all(tr.pending.get((j, s), 0) == 0 for s in range(3))]
        return len(tr.adj) - len(done), sum(tr.pending.get((j, s), 0) ** 0.5 for j in range(5) for s in range(3))
    while rest:
        t = min(rest, key=lambda t: live(order + [t]))
        order.append(t)
        rest.remove(t)
    return order


_FORM_SIGN = (1, -1, 1)
_SCHEME = _HK((0, 0, 1, 1, 2), (((0, 1), 2), ((2, 3), 0)))
_NAMES = list(_SCHEME.names)
_R = len(_NAMES)
_LHS_SLP = _slp([_SCHEME.lhs[p] for p in _NAMES])
_OUT_SLP = _slp([_SCHEME.out[p] for p in _NAMES])
_LHS_SIGN = dict(zip(_NAMES, _slp_signs(_LHS_SLP, {(i, s): _FORM_SIGN[s] for i in range(5) for s in range(3)})))
_W_FULL = _SCHEME.weights([(i, j) for i in range(5) for j in range(5)])
_W_K4 = _SCHEME.weights([(i, j) for i in range(4) for j in range(4)])
_NAMES_K4 = [p for p in _NAMES if p in _W_K4]
_D4 = _SCHEME.idx[4][4], _SCHEME.idx[4][5]
_LHS_SLP_K4 = _slp([_SCHEME.lhs[p] for p in _NAMES_K4])
_LHS_SIGN_K4 = dict(zip(_NAMES_K4, _slp_signs(_LHS_SLP_K4, {(i, s): _FORM_SIGN[s] for i in range(4) for s in range(3)})))


def _n2_products():
    res = []
    for i, j in ((0, 2), (1, 3)):
        w = _SCHEME.weights([(i, i), (i, j), (j, i), (j, j)])
        col = {i: 0, j: 1}
        for p in _NAMES:
            if p in w:
                res.append((p, {(col[c], s): v for (c, s), v in _SCHEME.out[p].items()},
                            {(a, col[b]): v for (a, b), v in w[p].items()}))
    for c in range(2):
        res.append((_D4[0], {(c, 1): 1}, {(4, c): 1}))
        res.append((_D4[1], {(c, 0): 1}, {(4, c): -1}))
    return res


_N2 = _n2_products()
_OUT_SLP_N2 = _slp([o for _, o, _ in _N2])
_N2_LHS = [_NAMES.index(p) for p, _, _ in _N2]
assert all(_LHS_SIGN_K4[p] == _LHS_SIGN[p] for p in _NAMES_K4)


class _Weights:
    def __init__(self, w, lhs_sign):
        w = {p: {k: lhs_sign[p] * c for k, c in d.items()} for p, d in w.items()}
        self.single = {p: next(iter(d)) for p, d in w.items() if len(d) == 1}
        self.sign = {p: next(iter(d.values())) if len(d) == 1 else 1 for p, d in w.items()}
        self.summed = [p for p in lhs_sign if p in w and p not in self.single]
        self.slp = _slp([w[p] for p in self.summed])
        self.used = sorted({k for p in self.summed for k in w[p]})


_V_FULL, _V_K4 = _Weights(_W_FULL, _LHS_SIGN), _Weights(_W_K4, _LHS_SIGN)
_V_N2 = _Weights({n: w for n, (_, _, w) in enumerate(_N2)}, {n: _LHS_SIGN[p] for n, (p, _, _) in enumerate(_N2)})
assert all(_V_K4.sign[p] == _V_FULL.sign[p] for p in _NAMES_K4) and all(_V_FULL.sign[p] == 1 for p in _D4)
_SIGN, _SIGN_N2 = [_V_FULL.sign[p] for p in _NAMES], [_V_N2.sign[n] for n in range(len(_N2))]


def _lhs_combos(slp, a1, a2):
    env = {}
    for i, (x, y) in enumerate(zip(a1, a2)):
        env[i, 0] = (1, x)
        env[i, 1] = (-1, y)
        env[i, 2] = (1, lax.sub(y, x))
    return [v for _, v in _run_slp(slp, env)]


def _columns(acc, ncol):
    c1, c2 = [], []
    for j in range(ncol):
        s2, v2 = acc[j, 2].get(1)
        for form, dst in ((1, c1), (0, c2)):
            tot = _Sum(*acc[j, form].get(s2))
            tot.add(-s2, v2)
            s, v = tot.get(1)
            dst.append(v if s > 0 else lax.neg(v))
    return c1, c2


_ORDER, _ORDER_N2 = _feed_order(_OUT_SLP), _feed_order(_OUT_SLP_N2)


def _lo(v):
    return lax.slice_in_dim(v, 0, v.shape[0] // 2, axis=0)


def _hi(v):
    return lax.slice_in_dim(v, v.shape[0] // 2, v.shape[0], axis=0)


def _cat(*vs):
    return lax.concatenate(vs, 0)


def _pack(v):
    return lax.bitcast_convert_type(pltpu.pack_elementwise([_lo(v), _hi(v)], packed_dtype=BF16), U32)


def _split(w):
    return _cat(*[pltpu.unpack_elementwise(w, index=i, packed_dtype=BF16, unpacked_dtype=F32)
                  for i in range(2)])


def _unpack(v):
    return pltpu.bitcast(v, BF16)


def _cmul(ar, ai, br, bi):
    return lax.sub(lax.mul(ar, br), lax.mul(ai, bi)), lax.add(lax.mul(ar, bi), lax.mul(ai, br))


def _cmad(ar, ai, br, bi, cr, ci):
    tr, ti = _cmul(ar, ai, br, bi)
    return lax.add(tr, cr), lax.add(ti, ci)


def default_plan(NB):
    R, B, C, D = (lambda b, k=k: (k, b) for k in "RBCD")
    G = lambda b, g: ("G", b, g)
    rest = tuple("x%d" % b for b in range(2, NB))
    ln = lambda b: [("stage", b), ("stats", b, 0), ("stats", b, 1), ("ln", b)]
    prep = lambda names, first, last: [(("prep", n), first, last) for n in names.split()]
    steps = [("start", "vec", "x0"), ("wait", "vec"), ("run", ("coefs",)),
             ("wait", "x0"), ("start", "bre", "bim"), ("run",) + tuple(ln(0)),
             ("wait", "bre", "bim"), ("start", "wr", "wg0", "wu0"), ("run", ("prep", "b0")),
             ("B", 0, 0), ("B", 0, 1), R(0), G(0, 0), G(0, 1), B(1), D(0)]
    tasks = prep("b1", ("B", 0, 0), ("B", 0, 0))
    tasks += [(("dma", ("wr", "wg0", "wu0"), ("x1", "wg1", "wu1")), ("B", 0, 1), ("B", 0, 1))]
    tasks += prep("r0 r1", ("B", 0, 1), ("B", 0, 1)) + prep("g0 u0", ("B", 0, 1), R(0))
    tasks += [(("dma", ("x1", "wg1", "wu1"), ("wd", "cre", "cim") + rest), R(0), G(0, 0))]
    tasks += [(t, R(0), G(0, 1)) for t in ln(1)] + prep("g1 u1", R(0), G(0, 0))
    tasks += [(("act_rest", 0), G(0, 0), G(0, 1)), (("act", 0, 0), G(0, 1), B(1)),
              (("dma", ("wd", "cre", "cim") + rest, ()), G(0, 1), B(1))]
    tasks += prep("d0 d1 d2", G(0, 1), B(1)) + [(("act", 0, 1), B(1), B(1))]
    tasks += [(("ucomb", 0), B(1), D(0)), (("ends", 0), B(1), R(1))] + prep("c0", B(1), R(1))
    tasks += [(("scan", 0), B(1), R(1))] + prep("c1", B(1), R(1)) + [(("hcomb", 0), B(1), R(1))]
    for b in range(1, NB):
        nxt = b + 1 < NB
        last = B(b + 1) if nxt else C(b)
        steps += [R(b), C(b - 1), G(b, 0), G(b, 1), last, D(b)]
        pre = [(t, D(b - 1), G(b, 1)) for t in ln(b + 1)[:3]] if nxt else []
        ssm = lambda end: [((t, b), D(b - 1), end) for t in ("ends", "scan", "hcomb")]
        fin = lambda end: [((t, b - 1), G(b, 0), end) for t in ("fin", "out")]
        tasks += [(("ucomb", b), D(b - 1), C(b - 1))] + pre + [(("act_rest", b), C(b - 1), G(b, 1))]
        if nxt:
            tasks += [(("ln", b + 1), D(b - 1), G(b, 1))] + fin(D(b))
            tasks += [(("act", b, 0), G(b, 1), last), (("act", b, 1), last, last)] + ssm(R(b + 1))
        else:
            tasks += ssm(G(b, 1)) + fin(last) + [(("act", b, 0), G(b, 1), last), (("act", b, 1), last, last)]
    tasks += [(("ysum", NB - 1), D(NB - 1), D(NB - 1))]
    steps += [("run", ("fin", NB - 1, True), ("out", NB - 1))]
    return steps, tasks


def _spread(cycles, work, lo, hi):
    def run(load, p0, p1, u):
        ends, idle = [], []
        for p in range(p0, p1):
            left = load * cycles[p]
            while u < hi[p] and left > 0:
                need = (int(u) + 1 - u) * work[int(u)][p]
                u, left = (int(u) + 1, left - need) if need <= left else (u + left / work[int(u)][p], 0)
            ends.append(u)
            idle.append(left > 0)
        return ends, idle

    def solve(p0, p1, u, last):
        if p0 == p1:
            return []
        need = lo[p0:p1 - 1] + [max(lo[p1 - 1], last)]
        a, b = 0.0, 8.0
        for _ in range(40):
            m = (a + b) / 2
            a, b = (a, m) if all(e >= n for e, n in zip(run(m, p0, p1, u)[0], need)) else (m, b)
        j = next((p0 + k for k, (e, n) in enumerate(zip(run(a, p0, p1, u)[0], need)) if e < n), p1 - 1)
        ends, idle = run(b, p0, j + 1, u)
        i = max([p0 + k + 1 for k in range(j - p0) if idle[k]], default=p0)
        ends[-1] = max(need[j - p0], u)
        return solve(p0, i, u, hi[i - 1]) + ends[i - p0:] + solve(j + 1, p1, ends[-1], last)

    return solve(0, len(cycles), 0.0, 0)


def build(Ls=(17, 17, 17, 13), nodma=0, debug=0, scopes=0, tail=0.5, PL=10, PW=5, DL=0, DS=40, dead='all', RF=0,
          inp_h=1, inp_o=0, SP=None, SE=-2, SS=-2, SU=None, SC=None, WCH=16,
          cap=((2.6, 0.33), (2.4, 0.55)), plan=None):
    NB = len(Ls)
    LM = max(Ls)
    T0 = [32 * sum(Ls[:b]) for b in range(NB)]
    steps, stream = plan(NB) if callable(plan) else plan or default_plan(NB)
    phases = [s for s in steps if s[0] in "BGRCD"]

    def n_tiles(key):
        return 40 if key[0] == "B" and len(key) == 3 else dict(B=80, G=80, R=58, C=80, D=114)[key[0]]

    nt = lambda i, j: (LANE * j, LANE * i)
    nn = lambda i, j: (LANE * i, LANE * j)
    tables = dict(b0=(_V_FULL, "bre", 0, nt), b1=(_V_FULL, "bim", 0, nt),
                  c0=(_V_FULL, "cre", 0, nt), c1=(_V_FULL, "cim", 0, nt),
                  g0=(_V_FULL, "wg", 0, nt), u0=(_V_FULL, "wu", 0, nt),
                  g1=(_V_FULL, "wg", 5 * LANE, nt), u1=(_V_FULL, "wu", 5 * LANE, nt),
                  r0=(_V_FULL, "wr", 0, nt), r1=(_V_N2, "wr", 5 * LANE, nt),
                  d0=(_V_FULL, "wd", 0, nn), d1=(_V_FULL, "wd", 5 * LANE, nn), d2=(_V_K4, "wd", 10 * LANE, nn))

    def task_cost(t):
        L = Ls[t[1]] if len(t) > 1 and not t[0].startswith(("prep", "dma")) else 0
        c40 = 2.6 * 40 + 5 * -(-40 // PL)
        c18 = 2.0 * 18 + 5 * -(-18 // PL)
        return dict(stage=130 * L, stats=140 * L, ln=395 * L, ucomb=4 * (c40 + 50) * L,
                    ends=5 * (37 * (L - 1) + 149), scan=5 * (82 * L + 4), hcomb=680 * L,
                    act=(4 * c40 + 170 + 330) * L, act_rest=(2 * c40 + 2 * c18 + 136 + 260) * L,
                    fin=2 * (2 * c40 + 195) * L, ysum=2 * (c40 + 140) * L, out=1, dma=1, coefs=600,
                    prep=8 * len(tables[t[-1]][0].used) if t[0] == "prep" else 0)[t[0]]

    def task_cycles(t, phase):
        L = Ls[t[1]] if len(t) > 1 and not t[0].startswith(("prep", "dma")) else 1
        alu, st = dict(stage=(30, 21), stats=(70, 8), ln=(154, 47), ucomb=(256, 60), ends=(205, 6),
                       scan=(280, 50), hcomb=(228, 92), act=(520, 67), act_rest=(375, 55), fin=(436, 60),
                       ysum=(208, 42), out=(0, 0), dma=(0, 0), coefs=(2500, 105), prep=dict(r1=(300, 60), d2=(950, 170)).get(t[-1], (1680, 255)))[t[0]]
        c = cap[phase[0] in "CD"]
        return max(L * alu / c[0], L * st / c[1], 1e-3)

    work = [[task_cycles(t, p) for p in phases] for t, _, _ in stream]
    cycles = [16 * Ls[p[1]] * (n_tiles(p) / 4 - tail) for p in phases]
    hi = [next((n for n, t in enumerate(stream) if phases.index(t[1]) > i), len(stream)) for i in range(len(phases))]
    lo = [max([n + 1 for n, t in enumerate(stream) if phases.index(t[2]) <= i], default=0) for i in range(len(phases))]
    target = [0.0] + _spread(cycles, work, lo, hi)

    def progress(i, x):
        u0, u1 = target[i], target[i + 1]
        knots = [u0] + list(range(int(u0) + 1, int(np.ceil(u1)))) + [u1]
        t = np.cumsum([0.0] + [(b - a) * work[int(a)][i] for a, b in zip(knots, knots[1:]) if b > a])
        return (float(np.interp(x * t[-1], t, knots[:len(t)])) if x < 1 else u1), t[-1] / cycles[i]

    if debug:
        for i, p in enumerate(phases):
            u = target[i + 1]
            print(p, "rate %.2f" % progress(i, 1)[1], lo[i], "%.2f" % u, hi[i], stream[min(int(u), len(stream) - 1)][0])

    def p_key(key):
        return ("C", key[1]) if key[0] in "CD" else key[:2] if key[0] == "B" else key

    p_set, busy = {}, []
    for i, p in enumerate(phases):
        k = p_key(p)
        if k not in p_set:
            user = dict(B=("ucomb",), R=("act_rest",), G=("act",), C=("fin",))[k[0]] + k[1:]
            end = next((phases.index(t[2]) for t in stream if t[0] == user), len(phases))
            p_set[k] = next((n for n, e in enumerate(busy) if e < i), len(busy))
            busy[p_set[k]:p_set[k] + 1] = [end]
    n_sets = len(busy)
    if debug:
        print('rate sets', n_sets)

    def kernel(x_hbm, lre_hbm, lim_hbm, bre_hbm, bim_hbm, cre_hbm, cim_hbm, ldt_hbm, dsk_hbm,
               wg_hbm, wu_hbm, wd_hbm, o_hbm, sc):
        in_sem, out_sem, zero_sem = sc["sem"]
        S, D = x_hbm.shape
        F = wg_hbm.shape[0]
        NL = D // LANE

        z = jnp.clip(pl.semaphore_read(zero_sem), 0, 1)

        class Buf:
            def __init__(self, ref):
                self.ref = ref
                if len(ref.shape) == 2:
                    n = 32 // ref.dtype.itemsize
                    end = ref.shape[0] - n
                    self.spare = ref.at[pl.ds(pl.multiple_of(end - n + n * z, n), n), pl.ds(0, LANE)]
                    self.zidx = (pl.ds(end, n), pl.ds(0, LANE))
                else:
                    self.spare = ref.at[ref.shape[0] - 2 + z, pl.ds(0, 8)]
                    self.zidx = (ref.shape[0] - 1, pl.ds(0, 8))
                self.ready = False

            def fence(self, v=None):
                v = jnp.zeros((8, LANE), F32) if v is None else v
                if self.ref.dtype == BF16:
                    v = pltpu.bitcast(v, BF16)
                elif self.ref.dtype != F32:
                    v = lax.bitcast_convert_type(v, self.ref.dtype)
                self.spare[...] = v

            def done(self):
                if not self.ready:
                    self.ref[self.zidx] = jnp.zeros((32 // self.ref.dtype.itemsize, LANE), self.ref.dtype)
                    self.ready = True
                self.fence()
                v = self.ref[self.zidx]
                return pltpu.bitcast(v, U32) if v.dtype == BF16 else lax.bitcast_convert_type(v, U32)

        bufs = jax.tree.map(Buf, sc["buf"])
        raw = bufs["raw"]
        xr = raw["x"]
        xl, hl, (dl,), (eb,), (cf,) = (bufs[k] for k in ("xl", "hl", "dl", "e", "coef"))
        xf, ub = bufs["xf"], bufs["u"]
        sb = bufs["s0"], bufs["s1"]
        hb = ub if inp_h else bufs["h"]
        of = bufs["of"] + xf

        def pbuf(key):
            return bufs["p%d" % p_set[p_key(key)]]

        copies, targets = {}, {}

        def copy(name, src, dst, target):
            targets[name] = target
            copies.setdefault(name, []).append(
                pltpu.make_async_copy(src, dst, in_sem.at[sum(map(len, copies.values()))]))

        def copy_rows(name, src, dst, r0, n):
            copy(name, src.at[pl.ds(r0, n)], dst.ref.at[pl.ds(r0, n)], dst)

        for b in range(NB):
            copy_rows("x%d" % b, x_hbm, xr, T0[b], 32 * Ls[b])
        for name, src in (("bre", bre_hbm), ("bim", bim_hbm), ("cre", cre_hbm), ("cim", cim_hbm)):
            copy_rows(name, src, raw[name], 0, D)
        for g in range(2):
            copy_rows("wg%d" % g, wg_hbm, raw["wg"], g * D, D)
            copy_rows("wu%d" % g, wu_hbm, raw["wu"], g * D, D)
        n = F - 2 * D
        for src, r0, rows, d0 in ((wg_hbm, 2 * D, n, 0), (wu_hbm, F - n % LANE, n % LANE, n),
                                  (wu_hbm, 2 * D, n - n % LANE, n + n % LANE)):
            copy("wr", src.at[pl.ds(r0, rows)], raw["wr"].ref.at[pl.ds(d0, rows)], raw["wr"])
        copy_rows("wd", wd_hbm, raw["wd"], 0, F)
        raw["wd"].ref[pl.ds(F, -F % LANE), :] = jnp.zeros((-F % LANE, D), BF16)
        for src, dst in zip((lre_hbm, lim_hbm, ldt_hbm, dsk_hbm), sc["vec"]):
            copy("vec", src, dst, cf)

        for kb in bufs["k"]:
            kb.ref[0] = jnp.full((8, LANE), 0.7978845608028654, F32)
            kb.ref[1] = jnp.full((8, LANE), 0.25, F32)

        pow_slot = {L: 6 + 8 * n for n, L in enumerate(sorted(set(Ls)))}

        def t_coefs():
            yield None, 600
            lre, lim, ldt, dsk = (_cat(*[v[:, LANE * c:LANE * c + LANE] for c in range(NL)])
                                  for v in (r[...].astype(F32).reshape(1, D) for r in sc["vec"]))
            dt = jnp.exp(ldt).astype(BF16).astype(F32)
            zr, zi = dt * lre, dt * lim
            mag = jnp.exp(zr)
            ar, ai = mag * jnp.cos(zi), mag * jnp.sin(zi)
            nr, ni = ar - 1.0, ai
            big = jnp.abs(lre) >= jnp.abs(lim)
            rat = jnp.where(big, lim / lre, lre / lim)
            den = jnp.where(big, lre + lim * rat, lre * rat + lim)
            qr = 2.0 * jnp.where(big, nr + ni * rat, nr * rat + ni) / den
            qi = 2.0 * jnp.where(big, ni - nr * rat, ni * rat - nr) / den
            consts = [ar, ai, dsk, qr, qi, -qr]
            for L in pow_slot:
                pr, pi, sr, si, n = None, None, ar, ai, L
                while n:
                    if n & 1:
                        pr, pi = (sr, si) if pr is None else _cmul(pr, pi, sr, si)
                    n >>= 1
                    if n:
                        sr, si = _cmul(sr, si, sr, si)
                for _ in range(4):
                    consts += [pr, pi]
                    pr, pi = _cmul(pr, pi, pr, pi)
            for n, v in enumerate(consts):
                for c in range(NL):
                    cf.ref[n * NL + c] = jnp.broadcast_to(v[c:c + 1], (8, LANE))
            yield cf, -4

        def coef(n, c, reps=1):
            v = cf.ref[n * NL + c]
            return v if reps == 1 else _cat(*[v] * reps)

        def t_prep(name):
            tab, src, row0, corner = tables[name]
            src, dest = raw[src], bufs["v"][name]
            for r0 in range(0, LANE, 16):
                env = {}
                for n, k in enumerate(tab.used):
                    if n % PW == 0:
                        yield src, min(PW, len(tab.used) - n)
                    row, col = corner(*k)
                    env[k] = 1, _split(pltpu.bitcast(src.ref[pl.ds(row0 + row + r0, 16), pl.ds(col, LANE)], U32))
                for n, (s, v) in enumerate(_run_slp(tab.slp, env, positive=True)):
                    dest.ref[n, pl.ds(r0 // 2, 8), :] = _pack(v if s > 0 else lax.neg(v))
                yield dest, None

        def weight_tile(name, i, j):
            _, src, row0, corner = tables[name]
            row, col = corner(i, j)
            return raw[src].ref[pl.ds(row0 + row, LANE), pl.ds(col, LANE)]

        def weight(name, p):
            tab = tables[name][0]
            if p in tab.single:
                return weight_tile(name, *tab.single[p])
            return _unpack(bufs["v"][name].ref[tab.summed.index(p)])

        def combos(key, q, t, v, slp=_OUT_SLP, order=_ORDER, sign=_SIGN, ncol=5):
            buf, n = pbuf(key)[q], len(order)
            tr = _Transposed(slp)
            for m, r in enumerate(order):
                if m % PL == 0:
                    yield buf, 5 + (2.6 if ncol == 5 else 2.0) * min(PL, n - m)
                tr.feed(r, buf.ref[t * _R + r, pl.ds(8 * v, 8), :], sign[r])
            return _columns(tr.adj, ncol)

        def lhs_store(slp, a1, a2, buf, q, slot):
            for n, v in enumerate(_lhs_combos(slp, a1, a2)):
                buf.ref[slot(n), pl.ds(8 * q, 8), :] = _pack(v)
            yield buf, None

        def in_rows(b, c, q, h):
            return [pl.ds((32 * c + h + 2 * t) * Ls[b] + q, 8, stride=4 * Ls[b]) for t in range(2)]

        def out_rows(b, c, q, v, h):
            return pl.ds((32 * c + 8 * (2 * h + v)) * Ls[b] + q, 8, stride=Ls[b])

        def load_in(buf, b, c, q, h):
            return _cat(*[buf[b].ref[s, :] for s in in_rows(b, c, q, h)])

        def t_stage(b):
            for r0 in range(0, 32 * Ls[b], 32):
                yield xr, 130
                for c in range(NL):
                    xf[b].ref[pl.ds(32 * Ls[b] * c + r0, 32), :] = (
                        xr.ref[pl.ds(T0[b] + r0, 32), pl.ds(LANE * c, LANE)].astype(F32))
                yield xf[b], None

        def t_stats(b, n):
            for q in range(Ls[b]):
                for h in range(2):
                    if n:
                        yield sb[0][b], 1
                    yield xf[b], 69 if n else 70
                    xv = [load_in(xf, b, c, q, h) for c in range(NL)]
                    if n:
                        mean = load_in(sb[0], b, 0, q, h)
                        xv = [lax.mul(d, d) for d in (lax.sub(v, mean) for v in xv)]
                    tot = xv[0]
                    for v in xv[1:]:
                        tot = lax.add(tot, v)
                    v = jnp.sum(tot, axis=-1, keepdims=True) * (1.0 / D)
                    v = jnp.broadcast_to(lax.rsqrt(v + 1e-5) if n else v, (16, LANE))
                    for s, part in zip(in_rows(b, 0, q, h), (_lo(v), _hi(v))):
                        sb[n][b].ref[s, :] = part
                if q % 4 == 3 or q == Ls[b] - 1:
                    yield sb[n][b], SS

        def t_ln(b):
            for q in range(Ls[b]):
                yield sb[0][b], 2
                yield sb[1][b], 3
                stats = [[load_in(sb[n], b, 0, q, h) for n in range(2)] for h in range(2)]
                halves = [[], []]
                for c in range(NL):
                    yield xf[b], (25, 25, 85, 115, 140)[c]
                    for h in range(2):
                        halves[h].append(lax.mul(lax.sub(load_in(xf, b, c, q, h), stats[h][0]), stats[h][1]))
                yield from lhs_store(_LHS_SLP, *halves, xl[b % 2], q, lambda r: r)

        def state(part, h, c):
            return (2 * part + h) * NL + c

        def t_ucomb(b):
            for q in range(Ls[b]):
                for part in range(2):
                    for v in range(2):
                        for h, cols in enumerate((yield from combos(("B", b), q, part, v))):
                            for c, val in enumerate(cols):
                                ub[q].ref[state(part, h, c), pl.ds(8 * v, 8), :] = val
                        yield ub[q], SU
                        yield None, 50

        carry = [None] * NL

        def t_ends(b):
            L = Ls[b]
            sub = lax.broadcasted_iota(jnp.int32, (8, LANE), 0)
            for c in range(NL):
                e = [None, None]
                for q in range(L):
                    yield ub[q], 37 if q else 9
                    if q == 0:
                        a = coef(0, c, 2), coef(1, c, 2)
                    for h in range(2):
                        u = ub[q].ref[state(0, h, c)], ub[q].ref[state(1, h, c)]
                        e[h] = _cmad(*a, *e[h], *u) if q else u
                pw = [(coef(pow_slot[L] + 2 * n, c), coef(pow_slot[L] + 2 * n + 1, c)) for n in range(4)]
                init = [[], []]
                for half in (_lo, _hi):
                    ev, od = [half(v) for v in e[0]], [half(v) for v in e[1]]
                    f = _cmad(*pw[0], *ev, *od)
                    if carry[c] is not None:
                        t = _cmul(*pw[1], *carry[c])
                        f = [lax.add(v, jnp.where(sub == 0, w, 0.0)) for v, w in zip(f, t)]
                    for n in range(3):
                        sh = [jnp.where(sub >= (1 << n), pltpu.roll(v, 1 << n, 0), 0.0) for v in f]
                        f = _cmad(*pw[n + 1], *sh, *f)
                    first = [jnp.where(sub == 0, 0.0 if carry[c] is None else carry[c][n], pltpu.roll(f[n], 1, 0))
                             for n in range(2)]
                    init[0].append(first)
                    init[1].append(_cmad(*pw[0], *first, *ev))
                    carry[c] = [jnp.broadcast_to(v[7:8], (8, LANE)) for v in f]
                for h in range(2):
                    for part in range(2):
                        eb.ref[state(part, h, c)] = _cat(init[h][0][part], init[h][1][part])
                yield None, 140
                yield eb, SE

        def t_scan(b):
            for c in range(NL):
                yield eb, 4
                a, (qr, qi, nqr) = (coef(0, c, 2), coef(1, c, 2)), (coef(n, c, 2) for n in (3, 4, 5))
                s = [(eb.ref[state(0, h, c)], eb.ref[state(1, h, c)]) for h in range(2)]
                for q in range(Ls[b]):
                    yield ub[q], 82
                    for h in range(2):
                        s[h] = _cmad(*a, *s[h], ub[q].ref[state(0, h, c)], ub[q].ref[state(1, h, c)])
                        hb[q].ref[state(0, h, c)] = lax.sub(lax.mul(qr, s[h][0]), lax.mul(qi, s[h][1]))
                        hb[q].ref[state(1, h, c)] = lax.sub(lax.mul(nqr, s[h][1]), lax.mul(qi, s[h][0]))
                    yield hb[q], SC

        def t_hcomb(b):
            for q in range(Ls[b]):
                for part in range(2):
                    hv = []
                    for c in range(NL):
                        yield hb[q], (20, 20, 75, 100, 125)[c]
                        c1, c2 = (hb[q].ref[state(part, h, c)] for h in range(2))
                        hv.append((_cat(_lo(c1), _lo(c2)), _cat(_hi(c1), _hi(c2))))
                    yield from lhs_store(_LHS_SLP, *zip(*hv), hl[b % 2], q, lambda r: part * _R + r)

        def gelu2(g, k):
            inner = lax.mul(g, lax.add(k, (0.7978845608028654 * 0.044715) * lax.mul(g, g)))
            return lax.add(g, lax.mul(g, lax.tanh(inner)))

        def t_act(b, g):
            kb = bufs["k"][4 * b + g]
            for q in range(Ls[b]):
                hm = [[], []]
                for v in range(2):
                    ga = yield from combos(("G", b, g), q, 0, v)
                    for c in range(NL):
                        yield kb, 17
                        k = kb.ref[0]
                        for h in range(2):
                            ga[h][c] = gelu2(ga[h][c], k)
                    up = yield from combos(("G", b, g), q, 1, v)
                    for c in range(NL):
                        hm[v].append(_cat(*[lax.mul(ga[h][c], up[h][c]) for h in range(2)]))
                yield from lhs_store(_LHS_SLP, *hm, dl, q, lambda r: g * _R + r)
                yield None, 330

        K4 = 2 * _R
        K4D = K4 + len(_NAMES_K4)

        def t_act_rest(b):
            kb = bufs["k"][4 * b + 2]
            lane = lax.broadcasted_iota(jnp.int32, (8, LANE), 1)
            for q in range(Ls[b]):
                hm = [[], []]
                for v in range(2):
                    ta = yield from combos(("R", b), q, 0, v)
                    for c in range(4):
                        yield kb, 17
                        k = kb.ref[0]
                        for h in range(2):
                            a = gelu2(ta[h][c], k)
                            if c == 3:
                                a = jnp.where(lane < LANE // 2, lax.mul(a, pltpu.roll(ta[h][c], LANE // 2, 1)), 0.0)
                            ta[h][c] = a
                    tb = yield from combos(("R", b), q, 1, v, _OUT_SLP_N2, _ORDER_N2, _SIGN_N2, 2)
                    for c in range(4):
                        hm[v].append(_cat(*[lax.mul(ta[h][c], (ta[h] + tb[h])[4 + c]) if c < 3 else ta[h][c]
                                            for h in range(2)]))
                for h in range(2):
                    for i in range(4):
                        dl.ref[K4D + 4 * h + i, pl.ds(8 * q, 8), :] = _pack(hm[h][i])
                yield from lhs_store(_LHS_SLP_K4, *hm, dl, q, lambda n: K4 + n)
                yield None, 260

        def ysum(b, q, v, emit):
            y = yield from combos(("C", b), q, 0, v)
            yield sb[0][b], 2
            yield sb[1][b], 3
            stats = [[sb[n][b].ref[out_rows(b, 0, q, v, h), :] for n in range(2)] for h in range(2)]
            for c in range(NL):
                yield xf[b], 27
                for h in range(2):
                    x = xf[b].ref[out_rows(b, c, q, v, h), :]
                    xn = lax.mul(lax.sub(x, stats[h][0]), stats[h][1])
                    emit(h, c, x, lax.add(y[h][c], lax.mul(xn, coef(2, c))))

        def t_ysum(b):
            for q in range(Ls[b]):
                for v in range(2):
                    def emit(h, c, x, s):
                        ub[q].ref[state(0, h, c), pl.ds(8 * v, 8), :] = s
                    yield from ysum(b, q, v, emit)
                    yield ub[q], None

        def t_fin(b, staged=False):
            kb = bufs["k"][4 * b + 3]
            for q in range(Ls[b]):
                for v in range(2):
                    g = yield from combos(("C", b), q, 1, v)
                    for c in range(NL):
                        yield kb, 11
                        k = kb.ref[1]
                        for h in range(2):
                            zz = lax.mul(k, g[h][c])
                            g[h][c] = lax.add(zz, lax.mul(zz, lax.tanh(zz)))

                    def emit(h, c, x, s):
                        of[b].ref[out_rows(b, c, q, v, h), :] = lax.add(x, lax.mul(s, g[h][c]))
                    if staged:
                        yield ub[q], 100
                        for c in range(NL):
                            for h in range(2):
                                emit(h, c, xf[b].ref[out_rows(b, c, q, v, h), :],
                                     ub[q].ref[state(0, h, c), pl.ds(8 * v, 8), :])
                    else:
                        yield from ysum(b, q, v, emit)
                    yield of[b], None

        out_copies = []

        def t_out(b):
            yield None, 1
            T = 32 * Ls[b]
            for c in range(NL):
                cp = pltpu.make_async_copy(of[b].ref.at[pl.ds(c * T, T)],
                                           o_hbm.at[pl.ds(T0[b], T), pl.ds(LANE * c, LANE)], out_sem.at[b * NL + c])
                cp.start()
                out_copies.append(cp)
            yield of[b], -2

        tasks = dict(coefs=t_coefs, ysum=t_ysum, stage=t_stage, stats=t_stats, ln=t_ln, ucomb=t_ucomb,
                     ends=t_ends, scan=t_scan, hcomb=t_hcomb, act=t_act, act_rest=t_act_rest, fin=t_fin,
                     out=t_out, dma=lambda *_: iter(()), prep=t_prep)

        def dots(key):
            kind, b = key[0], key[1]
            w = lambda *a: functools.partial(weight, *a)
            res = []
            for r, p in enumerate(_NAMES):
                if kind == "B":
                    ts = key[2:] or (0, 1)
                    res.append((xl[b % 2], [r], [w("b%d" % t, p) for t in ts], NT, [t * _R + r for t in ts]))
                elif kind == "G":
                    res.append((xl[b % 2], [r], [w(t + str(key[2]), p) for t in "gu"], NT, [r, _R + r]))
                elif kind == "R":
                    extra = [n for n, rr in enumerate(_N2_LHS) if rr == r]
                    res.append((xl[b % 2], [r], [w("r0", p)] + [w("r1", n) for n in extra], NT,
                                [r] + [_R + n for n in extra]))
                elif kind == "C":
                    res.append((hl[b % 2], [r, _R + r], [w("c0", p), w("c1", p)], NT, [r]))
                else:
                    lhs, rhs = [r, _R + r], [w("d0", p), w("d1", p)]
                    if p in _W_K4:
                        lhs.append(K4 + _NAMES_K4.index(p))
                        rhs.append(w("d2", p))
                    if p in _D4:
                        lhs += [K4D + 4 * _D4.index(p) + i for i in range(4)]
                        rhs += [functools.partial(weight_tile, "d2", i, 4) for i in range(4)]
                    res.append((dl, lhs, rhs, NN, [_R + r]))
            return res

        due = {}

        def items():
            for n, (t, _, _) in enumerate(stream):
                done, total = 0.0, task_cost(t)
                for buf, cost in tasks[t[0]](*t[1:]):
                    if cost is not None and cost >= 0:
                        yield buf, cost, n + done / total
                        done += cost
                    elif dead == 'all' or t[0] == "out" or t[0] in dead:
                        yield buf, cost, -1

        dma = [(n,) + t[1:] for n, (t, _, _) in enumerate(stream) if t[0] == "dma"]
        gen = items()
        st = dict(issued=0, item=next(gen, None), mark=None)

        def run_phase(key):
            L, n_phase = Ls[key[1]], phases.index(key)
            out = pbuf(key)
            first = st["issued"] // 4
            nslots = (n_tiles(key) / 4 - tail) * L
            released = first - 1
            todo, weights = dots(key), {}
            for nd, (lbuf, lhs, rhs, dims, dst) in enumerate(todo):
                tiles = []
                for n, slot in enumerate(lhs):
                    rnd = (st["issued"] + n) // 4
                    waits = {}
                    for k in [k for k in due if k[0] <= rnd]:
                        waits.setdefault(min(k[1], L - 1) if k[0] == rnd else 0, []).extend(due.pop(k))
                    if waits:
                        pieces = [lbuf.ref[slot, pl.ds(8 * q, 8), :] for q in range(L)]
                        for q, zs in waits.items():
                            for v in zs:
                                pieces[q] = lax.bitwise_or(pieces[q], v)
                        tiles.append(_cat(*pieces))
                    else:
                        tiles.append(lbuf.ref[slot, pl.ds(0, 8 * L), :])
                a = tiles[0] if len(tiles) == 1 else lax.concatenate(tiles, 1)
                w = weights.pop(nd, None) or [load() for load in rhs]
                w = w[0] if len(w) == 1 else lax.concatenate(w, 1 if (dims is NT and len(lhs) > 1) else 0)
                v = lax.dot_general(_unpack(a), w, dims, preferred_element_type=F32)
                st["issued"] += len(rhs)
                rnd = (st["issued"] - 1) // 4
                if rnd > released and dma and dma[0][0] < progress(n_phase, (rnd - first + 1) * L / nslots)[0]:
                    for n in range(nd + 1, min(nd + 3, len(todo))):
                        weights[n] = [load() for load in todo[n][2]]
                    _, waits, starts = dma.pop(0)
                    run_step(("wait",) + waits)
                    run_step(("start",) + starts)
                    for name in starts:
                        due.setdefault((rnd + 2, 0), []).append(targets[name].done())
                for n, slot in enumerate(dst):
                    for q in range(L):
                        out[q].ref[slot] = lax.slice(v, (16 * q, LANE * n), (16 * q + 16, LANE * n + LANE))
                if rnd == released:
                    continue
                released = rnd
                for q in range(L):
                    fenced = []
                    goal = progress(n_phase, ((rnd - first) * L + q + 1) / nslots)[0] - 1e-6
                    while st["item"] is not None and st["item"][2] < goal:
                        buf, cost, _ = st["item"]
                        if cost is None or cost < 0:
                            due.setdefault((rnd + 1 - (cost or 0) + (q + DL) // L, (q + DL) % L), []).append(buf.done())
                        else:
                            if buf is not None and buf not in fenced:
                                fenced.append(buf)
                                buf.fence(lax.slice(v, (16 * q, v.shape[1] - LANE), (16 * q + 8, v.shape[1])))
                        st["item"] = next(gen, None)
            assert st["item"] is None or st["item"][2] >= lo[n_phase] - 1e-6, (key, st["item"])

        def run_step(step):
            if step[0] in ("start", "wait"):
                for n in step[1:]:
                    for cp in copies[n]:
                        if not nodma:
                            cp.start() if step[0] == "start" else cp.wait()
            elif step[0] == "run":
                for t in step[1:]:
                    fenced, last = [], None
                    for buf, cost in tasks[t[0]](*t[1:]):
                        if cost is None or cost < 0:
                            last = buf
                        elif buf is not None and (RF or buf not in fenced):
                            fenced.append(buf)
                            buf.fence()
                    last.fence()
            else:
                run_phase(step)

        for n, step in enumerate(steps):
            if scopes:
                with jax.named_scope("s%02d_%s" % (n, "".join(map(str, step[:3] if step[0] in "BGRCD" else step[:1])))):
                    run_step(step)
            else:
                run_step(step)
        assert st["item"] is None
        if S != 2048:
            acc = jnp.zeros((8, LANE), F32)
            for k, v in bufs.items():
                if k[0] in "pv" or k in ("xl", "hl", "dl", "h", "u"):
                    for buf in (v.values() if k == "v" else v):
                        acc = acc + lax.bitcast_convert_type(buf.ref[z, pl.ds(0, 8), :], F32)
            of[0].ref[pl.ds(0, 8), :] = acc
            cp = pltpu.make_async_copy(of[0].ref.at[pl.ds(0, 8)], o_hbm.at[pl.ds(0, 8), pl.ds(0, LANE)], in_sem.at[0])
            cp.start()
            cp.wait()
        for cp in out_copies:
            cp.wait()

    def fn(A_x, A_Lambda_re, A_Lambda_im, A_B_re, A_B_im, A_C_re, A_C_im, A_log_dt, A_Dskip,
           B_x, B_w_gate, B_w_up, B_w_down):
        _, S, D = A_x.shape
        x = A_x.reshape(S, D)
        if S != 32 * sum(Ls):
            S = 32 * sum(Ls)
            x = x[:S]
        F = B_w_gate.shape[1]
        NL = D // LANE
        slots = lambda n, rows, dtype: pltpu.VMEM((n + 2, rows, LANE), dtype)
        blk = lambda n: [pltpu.VMEM((32 * L * n + 16, LANE), F32) for L in Ls]
        buf = dict(
            raw={k: pltpu.VMEM((n + 32, D), BF16) for k, n in dict(
                x=S, bre=D, bim=D, cre=D, cim=D, wg=2 * D, wu=2 * D, wr=2 * (F - 2 * D), wd=F + -F % LANE).items()},
            v={k: slots(len(t[0].summed), LANE // 2, U32) for k, t in tables.items()},
            xf=blk(NL), s0=blk(1), s1=blk(1), of=blk(NL)[:1], h=[] if inp_h else [slots(4 * NL, 16, F32)] * LM,
            xl=[slots(_R, 8 * LM, U32)] * 2, hl=[slots(2 * _R, 8 * LM, U32)] * 2,
            dl=[slots(2 * _R + len(_NAMES_K4) + 8, 8 * LM, U32)],
            u=[slots(4 * NL, 16, F32)] * LM, e=[slots(4 * NL, 16, F32)],
            k=[slots(2, 8, F32)] * (4 * NB), coef=[slots((6 + 8 * len(set(Ls))) * NL, 8, F32)],
        )
        for n in range(n_sets):
            buf["p%d" % n] = [slots(2 * _R, 16, F32)] * LM
        out = pl.pallas_call(
            kernel,
            in_specs=[pl.BlockSpec(memory_space=pl.ANY)] * 12,
            out_specs=pl.BlockSpec(memory_space=pl.ANY),
            out_shape=jax.ShapeDtypeStruct((S, D), F32),
            scratch_shapes=[dict(
                buf=buf, vec=[pltpu.VMEM((D,), BF16)] * 4,
                sem=[pltpu.SemaphoreType.DMA((15 + NB,)), pltpu.SemaphoreType.DMA((NB * NL,)),
                     pltpu.SemaphoreType.REGULAR],
            )],
            compiler_params=pltpu.CompilerParams(vmem_limit_bytes=126 * 2**20),
        )(x, A_Lambda_re, A_Lambda_im, A_B_re, A_B_im, A_C_re, A_C_im,
          A_log_dt, A_Dskip, B_w_gate.T, B_w_up.T, B_w_down)
        return out.reshape(1, S, D)
    return fn


@jax.jit
def pallas_recurrent_scan__ssm_conv_s5__geglu_ffn__prompt_kernel(
    A_x, A_Lambda_re, A_Lambda_im, A_B_re, A_B_im, A_C_re, A_C_im, A_log_dt, A_Dskip,
    B_x, B_w_gate, B_w_up, B_w_down,
):
    return build()(A_x, A_Lambda_re, A_Lambda_im, A_B_re, A_B_im, A_C_re, A_C_im, A_log_dt, A_Dskip,
                   B_x, B_w_gate, B_w_up, B_w_down)
```

```python
import functools

import numpy as np
import jax
import jax.numpy as jnp
from jax import lax
import jax.experimental.pallas as pl
import jax.experimental.pallas.tpu as pltpu

F32 = jnp.float32
BF16 = jnp.bfloat16
U32 = jnp.uint32
LANE = 128
NT = (((1,), (1,)), ((), ()))
NN = (((1,), (0,)), ((), ()))


def _acc(d, k, c):
    d[k] = d.get(k, 0) + c
    if d[k] == 0:
        del d[k]


class _HK:
    def __init__(self, methods, via):
        self.names, self.lhs, self.out = [], {}, {}
        n = len(methods)
        self.idx = [self._index(str(i), {i: 1}, {i: 1}, m) for i, m in enumerate(methods)]
        self.y, virt = {}, {}
        for i in range(n):
            self.y[i, i] = {self.idx[i][4]: 1, self.idx[i][5]: -1}
        for i in range(n):
            for j in range(n):
                if (methods[i] + 1) % 3 == methods[j]:
                    self.y[i, j], self.y[j, i], v = self._pair(self.idx[i], self.idx[j])
                    virt[i, j] = (v, 1)
                    virt[j, i] = (v, -1)
        for (i, j), l in via:
            v, sg = virt[j, l]
            if (methods[i] + 1) % 3 == v[3]:
                yiv, yvi, _ = self._pair(self.idx[i], v)
            else:
                yvi, yiv, _ = self._pair(v, self.idx[i])
            d = dict(yiv)
            for k, c in self.y[i, l].items():
                _acc(d, k, -c)
            self.y[i, j] = d
            d = {k: sg * c for k, c in yvi.items()}
            for k, c in self.y[l, i].items():
                _acc(d, k, c)
            self.y[j, i] = d
        assert len(self.y) == n * n

    def _prod(self, name, lhs, out):
        self.names.append(name)
        self.lhs[name], self.out[name] = lhs, out

    def _index(self, name, a, c, m):
        m1, m2 = (m + 1) % 3, (m + 2) % 3
        d1, d2 = name + ".1", name + ".2"
        self._prod(d1, {(i, m1): v for i, v in a.items()}, {(j, m2): v for j, v in c.items()})
        self._prod(d2, {(i, m2): v for i, v in a.items()}, {(j, m1): v for j, v in c.items()})
        return (name, a, c, m, d1, d2)

    def _pair(self, I, J):
        s = I[3]
        s1 = (s + 1) % 3
        assert s1 == J[3]
        a, c, lhs, out = dict(I[1]), dict(I[2]), {}, {}
        for k, v in J[1].items():
            _acc(a, k, -v)
        for k, v in J[2].items():
            _acc(c, k, v)
        V = self._index("(%s-%s)" % (I[0], J[0]), a, c, (s + 2) % 3)
        for k, v in I[1].items():
            _acc(lhs, (k, s1), v)
        for k, v in J[1].items():
            _acc(lhs, (k, s), v)
        for k, v in I[2].items():
            _acc(out, (k, s1), v)
        for k, v in J[2].items():
            _acc(out, (k, s), -v)
        sn = "S(%s,%s)" % (I[0], J[0])
        self._prod(sn, lhs, out)
        return ({sn: 1, V[4]: 1, I[5]: 1, J[5]: -1}, {sn: 1, V[5]: 1, I[4]: 1, J[4]: -1}, V)

    def weights(self, entries):
        w = {}
        for ij in entries:
            for p, c in self.y[ij].items():
                _acc(w.setdefault(p, {}), ij, c)
        return {p: d for p, d in w.items() if d}


def _slp(targets):
    ts = [dict(t) for t in targets]
    ops = []
    while any(len(t) > 1 for t in ts):
        cnt = {}
        for t in ts:
            ks = sorted(t, key=repr)
            for x in range(len(ks)):
                for y in range(x + 1, len(ks)):
                    key = (ks[x], ks[y], t[ks[x]] * t[ks[y]])
                    cnt[key] = cnt.get(key, 0) + 1
        a, b, sg = max(cnt, key=lambda k: cnt[k])
        new = ("t", len(ops))
        ops.append((new, a, b, sg))
        for t in ts:
            if a in t and b in t and t[a] * t[b] == sg:
                t[new] = t.pop(a)
                del t[b]
    return ops, [next(iter(t.items()))[::-1] for t in ts]


def _run_slp(slp, env, positive=False):
    ops, results = slp
    env = dict(env)
    inner = {v for _, a, b, _ in ops for v in (a, b)}
    want = {v: s for s, v in results if positive and v not in inner}
    for new, a, b, sg in ops:
        (sp, vp), (sq, vq) = env[a], env[b]
        sq = sq * sg
        if sp == sq:
            env[new] = sp, lax.add(vp, vq)
        else:
            s = want.get(new, 1)
            env[new] = s, (lax.sub(vp, vq) if sp == s else lax.sub(vq, vp))
    return [(s * env[v][0], env[v][1]) for s, v in results]


def _slp_signs(slp, env_signs):
    ops, results = slp
    env = dict(env_signs)
    for new, a, b, sg in ops:
        sp, sq = env[a], sg * env[b]
        env[new] = sp if sp == sq else 1
    return [s * env[v] for s, v in results]


class _Sum:
    def __init__(self, sign, value):
        self.terms = [(sign, value)]

    def get(self, sign):
        if len(self.terms) == 2:
            (sp, vp), (sq, vq) = self.terms
            if sp == sq:
                return sp, lax.add(vp, vq)
            return sign, (lax.sub(vp, vq) if sp == sign else lax.sub(vq, vp))
        return self.terms[0]

    def add(self, sign, value):
        self.terms = [self.get(-sign), (sign, value)]


class _Transposed:
    def __init__(self, slp, dry=False):
        ops, self.results = slp
        self.dry, self.adj = dry, {}
        self.split = {new: (a, b, sg) for new, a, b, sg in ops}
        self.pending = {}
        for v in [v for _, v in self.results] + [v for _, a, b, _ in ops for v in (a, b)]:
            self.pending[v] = self.pending.get(v, 0) + 1

    def put(self, v, sign, val):
        if v not in self.adj:
            self.adj[v] = _Sum(sign, val)
        elif not self.dry:
            self.adj[v].add(sign, val)
        self.pending[v] -= 1
        if self.pending[v] == 0 and v in self.split:
            a, b, sg = self.split[v]
            s, val = self.adj.pop(v).get(1)
            self.put(a, s, val)
            self.put(b, s * sg, val)

    def feed(self, t, val, sign=1):
        s, v = self.results[t]
        self.put(v, s * sign, val)


def _feed_order(slp):
    order, rest = [], list(range(len(slp[1])))

    def live(seq):
        tr = _Transposed(slp, dry=True)
        for t in seq:
            tr.feed(t, None)
        done = [j for j in range(5) if all(tr.pending.get((j, s), 0) == 0 for s in range(3))]
        return len(tr.adj) - len(done), sum(tr.pending.get((j, s), 0) ** 0.5 for j in range(5) for s in range(3))
    while rest:
        t = min(rest, key=lambda t: live(order + [t]))
        order.append(t)
        rest.remove(t)
    return order


_FORM_SIGN = (1, -1, 1)
_SCHEME = _HK((0, 0, 1, 1, 2), (((0, 1), 2), ((2, 3), 0)))
_NAMES = list(_SCHEME.names)
_R = len(_NAMES)
_LHS_SLP = _slp([_SCHEME.lhs[p] for p in _NAMES])
_OUT_SLP = _slp([_SCHEME.out[p] for p in _NAMES])
_LHS_SIGN = dict(zip(_NAMES, _slp_signs(_LHS_SLP, {(i, s): _FORM_SIGN[s] for i in range(5) for s in range(3)})))
_W_FULL = _SCHEME.weights([(i, j) for i in range(5) for j in range(5)])
_W_K4 = _SCHEME.weights([(i, j) for i in range(4) for j in range(4)])
_NAMES_K4 = [p for p in _NAMES if p in _W_K4]
_D4 = _SCHEME.idx[4][4], _SCHEME.idx[4][5]
_LHS_SLP_K4 = _slp([_SCHEME.lhs[p] for p in _NAMES_K4])
_LHS_SIGN_K4 = dict(zip(_NAMES_K4, _slp_signs(_LHS_SLP_K4, {(i, s): _FORM_SIGN[s] for i in range(4) for s in range(3)})))


def _n2_products():
    res = []
    for i, j in ((0, 2), (1, 3)):
        w = _SCHEME.weights([(i, i), (i, j), (j, i), (j, j)])
        col = {i: 0, j: 1}
        for p in _NAMES:
            if p in w:
                res.append((p, {(col[c], s): v for (c, s), v in _SCHEME.out[p].items()},
                            {(a, col[b]): v for (a, b), v in w[p].items()}))
    for c in range(2):
        res.append((_D4[0], {(c, 1): 1}, {(4, c): 1}))
        res.append((_D4[1], {(c, 0): 1}, {(4, c): -1}))
    return res


_N2 = _n2_products()
_OUT_SLP_N2 = _slp([o for _, o, _ in _N2])
_N2_LHS = [_NAMES.index(p) for p, _, _ in _N2]
assert all(_LHS_SIGN_K4[p] == _LHS_SIGN[p] for p in _NAMES_K4)


class _Weights:
    def __init__(self, w, lhs_sign):
        w = {p: {k: lhs_sign[p] * c for k, c in d.items()} for p, d in w.items()}
        self.single = {p: next(iter(d)) for p, d in w.items() if len(d) == 1}
        self.sign = {p: next(iter(d.values())) if len(d) == 1 else 1 for p, d in w.items()}
        self.summed = [p for p in lhs_sign if p in w and p not in self.single]
        self.slp = _slp([w[p] for p in self.summed])
        self.used = sorted({k for p in self.summed for k in w[p]})


_V_FULL, _V_K4 = _Weights(_W_FULL, _LHS_SIGN), _Weights(_W_K4, _LHS_SIGN)
_V_N2 = _Weights({n: w for n, (_, _, w) in enumerate(_N2)}, {n: _LHS_SIGN[p] for n, (p, _, _) in enumerate(_N2)})
assert all(_V_K4.sign[p] == _V_FULL.sign[p] for p in _NAMES_K4) and all(_V_FULL.sign[p] == 1 for p in _D4)
_SIGN, _SIGN_N2 = [_V_FULL.sign[p] for p in _NAMES], [_V_N2.sign[n] for n in range(len(_N2))]


def _lhs_combos(slp, a1, a2):
    env = {}
    for i, (x, y) in enumerate(zip(a1, a2)):
        env[i, 0] = (1, x)
        env[i, 1] = (-1, y)
        env[i, 2] = (1, lax.sub(y, x))
    return [v for _, v in _run_slp(slp, env)]


def _columns(acc, ncol):
    c1, c2 = [], []
    for j in range(ncol):
        s2, v2 = acc[j, 2].get(1)
        for form, dst in ((1, c1), (0, c2)):
            tot = _Sum(*acc[j, form].get(s2))
            tot.add(-s2, v2)
            s, v = tot.get(1)
            dst.append(v if s > 0 else lax.neg(v))
    return c1, c2


_ORDER, _ORDER_N2 = _feed_order(_OUT_SLP), _feed_order(_OUT_SLP_N2)


def _lo(v):
    return lax.slice_in_dim(v, 0, v.shape[0] // 2, axis=0)


def _hi(v):
    return lax.slice_in_dim(v, v.shape[0] // 2, v.shape[0], axis=0)


def _cat(*vs):
    return lax.concatenate(vs, 0)


def _pack(v):
    return lax.bitcast_convert_type(pltpu.pack_elementwise([_lo(v), _hi(v)], packed_dtype=BF16), U32)


def _split(w):
    return _cat(*[pltpu.unpack_elementwise(w, index=i, packed_dtype=BF16, unpacked_dtype=F32)
                  for i in range(2)])


def _unpack(v):
    return pltpu.bitcast(v, BF16)


def _cmul(ar, ai, br, bi):
    return lax.sub(lax.mul(ar, br), lax.mul(ai, bi)), lax.add(lax.mul(ar, bi), lax.mul(ai, br))


def _cmad(ar, ai, br, bi, cr, ci):
    tr, ti = _cmul(ar, ai, br, bi)
    return lax.add(tr, cr), lax.add(ti, ci)


def _subset(key):
    if key[0] == "b":
        single = key[3] == 0
        return _NAMES if key[3] is None else [p for p in _NAMES if (p in _V_FULL.single) == single]
    if key[0] == "d":
        return [p for p in _NAMES if min(j for j, _ in _SCHEME.out[p]) == key[2]]
    return _NAMES


def default_plan(NB):
    R, B, C, D = (lambda b, k=k: (k, b) for k in "RBCD")
    G = lambda b, g: ("G", b, g)
    ln = lambda b: [("stage", b), ("stats", b, 0), ("stats", b, 1), ("ln", b)]
    prep = lambda names, first, last: [(("prep", n), first, last) for n in names.split()]
    rest = tuple("x%d" % b for b in range(2, NB))
    b0, b1, b2 = ("b", 0, 0, 0), ("b", 0, 0, 1), ("b", 0, 1, None)
    steps = [("start", "vec", "x0", "bre", "bim", "wr", "wg0", "wu0", "x1", "wg1", "wu1", "wd", "cre", "cim") + rest,
             ("wait", "vec"), ("run", ("coefs",)), ("wait", "x0"), ("run", ("stage", 0), ("norm", 0)),
             ("wait", "bre"), b0, b1, b2, R(0), G(0, 0), G(0, 1), B(1), D(0)]
    tasks = prep("b0", b0, b0) + [(("dma", "bim"), b1, b1)] + prep("b1", b1, b1)
    tasks += [(("dma", "wr"), b2, b2)] + prep("r0 r1", b2, b2) + [(("ucomb", 0, 0, 0.4), R(0), R(0))]
    tasks += [(("dma", "wg0", "wu0", "x1"), R(0), R(0))] + prep("g0 u0", R(0), R(0))
    tasks += [(t, R(0), G(0, 1)) for t in ln(1)[:3]]
    tasks += [(("dma", "wg1", "wu1"), G(0, 0), G(0, 0))] + prep("g1 u1", G(0, 0), G(0, 0))
    tasks += [(("act_rest", 0), G(0, 0), G(0, 1)), (ln(1)[3], G(0, 0), G(0, 1)), (("act", 0, 0), G(0, 1), B(1)),
              (("dma", "wd", "cre", "cim") + rest, G(0, 1), B(1))]
    tasks += prep("d0 d1 d2", G(0, 1), B(1)) + [(("act", 0, 1), B(1), B(1))]
    tasks += [(("ucomb", 0, 0.4, 1), B(1), D(0)), (("ends", 0), B(1), R(1))] + prep("c0", B(1), R(1))
    tasks += [(("scan", 0), B(1), R(1))] + prep("c1", B(1), R(1)) + [(("hcomb", 0), B(1), R(1))]
    for b in range(1, NB):
        nxt = b + 1 < NB
        last = B(b + 1) if nxt else C(b)
        down = [D(b)] if nxt else [("d", b, c) for c in range(5)]
        steps += [R(b), C(b - 1), G(b, 0), G(b, 1), last] + down
        fin = lambda end: [((t, b - 1), G(b, 0), end) for t in ("fin", "out")]
        acts = [(("act", b, 0), G(b, 1), last), (("act", b, 1), last, last)]
        rest = [(("act_rest", b), C(b - 1), G(b, 1))]
        norm = [(t, D(b - 1), G(b, 1)) for t in ln(b + 1)] if nxt else []
        ssm = [((t, b), D(b - 1), R(b + 1) if nxt else G(b, 1)) for t in ("ends", "scan", "hcomb")]
        tasks += (norm[:2] if b == 1 else []) + [(("ucomb", b), D(b - 1), C(b - 1))] + (norm[2:3] if b == 1 else [])
        if b + 2 < NB:
            ahead = [(t, D(b), G(b + 1, 1)) for t in ln(b + 2)]
            tasks += rest + norm[3:] + fin(down[0]) + acts + ssm[:1] + ahead[:2] + ssm[1:2] + ahead[2:3] + ssm[2:]
        elif nxt:
            tasks += rest + norm[3:] + fin(down[0]) + acts + ssm
        else:
            tasks += ssm[:1] + rest + ssm[1:] + fin(last) + acts + [(("ysum", b), down[0], down[0])]
            tasks += [(("column", b, c), down[c + 1], down[-1]) for c in range(4)]
            steps += [("run", ("column", b, 4))]
    return steps, tasks


def _spread(cycles, work, lo, hi):
    def run(load, p0, p1, u):
        ends, idle = [], []
        for p in range(p0, p1):
            left = load * cycles[p]
            while u < hi[p] and left > 0:
                need = (int(u) + 1 - u) * work[int(u)][p]
                u, left = (int(u) + 1, left - need) if need <= left else (u + left / work[int(u)][p], 0)
            ends.append(u)
            idle.append(left > 0)
        return ends, idle

    def solve(p0, p1, u, last):
        if p0 == p1:
            return []
        need = lo[p0:p1 - 1] + [max(lo[p1 - 1], last)]
        a, b = 0.0, 8.0
        for _ in range(40):
            m = (a + b) / 2
            a, b = (a, m) if all(e >= n for e, n in zip(run(m, p0, p1, u)[0], need)) else (m, b)
        j = next((p0 + k for k, (e, n) in enumerate(zip(run(a, p0, p1, u)[0], need)) if e < n), p1 - 1)
        ends, idle = run(b, p0, j + 1, u)
        i = max([p0 + k + 1 for k in range(j - p0) if idle[k]], default=p0)
        ends[-1] = max(need[j - p0], u)
        return solve(p0, i, u, hi[i - 1]) + ends[i - p0:] + solve(j + 1, p1, ends[-1], last)

    return solve(0, len(cycles), 0.0, 0)


def build(Ls=(17, 17, 17, 13), nodma=0, debug=0, scopes=0, tail=0.5, PL=10, PW=9, DW=17, AV=560, AG=0, LG=60, KF=1, HS=0, HD=0, DS=40, free=(), TW=100, TR=100, TU=50, KW=17, RF=2, SQ=1,
          inp_h=1, inp_o=0, SP=None, SE=-2, SS=-1, SU=-1, squeeze=None, SC=None, WCH=16,
          cap=((2.6, 0.33), (2.4, 0.55)), plan=None):
    NB = len(Ls)
    LM = max(Ls)
    T0 = [32 * sum(Ls[:b]) for b in range(NB)]
    steps, stream = plan(NB) if callable(plan) else plan or default_plan(NB)
    phases = [s for s in steps if s[0] in tuple("BGRCDbd")]

    def n_tiles(key):
        if key[0] in "Dd":
            return sum(2 + (p in _W_K4) + 4 * (p in _D4) for p in _subset(key))
        return dict(B=2 * _R, G=2 * _R, R=_R + len(_N2), C=2 * _R, b=len(_subset(key)))[key[0]]

    def span(t):
        L = Ls[t[1]]
        return range(round(t[2] * L), round(t[3] * L)) if t[0] == "ucomb" and len(t) > 2 else range(L)

    nt = lambda i, j: (LANE * j, LANE * i)
    nn = lambda i, j: (LANE * i, LANE * j)
    tables = dict(b0=(_V_FULL, "bre", 0, nt), b1=(_V_FULL, "bim", 0, nt),
                  c0=(_V_FULL, "cre", 0, nt), c1=(_V_FULL, "cim", 0, nt),
                  g0=(_V_FULL, "wg", 0, nt), u0=(_V_FULL, "wu", 0, nt),
                  g1=(_V_FULL, "wg", 5 * LANE, nt), u1=(_V_FULL, "wu", 5 * LANE, nt),
                  r0=(_V_FULL, "wr", 0, nt), r1=(_V_N2, "wr", 5 * LANE, nt),
                  d0=(_V_FULL, "wd", 0, nn), d1=(_V_FULL, "wd", 5 * LANE, nn), d2=(_V_K4, "wd", 10 * LANE, nn))

    def task_cost(t):
        L = len(span(t)) if len(t) > 1 and not t[0].startswith(("prep", "dma")) else 0
        c40 = 2.6 * 40 + 5 * -(-40 // PL)
        c18 = 2.0 * 18 + 5 * -(-18 // PL)
        return dict(stage=130 * L, stats=140 * L, ln=(395 + 3 * LG) * L, ucomb=4 * (c40 + TU) * L,
                    ends=5 * (37 * (L - 1) + 149), scan=5 * (82 * L + 4), hcomb=(680 + 6 * LG) * L,
                    act=(4 * c40 + 10 * KW + TW + 3 * AG) * L, act_rest=(2 * c40 + 2 * c18 + 8 * KW + TR + 2 * AG) * L,
                    fin=2 * (2 * c40 + 195) * L, ysum=2 * (c40 + 140) * L, out=1, dma=1, column=6 * L + 1, coefs=600,
                    prep=8 * len(tables[t[-1]][0].used) if t[0] == "prep" else 0)[t[0]]

    def task_cycles(t, phase):
        L = len(span(t)) if len(t) > 1 and not t[0].startswith(("prep", "dma")) else 1
        alu, st = dict(stage=(30, 21), stats=(70, 8), ln=(154, 47), ucomb=(350, 48), ends=(205, 6),
                       scan=(280, 50), hcomb=(228, 92), act=(AV, 67), act_rest=(375, 55), fin=(470, 60),
                       ysum=(208, 42), out=(0, 0), dma=(0, 0), column=(90, 12), coefs=(2500, 105), prep=dict(r1=(300, 60), d2=(950, 170)).get(t[-1], (1680, 255)))[t[0]]
        c = cap[phase[0] in "CDd"]
        return max(L * alu / c[0], L * st / c[1], 1e-3)

    work = [[task_cycles(t, p) for p in phases] for t, _, _ in stream]
    rounds = lambda p: max(n_tiles(p) / 4 - tail, 1.0)
    cycles = [16 * Ls[p[1]] * rounds(p) for p in phases]
    hi = [next((n for n, t in enumerate(stream) if phases.index(t[1]) > i), len(stream)) for i in range(len(phases))]
    lo = [max([n + 1 for n, t in enumerate(stream) if phases.index(t[2]) <= i], default=0) for i in range(len(phases))]
    target = [0.0] + _spread(cycles, work, lo, hi)

    def progress(i, x):
        u0, u1 = target[i], target[i + 1]
        knots = [u0] + list(range(int(u0) + 1, int(np.ceil(u1)))) + [u1]
        t = np.cumsum([0.0] + [(b - a) * work[int(a)][i] for a, b in zip(knots, knots[1:]) if b > a])
        return (float(np.interp(x * t[-1], t, knots[:len(t)])) if x < 1 else u1), t[-1] / cycles[i]

    if debug:
        for i, p in enumerate(phases):
            u = target[i + 1]
            print(p, "rate %.2f" % progress(i, 1)[1], lo[i], "%.2f" % u, hi[i], stream[min(int(u), len(stream) - 1)][0])

    def p_key(key):
        return ("C", key[1]) if key[0] in "CDd" else ("B", key[1]) if key[0] == "b" else key

    p_set, busy = {}, []
    for i, p in enumerate(phases):
        k = p_key(p)
        if k not in p_set:
            user = dict(B=("ucomb",), R=("act_rest",), G=("act",), C=("fin",))[k[0]] + k[1:]
            end = max((phases.index(t[2]) for t in stream if t[0][:len(user)] == user), default=len(phases))
            p_set[k] = next((n for n, e in enumerate(busy) if e < i), len(busy))
            busy[p_set[k]:p_set[k] + 1] = [end]
    n_sets = len(busy)
    if debug:
        print('rate sets', n_sets)

    def kernel(x_hbm, lre_hbm, lim_hbm, bre_hbm, bim_hbm, cre_hbm, cim_hbm, ldt_hbm, dsk_hbm,
               wg_hbm, wu_hbm, wd_hbm, o_hbm, sc):
        in_sem, out_sem, zero_sem = sc["sem"]
        S, D = x_hbm.shape
        F = wg_hbm.shape[0]
        NL = D // LANE

        z = jnp.clip(pl.semaphore_read(zero_sem), 0, 1)

        class Buf:
            def __init__(self, ref):
                self.ref = ref
                if len(ref.shape) == 2:
                    n = 32 // ref.dtype.itemsize
                    end = ref.shape[0] - n
                    self.spare = ref.at[pl.ds(pl.multiple_of(end - n + n * z, n), n), pl.ds(0, LANE)]
                    self.zidx = (pl.ds(end, n), pl.ds(0, LANE))
                else:
                    self.spare = ref.at[ref.shape[0] - 2 + z, pl.ds(0, 8)]
                    self.zidx = (ref.shape[0] - 1, pl.ds(0, 8))
                self.ready = False

            def fence(self, v=None):
                v = jnp.zeros((8, LANE), F32) if v is None else v
                if self.ref.dtype == BF16:
                    v = pltpu.bitcast(v, BF16)
                elif self.ref.dtype != F32:
                    v = lax.bitcast_convert_type(v, self.ref.dtype)
                self.spare[...] = v

            def done(self):
                if not self.ready:
                    self.ref[self.zidx] = jnp.zeros((32 // self.ref.dtype.itemsize, LANE), self.ref.dtype)
                    self.ready = True
                self.fence()
                v = self.ref[self.zidx]
                return pltpu.bitcast(v, U32) if v.dtype == BF16 else lax.bitcast_convert_type(v, U32)

        bufs = jax.tree.map(Buf, sc["buf"])
        raw = bufs["raw"]
        xr = raw["x"]
        xl, hl, (dl,), (eb,), (cf,) = (bufs[k] for k in ("xl", "hl", "dl", "e", "coef"))
        xf, ub = bufs["xf"], bufs["u"]
        sb = bufs["s0"], bufs["s1"]
        hb = ub if inp_h else bufs["h"]
        of = bufs["of"]

        def pbuf(key):
            return bufs["p%d" % p_set[p_key(key)]]

        copies, targets = {}, {}

        def copy(name, src, dst, target):
            targets[name] = target
            copies.setdefault(name, []).append(
                pltpu.make_async_copy(src, dst, in_sem.at[sum(map(len, copies.values()))]))

        def copy_rows(name, src, dst, r0, n):
            copy(name, src.at[pl.ds(r0, n)], dst.ref.at[pl.ds(r0, n)], dst)

        for b in range(NB):
            copy_rows("x%d" % b, x_hbm, xr, T0[b], 32 * Ls[b])
        for name, src in (("bre", bre_hbm), ("bim", bim_hbm), ("cre", cre_hbm), ("cim", cim_hbm)):
            copy_rows(name, src, raw[name], 0, D)
        for g in range(2):
            copy_rows("wg%d" % g, wg_hbm, raw["wg"], g * D, D)
            copy_rows("wu%d" % g, wu_hbm, raw["wu"], g * D, D)
        n = F - 2 * D
        for src, r0, rows, d0 in ((wg_hbm, 2 * D, n, 0), (wu_hbm, F - n % LANE, n % LANE, n),
                                  (wu_hbm, 2 * D, n - n % LANE, n + n % LANE)):
            copy("wr", src.at[pl.ds(r0, rows)], raw["wr"].ref.at[pl.ds(d0, rows)], raw["wr"])
        copy_rows("wd", wd_hbm, raw["wd"], 0, F)
        raw["wd"].ref[pl.ds(F, -F % LANE), :] = jnp.zeros((-F % LANE, D), BF16)
        for src, dst in zip((lre_hbm, lim_hbm, ldt_hbm, dsk_hbm), sc["vec"]):
            copy("vec", src, dst, cf)

        for kb in bufs["k"]:
            kb.ref[0] = jnp.full((8, LANE), 0.7978845608028654, F32)
            kb.ref[1] = jnp.full((8, LANE), 0.25, F32)

        pow_slot = {L: 6 + 8 * n for n, L in enumerate(sorted(set(Ls)))}

        def t_coefs():
            yield None, 600
            lre, lim, ldt, dsk = (_cat(*[v[:, LANE * c:LANE * c + LANE] for c in range(NL)])
                                  for v in (r[...].astype(F32).reshape(1, D) for r in sc["vec"]))
            dt = jnp.exp(ldt).astype(BF16).astype(F32)
            zr, zi = dt * lre, dt * lim
            mag = jnp.exp(zr)
            ar, ai = mag * jnp.cos(zi), mag * jnp.sin(zi)
            nr, ni = ar - 1.0, ai
            big = jnp.abs(lre) >= jnp.abs(lim)
            rat = jnp.where(big, lim / lre, lre / lim)
            den = jnp.where(big, lre + lim * rat, lre * rat + lim)
            qr = 2.0 * jnp.where(big, nr + ni * rat, nr * rat + ni) / den
            qi = 2.0 * jnp.where(big, ni - nr * rat, ni * rat - nr) / den
            consts = [ar, ai, dsk, qr, qi, -qr]
            for L in pow_slot:
                pr, pi, sr, si, n = None, None, ar, ai, L
                while n:
                    if n & 1:
                        pr, pi = (sr, si) if pr is None else _cmul(pr, pi, sr, si)
                    n >>= 1
                    if n:
                        sr, si = _cmul(sr, si, sr, si)
                for _ in range(4):
                    consts += [pr, pi]
                    pr, pi = _cmul(pr, pi, pr, pi)
            for n, v in enumerate(consts):
                for c in range(NL):
                    cf.ref[n * NL + c] = jnp.broadcast_to(v[c:c + 1], (8, LANE))
            yield cf, -4

        def coef(n, c, reps=1):
            v = cf.ref[n * NL + c]
            return v if reps == 1 else _cat(*[v] * reps)

        def t_prep(name):
            tab, src, row0, corner = tables[name]
            src, dest = raw[src], bufs["v"][name]
            for r0 in range(0, LANE, 16):
                env = {}
                for n, k in enumerate(tab.used):
                    if n % PW == 0:
                        yield src, min(PW, len(tab.used) - n)
                    row, col = corner(*k)
                    env[k] = 1, _split(pltpu.bitcast(src.ref[pl.ds(row0 + row + r0, 16), pl.ds(col, LANE)], U32))
                for n, (s, v) in enumerate(_run_slp(tab.slp, env, positive=True)):
                    dest.ref[n, pl.ds(r0 // 2, 8), :] = _pack(v if s > 0 else lax.neg(v))
                yield dest, None

        def weight_tile(name, i, j):
            _, src, row0, corner = tables[name]
            row, col = corner(i, j)
            return raw[src].ref[pl.ds(row0 + row, LANE), pl.ds(col, LANE)]

        def weight(name, p):
            tab = tables[name][0]
            if p in tab.single:
                return weight_tile(name, *tab.single[p])
            return _unpack(bufs["v"][name].ref[tab.summed.index(p)])

        def combos(key, q, t, v, slp=_OUT_SLP, order=_ORDER, sign=_SIGN, ncol=5):
            buf, n = pbuf(key)[q], len(order)
            tr = _Transposed(slp)
            for m, r in enumerate(order):
                if m % PL == 0:
                    yield buf, 5 + (2.6 if ncol == 5 else 2.0) * min(PL, n - m)
                tr.feed(r, buf.ref[t * _R + r, pl.ds(8 * v, 8), :], sign[r])
            return _columns(tr.adj, ncol)

        def lhs_store(slp, names, a1, a2, buf, q, slot, gap=0):
            vals = _lhs_combos(slp, a1, a2)
            last = [max(2, *(i for i, _ in _SCHEME.lhs[p])) for p in names]
            for i in sorted(set(last)):
                for n, v in enumerate(vals):
                    if last[n] == i:
                        buf.ref[slot(n), pl.ds(8 * q, 8), :] = _pack(v)
                if gap or i == max(last):
                    yield buf, None
                    if gap:
                        yield None, gap

        def in_rows(b, c, q, h):
            return [pl.ds((32 * c + h + 2 * t) * Ls[b] + q, 8, stride=4 * Ls[b]) for t in range(2)]

        def out_rows(b, c, q, v, h):
            return pl.ds((32 * c + 8 * (2 * h + v)) * Ls[b] + q, 8, stride=Ls[b])

        def load_in(buf, b, c, q, h):
            return _cat(*[buf[b].ref[s, :] for s in in_rows(b, c, q, h)])

        def t_stage(b):
            for r0 in range(0, 32 * Ls[b], 32):
                yield xr, 130
                for c in range(NL):
                    xf[b].ref[pl.ds(32 * Ls[b] * c + r0, 32), :] = (
                        xr.ref[pl.ds(T0[b] + r0, 32), pl.ds(LANE * c, LANE)].astype(F32))
                yield xf[b], None

        def row_mean(tiles):
            tot = jnp.sum(functools.reduce(lax.add, tiles), axis=-1, keepdims=True) * (1.0 / D)
            return jnp.broadcast_to(tot, tiles[0].shape)

        def t_stats(b, n):
            for q in range(Ls[b]):
                for h in range(2):
                    if n:
                        yield sb[0][b], 1
                    yield xf[b], 69 if n else 70
                    xv = [load_in(xf, b, c, q, h) for c in range(NL)]
                    if n:
                        mean = load_in(sb[0], b, 0, q, h)
                        xv = [lax.mul(d, d) for d in (lax.sub(v, mean) for v in xv)]
                    v = lax.rsqrt(row_mean(xv) + 1e-5) if n else row_mean(xv)
                    for s, part in zip(in_rows(b, 0, q, h), (_lo(v), _hi(v))):
                        sb[n][b].ref[s, :] = part
                if q % SQ == SQ - 1 or q == Ls[b] - 1:
                    yield sb[n][b], SS

        def t_ln(b):
            for q in range(Ls[b]):
                yield sb[0][b], 2
                yield sb[1][b], 3
                stats = [[load_in(sb[n], b, 0, q, h) for n in range(2)] for h in range(2)]
                halves = [[], []]
                for c in range(NL):
                    yield xf[b], (25, 25, 85, 115, 140)[c]
                    for h in range(2):
                        halves[h].append(lax.mul(lax.sub(load_in(xf, b, c, q, h), stats[h][0]), stats[h][1]))
                yield from lhs_store(_LHS_SLP, _NAMES, *halves, xl[b % 2], q, lambda r: r, LG)

        def t_norm(b):
            yield xf[b], 1
            for q in range(Ls[b]):
                halves = []
                for h in range(2):
                    xv = [load_in(xf, b, c, q, h) for c in range(NL)]
                    mean = row_mean(xv)
                    xv = [lax.sub(v, mean) for v in xv]
                    rstd = lax.rsqrt(row_mean([lax.mul(d, d) for d in xv]) + 1e-5)
                    halves.append([lax.mul(d, rstd) for d in xv])
                    for n, v in enumerate((mean, rstd)):
                        for s, part in zip(in_rows(b, 0, q, h), (_lo(v), _hi(v))):
                            sb[n][b].ref[s, :] = part
                yield from lhs_store(_LHS_SLP, _NAMES, *halves, xl[b % 2], q, lambda r: r, LG)

        def state(part, h, c):
            return (2 * part + h) * NL + c

        def t_ucomb(b, *part):
            for q in span(("ucomb", b) + part):
                for t in range(2):
                    for v in range(2):
                        for h, cols in enumerate((yield from combos(("B", b), q, t, v))):
                            for c, val in enumerate(cols):
                                ub[q].ref[state(t, h, c), pl.ds(8 * v, 8), :] = val
                        yield ub[q], SU
                        yield None, TU

        carry = [None] * NL

        def t_ends(b):
            L = Ls[b]
            sub = lax.broadcasted_iota(jnp.int32, (8, LANE), 0)
            for c in range(NL):
                e = [None, None]
                for q in range(L):
                    yield ub[q], 37 if q else 9
                    if q == 0:
                        a = coef(0, c, 2), coef(1, c, 2)
                    for h in range(2):
                        u = ub[q].ref[state(0, h, c)], ub[q].ref[state(1, h, c)]
                        e[h] = _cmad(*a, *e[h], *u) if q else u
                pw = [(coef(pow_slot[L] + 2 * n, c), coef(pow_slot[L] + 2 * n + 1, c)) for n in range(4)]
                init = [[], []]
                for half in (_lo, _hi):
                    ev, od = [half(v) for v in e[0]], [half(v) for v in e[1]]
                    f = _cmad(*pw[0], *ev, *od)
                    if carry[c] is not None:
                        t = _cmul(*pw[1], *carry[c])
                        f = [lax.add(v, jnp.where(sub == 0, w, 0.0)) for v, w in zip(f, t)]
                    for n in range(3):
                        sh = [jnp.where(sub >= (1 << n), pltpu.roll(v, 1 << n, 0), 0.0) for v in f]
                        f = _cmad(*pw[n + 1], *sh, *f)
                    first = [jnp.where(sub == 0, 0.0 if carry[c] is None else carry[c][n], pltpu.roll(f[n], 1, 0))
                             for n in range(2)]
                    init[0].append(first)
                    init[1].append(_cmad(*pw[0], *first, *ev))
                    carry[c] = [jnp.broadcast_to(v[7:8], (8, LANE)) for v in f]
                for h in range(2):
                    for part in range(2):
                        eb.ref[state(part, h, c)] = _cat(init[h][0][part], init[h][1][part])
                yield None, 140
                yield eb, SE

        def t_scan(b):
            for c in range(NL):
                yield eb, 4
                a, (qr, qi, nqr) = (coef(0, c, 2), coef(1, c, 2)), (coef(n, c, 2) for n in (3, 4, 5))
                s = [(eb.ref[state(0, h, c)], eb.ref[state(1, h, c)]) for h in range(2)]
                for q in range(Ls[b]):
                    yield ub[q], 82
                    for h in range(2):
                        s[h] = _cmad(*a, *s[h], ub[q].ref[state(0, h, c)], ub[q].ref[state(1, h, c)])
                        hb[q].ref[state(0, h, c)] = lax.sub(lax.mul(qr, s[h][0]), lax.mul(qi, s[h][1]))
                        hb[q].ref[state(1, h, c)] = lax.sub(lax.mul(nqr, s[h][1]), lax.mul(qi, s[h][0]))
                    yield hb[q], SC

        def t_hcomb(b):
            for q in range(Ls[b]):
                for part in range(2):
                    hv = []
                    for c in range(NL):
                        yield hb[q], (20, 20, 75, 100, 125)[c]
                        c1, c2 = (hb[q].ref[state(part, h, c)] for h in range(2))
                        hv.append((_cat(_lo(c1), _lo(c2)), _cat(_hi(c1), _hi(c2))))
                    yield from lhs_store(_LHS_SLP, _NAMES, *zip(*hv), hl[b % 2], q, lambda r: part * _R + r, LG)

        def gelu2(g, k):
            inner = lax.mul(g, lax.add(k, (0.7978845608028654 * 0.044715) * lax.mul(g, g)))
            return lax.add(g, lax.mul(g, lax.tanh(inner)))

        def t_act(b, g):
            kb, tb = bufs["k"][4 * b + g], bufs["t"][2 * b + g]
            for q in range(Ls[b]):
                hm = [[], []]
                for v in range(2):
                    ga = yield from combos(("G", b, g), q, 0, v)
                    for c in range(NL):
                        if KF == 1 or (KF == 2 and c == 0):
                            yield kb, KW * (1 if KF == 1 else NL)
                            k = kb.ref[0]
                        elif KF == 0:
                            yield None, KW
                            k = jnp.full((8, LANE), 0.7978845608028654, F32)
                        for h in range(2):
                            ga[h][c] = gelu2(ga[h][c], k)
                    up = yield from combos(("G", b, g), q, 1, v)
                    for c in range(NL):
                        hm[v].append(_cat(*[lax.mul(ga[h][c], up[h][c]) for h in range(2)]))
                        if v < HS:
                            tb.ref[(2 * (q % 2) + v) * NL + c] = hm[v][c]
                    if v < HS and HD:
                        yield tb, None
                if HS:
                    yield tb, 0
                    for v in range(HS):
                        hm[v] = [tb.ref[(2 * (q % 2) + v) * NL + c] for c in range(NL)]
                yield from lhs_store(_LHS_SLP, _NAMES, *hm, dl, q, lambda r: g * _R + r, AG)
                yield None, TW

        K4 = 2 * _R
        K4D = K4 + len(_NAMES_K4)

        def t_act_rest(b):
            kb = bufs["k"][4 * b + 2]
            lane = lax.broadcasted_iota(jnp.int32, (8, LANE), 1)
            for q in range(Ls[b]):
                hm = [[], []]
                for v in range(2):
                    ta = yield from combos(("R", b), q, 0, v)
                    for c in range(4):
                        yield kb, KW
                        k = kb.ref[0]
                        for h in range(2):
                            a = gelu2(ta[h][c], k)
                            if c == 3:
                                a = jnp.where(lane < LANE // 2, lax.mul(a, pltpu.roll(ta[h][c], LANE // 2, 1)), 0.0)
                            ta[h][c] = a
                    tb = yield from combos(("R", b), q, 1, v, _OUT_SLP_N2, _ORDER_N2, _SIGN_N2, 2)
                    for c in range(4):
                        hm[v].append(_cat(*[lax.mul(ta[h][c], (ta[h] + tb[h])[4 + c]) if c < 3 else ta[h][c]
                                            for h in range(2)]))
                for h in range(2):
                    for i in range(4):
                        dl.ref[K4D + 4 * h + i, pl.ds(8 * q, 8), :] = _pack(hm[h][i])
                yield from lhs_store(_LHS_SLP_K4, _NAMES_K4, *hm, dl, q, lambda n: K4 + n, AG)
                yield None, TR

        def ysum(b, q, v, emit):
            y = yield from combos(("C", b), q, 0, v)
            yield sb[0][b], 2
            yield sb[1][b], 3
            stats = [[sb[n][b].ref[out_rows(b, 0, q, v, h), :] for n in range(2)] for h in range(2)]
            for c in range(NL):
                yield xf[b], 27
                for h in range(2):
                    x = xf[b].ref[out_rows(b, c, q, v, h), :]
                    xn = lax.mul(lax.sub(x, stats[h][0]), stats[h][1])
                    emit(h, c, x, lax.add(y[h][c], lax.mul(xn, coef(2, c))))

        def t_ysum(b):
            for q in range(Ls[b]):
                for v in range(2):
                    def emit(h, c, x, s):
                        ub[q].ref[state(0, h, c), pl.ds(8 * v, 8), :] = s
                    yield from ysum(b, q, v, emit)
                    yield ub[q], None

        def silu(d, k):
            zz = lax.mul(k, d)
            return lax.add(zz, lax.mul(zz, lax.tanh(zz)))

        def t_fin(b):
            kb = bufs["k"][4 * b + 3]
            for q in range(Ls[b]):
                for v in range(2):
                    g = yield from combos(("C", b), q, 1, v)
                    for c in range(NL):
                        yield kb, 11
                        k = kb.ref[1]
                        for h in range(2):
                            g[h][c] = silu(g[h][c], k)

                    def emit(h, c, x, s):
                        of[b].ref[out_rows(b, c, q, v, h), :] = lax.add(x, lax.mul(s, g[h][c]))
                    yield from ysum(b, q, v, emit)
                    yield of[b], None

        out_copies = []

        def write_out(b, c, src):
            T = 32 * Ls[b]
            cp = pltpu.make_async_copy(src, o_hbm.at[pl.ds(T0[b], T), pl.ds(LANE * c, LANE)], out_sem.at[b * NL + c])
            cp.start()
            out_copies.append(cp)

        def t_out(b):
            yield None, 1
            for c in range(NL):
                write_out(b, c, of[b].ref.at[pl.ds(32 * Ls[b] * c, 32 * Ls[b])])
            yield of[b], -2

        def t_column(b, c):
            kb, dest = bufs["k"][4 * b + 3], bufs["oc"][c]
            terms = sorted((s, r, sign * _SIGN[r]) for r, p in enumerate(_NAMES)
                           for (j, s), sign in _SCHEME.out[p].items() if j == c)
            for q in range(Ls[b]):
                buf = pbuf(("C", b))[q]
                yield buf, 3
                acc = {}
                for s, r, sign in terms:
                    val = buf.ref[_R + r]
                    if (0, s) in acc:
                        acc[0, s].add(sign, val)
                    else:
                        acc[0, s] = _Sum(sign, val)
                yield kb, 1
                k = _cat(*[kb.ref[1]] * 2)
                g = [silu(d[0], k) for d in _columns(acc, 1)]
                yield ub[q], 2
                for h in range(2):
                    res = lax.mul(ub[q].ref[state(0, h, c)], g[h])
                    for v, part in enumerate((_lo(res), _hi(res))):
                        dest.ref[out_rows(b, 0, q, v, h), :] = lax.add(xf[b].ref[out_rows(b, c, q, v, h), :], part)
                yield dest, None
            yield None, 1
            write_out(b, c, dest.ref.at[pl.ds(0, 32 * Ls[b])])
            yield dest, None

        tasks = dict(column=t_column, norm=t_norm, coefs=t_coefs, ysum=t_ysum, stage=t_stage, stats=t_stats, ln=t_ln, ucomb=t_ucomb,
                     ends=t_ends, scan=t_scan, hcomb=t_hcomb, act=t_act, act_rest=t_act_rest, fin=t_fin,
                     out=t_out, dma=lambda *_: iter(()), prep=t_prep)

        def dots(key):
            kind, b = key[0], key[1]
            w = lambda *a: functools.partial(weight, *a)
            res = []
            for p in _subset(key):
                r = _NAMES.index(p)
                if kind in "Bb":
                    ts = key[2:3] or (0, 1)
                    res.append((xl[b % 2], [r], [w("b%d" % t, p) for t in ts], NT, [t * _R + r for t in ts]))
                elif kind == "G":
                    res.append((xl[b % 2], [r], [w(t + str(key[2]), p) for t in "gu"], NT, [r, _R + r]))
                elif kind == "R":
                    extra = [n for n, rr in enumerate(_N2_LHS) if rr == r]
                    res.append((xl[b % 2], [r], [w("r0", p)] + [w("r1", n) for n in extra], NT,
                                [r] + [_R + n for n in extra]))
                elif kind == "C":
                    res.append((hl[b % 2], [r, _R + r], [w("c0", p), w("c1", p)], NT, [r]))
                else:
                    lhs, rhs = [r, _R + r], [w("d0", p), w("d1", p)]
                    if p in _W_K4:
                        lhs.append(K4 + _NAMES_K4.index(p))
                        rhs.append(w("d2", p))
                    if p in _D4:
                        for i in (0, 2):
                            res.append((dl, lhs, rhs, NN, None))
                            lhs = [K4D + 4 * _D4.index(p) + i + t for t in range(2)]
                            rhs = [functools.partial(weight_tile, "d2", i + t, 4) for t in range(2)]
                    res.append((dl, lhs, rhs, NN, [_R + r]))
            return res

        due = {}

        def items():
            for n, (t, _, _) in enumerate(stream):
                done, total = 0.0, task_cost(t)
                for buf, cost in tasks[t[0]](*t[1:]):
                    if cost is not None and cost >= 0:
                        yield buf, cost, n + done / total
                        done += cost
                    elif t[0] not in free:
                        yield buf, cost, -1

        dma = [(n, t[1:]) for n, (t, _, _) in enumerate(stream) if t[0] == "dma"]
        gen = items()
        st = dict(issued=0, item=next(gen, None), mark=None)

        def run_phase(key):
            L, n_phase = Ls[key[1]], phases.index(key)
            out = pbuf(key)
            first = st["issued"] // 4
            nslots = rounds(key) * L
            if squeeze and key in squeeze:
                nslots = squeeze[key] * L / 16
            released = first - 1
            todo, weights, part = dots(key), {}, None
            for nd, (lbuf, lhs, rhs, dims, dst) in enumerate(todo):
                tiles = []
                for n, slot in enumerate(lhs):
                    rnd = (st["issued"] + n) // 4
                    waits = {}
                    for k in [k for k in due if k[0] <= rnd]:
                        waits.setdefault(min(k[1], L - 1), []).extend(due.pop(k))
                    if waits:
                        pieces = [lbuf.ref[slot, pl.ds(8 * q, 8), :] for q in range(L)]
                        for q, zs in waits.items():
                            for v in zs:
                                pieces[q] = lax.bitwise_or(pieces[q], v)
                        tiles.append(_cat(*pieces))
                    else:
                        tiles.append(lbuf.ref[slot, pl.ds(0, 8 * L), :])
                a = tiles[0] if len(tiles) == 1 else lax.concatenate(tiles, 1)
                w = weights.pop(nd, None) or [load() for load in rhs]
                w = w[0] if len(w) == 1 else lax.concatenate(w, 1 if (dims is NT and len(lhs) > 1) else 0)
                v = lax.dot_general(_unpack(a), w, dims, preferred_element_type=F32)
                if part is not None:
                    v = lax.add(part, v)
                part = None if dst else v
                st["issued"] += len(rhs)
                rnd = (st["issued"] - 1) // 4
                if rnd > released and dma and dma[0][0] < progress(n_phase, (rnd - first + 1) * L / nslots)[0]:
                    for n in range(nd + 1, min(nd + 3, len(todo))):
                        weights[n] = [load() for load in todo[n][2]]
                    run_step(("wait",) + dma.pop(0)[1])
                for n, slot in enumerate(dst or ()):
                    for q in range(L):
                        out[q].ref[slot] = lax.slice(v, (16 * q, LANE * n), (16 * q + 16, LANE * n + LANE))
                if rnd == released:
                    continue
                released = rnd
                for q in range(L):
                    fenced = []
                    goal = progress(n_phase, ((rnd - first) * L + q + 1) / nslots)[0] - 1e-6
                    while st["item"] is not None and st["item"][2] < goal:
                        buf, cost, _ = st["item"]
                        if cost is None or cost < 0:
                            late = q + max(L, DW * (1 - (cost or 0)))
                            due.setdefault((rnd + late // L, late % L), []).append(buf.done())
                        else:
                            if buf is not None and buf not in fenced:
                                fenced.append(buf)
                                buf.fence(lax.slice(v, (16 * q, v.shape[1] - LANE), (16 * q + 8, v.shape[1])))
                        st["item"] = next(gen, None)
            while st["item"] is not None and st["item"][2] < lo[n_phase] - 1e-6:
                buf, cost, _ = st["item"]
                if buf is not None:
                    buf.fence(lax.slice(v, (16 * L - 8, v.shape[1] - LANE), (16 * L, v.shape[1])))
                st["item"] = next(gen, None)

        def run_step(step):
            if step[0] in ("start", "wait"):
                for n in step[1:]:
                    for cp in copies[n]:
                        if not nodma:
                            cp.start() if step[0] == "start" else cp.wait()
            elif step[0] == "run":
                for t in step[1:]:
                    fenced, last = [], None
                    for buf, cost in tasks[t[0]](*t[1:]):
                        if cost is None or cost < 0:
                            last = buf
                        elif buf is not None and buf not in fenced:
                            fenced.append(buf)
                            buf.fence()
                    last.fence()
            else:
                run_phase(step)

        for n, step in enumerate(steps):
            if scopes:
                with jax.named_scope("s%02d_%s" % (n, "".join(map(str, step[:4] if step in phases else step[:1])))):
                    run_step(step)
            else:
                run_step(step)
        assert st["item"] is None
        if S != 2048:
            acc = jnp.zeros((8, LANE), F32)
            for k, v in bufs.items():
                if k[0] in "pv" or k in ("xl", "hl", "dl", "h", "u"):
                    for buf in (v.values() if k == "v" else v):
                        acc = acc + lax.bitcast_convert_type(buf.ref[z, pl.ds(0, 8), :], F32)
            of[0].ref[pl.ds(0, 8), :] = acc
            cp = pltpu.make_async_copy(of[0].ref.at[pl.ds(0, 8)], o_hbm.at[pl.ds(0, 8), pl.ds(0, LANE)], in_sem.at[0])
            cp.start()
            cp.wait()
        for cp in out_copies:
            cp.wait()

    def fn(A_x, A_Lambda_re, A_Lambda_im, A_B_re, A_B_im, A_C_re, A_C_im, A_log_dt, A_Dskip,
           B_x, B_w_gate, B_w_up, B_w_down):
        _, S, D = A_x.shape
        x = A_x.reshape(S, D)
        if S != 32 * sum(Ls):
            S = 32 * sum(Ls)
            x = x[:S]
        F = B_w_gate.shape[1]
        NL = D // LANE
        slots = lambda n, rows, dtype: pltpu.VMEM((n + 2, rows, LANE), dtype)
        blk = lambda n: [pltpu.VMEM((32 * L * n + 16, LANE), F32) for L in Ls]
        buf = dict(
            raw={k: pltpu.VMEM((n + 32, D), BF16) for k, n in dict(
                x=S, bre=D, bim=D, cre=D, cim=D, wg=2 * D, wu=2 * D, wr=2 * (F - 2 * D), wd=F + -F % LANE).items()},
            v={k: slots(len(t[0].summed), LANE // 2, U32) for k, t in tables.items()},
            xf=blk(NL), s0=blk(1), s1=blk(1), of=blk(NL)[:-1], oc=blk(1)[-1:] * NL, h=[] if inp_h else [slots(4 * NL, 16, F32)] * LM,
            xl=[slots(_R, 8 * LM, U32)] * 2, hl=[slots(2 * _R, 8 * LM, U32)] * 2,
            dl=[slots(2 * _R + len(_NAMES_K4) + 8, 8 * LM, U32)],
            u=[slots(4 * NL, 16, F32)] * LM, e=[slots(4 * NL, 16, F32)],
            k=[slots(2, 8, F32)] * (4 * NB), t=[slots(4 * NL, 16, F32)] * (2 * NB), coef=[slots((6 + 8 * len(set(Ls))) * NL, 8, F32)],
        )
        for n in range(n_sets):
            buf["p%d" % n] = [slots(2 * _R, 16, F32)] * LM
        out = pl.pallas_call(
            kernel,
            in_specs=[pl.BlockSpec(memory_space=pl.ANY)] * 12,
            out_specs=pl.BlockSpec(memory_space=pl.ANY),
            out_shape=jax.ShapeDtypeStruct((S, D), F32),
            scratch_shapes=[dict(
                buf=buf, vec=[pltpu.VMEM((D,), BF16)] * 4,
                sem=[pltpu.SemaphoreType.DMA((15 + NB,)), pltpu.SemaphoreType.DMA((NB * NL,)),
                     pltpu.SemaphoreType.REGULAR],
            )],
            compiler_params=pltpu.CompilerParams(vmem_limit_bytes=126 * 2**20),
        )(x, A_Lambda_re, A_Lambda_im, A_B_re, A_B_im, A_C_re, A_C_im,
          A_log_dt, A_Dskip, B_w_gate.T, B_w_up.T, B_w_down)
        return out.reshape(1, S, D)
    return fn


@jax.jit
def pallas_recurrent_scan__ssm_conv_s5__geglu_ffn__prompt_kernel(
    A_x, A_Lambda_re, A_Lambda_im, A_B_re, A_B_im, A_C_re, A_C_im, A_log_dt, A_Dskip,
    B_x, B_w_gate, B_w_up, B_w_down,
):
    return build()(A_x, A_Lambda_re, A_Lambda_im, A_B_re, A_B_im, A_C_re, A_C_im, A_log_dt, A_Dskip,
                   B_x, B_w_gate, B_w_up, B_w_down)
```

```python
import functools

import numpy as np
import jax
import jax.numpy as jnp
from jax import lax
import jax.experimental.pallas as pl
import jax.experimental.pallas.tpu as pltpu

F32 = jnp.float32
BF16 = jnp.bfloat16
U32 = jnp.uint32
LANE = 128
NT = (((1,), (1,)), ((), ()))
NN = (((1,), (0,)), ((), ()))


def _acc(d, k, c):
    d[k] = d.get(k, 0) + c
    if d[k] == 0:
        del d[k]


class _HK:
    def __init__(self, methods, via):
        self.names, self.lhs, self.out = [], {}, {}
        n = len(methods)
        self.idx = [self._index(str(i), {i: 1}, {i: 1}, m) for i, m in enumerate(methods)]
        self.y, virt = {}, {}
        for i in range(n):
            self.y[i, i] = {self.idx[i][4]: 1, self.idx[i][5]: -1}
        for i in range(n):
            for j in range(n):
                if (methods[i] + 1) % 3 == methods[j]:
                    self.y[i, j], self.y[j, i], v = self._pair(self.idx[i], self.idx[j])
                    virt[i, j] = (v, 1)
                    virt[j, i] = (v, -1)
        for (i, j), l in via:
            v, sg = virt[j, l]
            if (methods[i] + 1) % 3 == v[3]:
                yiv, yvi, _ = self._pair(self.idx[i], v)
            else:
                yvi, yiv, _ = self._pair(v, self.idx[i])
            d = dict(yiv)
            for k, c in self.y[i, l].items():
                _acc(d, k, -c)
            self.y[i, j] = d
            d = {k: sg * c for k, c in yvi.items()}
            for k, c in self.y[l, i].items():
                _acc(d, k, c)
            self.y[j, i] = d
        assert len(self.y) == n * n

    def _prod(self, name, lhs, out):
        self.names.append(name)
        self.lhs[name], self.out[name] = lhs, out

    def _index(self, name, a, c, m):
        m1, m2 = (m + 1) % 3, (m + 2) % 3
        d1, d2 = name + ".1", name + ".2"
        self._prod(d1, {(i, m1): v for i, v in a.items()}, {(j, m2): v for j, v in c.items()})
        self._prod(d2, {(i, m2): v for i, v in a.items()}, {(j, m1): v for j, v in c.items()})
        return (name, a, c, m, d1, d2)

    def _pair(self, I, J):
        s = I[3]
        s1 = (s + 1) % 3
        assert s1 == J[3]
        a, c, lhs, out = dict(I[1]), dict(I[2]), {}, {}
        for k, v in J[1].items():
            _acc(a, k, -v)
        for k, v in J[2].items():
            _acc(c, k, v)
        V = self._index("(%s-%s)" % (I[0], J[0]), a, c, (s + 2) % 3)
        for k, v in I[1].items():
            _acc(lhs, (k, s1), v)
        for k, v in J[1].items():
            _acc(lhs, (k, s), v)
        for k, v in I[2].items():
            _acc(out, (k, s1), v)
        for k, v in J[2].items():
            _acc(out, (k, s), -v)
        sn = "S(%s,%s)" % (I[0], J[0])
        self._prod(sn, lhs, out)
        return ({sn: 1, V[4]: 1, I[5]: 1, J[5]: -1}, {sn: 1, V[5]: 1, I[4]: 1, J[4]: -1}, V)

    def weights(self, entries):
        w = {}
        for ij in entries:
            for p, c in self.y[ij].items():
                _acc(w.setdefault(p, {}), ij, c)
        return {p: d for p, d in w.items() if d}


def _slp(targets):
    ts = [dict(t) for t in targets]
    ops = []
    while any(len(t) > 1 for t in ts):
        cnt = {}
        for t in ts:
            ks = sorted(t, key=repr)
            for x in range(len(ks)):
                for y in range(x + 1, len(ks)):
                    key = (ks[x], ks[y], t[ks[x]] * t[ks[y]])
                    cnt[key] = cnt.get(key, 0) + 1
        a, b, sg = max(cnt, key=lambda k: cnt[k])
        new = ("t", len(ops))
        ops.append((new, a, b, sg))
        for t in ts:
            if a in t and b in t and t[a] * t[b] == sg:
                t[new] = t.pop(a)
                del t[b]
    return ops, [next(iter(t.items()))[::-1] for t in ts]


def _signed_sum(p, q, sign=1):
    (sp, vp), (sq, vq) = p, q
    if sp == sq:
        return sp, lax.add(vp, vq)
    return sign, (lax.sub(vp, vq) if sp == sign else lax.sub(vq, vp))


def _slp_signs(slp, signs):
    ops, results = slp
    signs = dict(signs)
    for new, a, b, sg in ops:
        signs[new] = signs[a] if signs[a] == sg * signs[b] else 1
    return [s * signs[v] for s, v in results]


class _Sum:
    def __init__(self, sign, value):
        self.terms = [(sign, value)]

    def get(self, sign):
        return _signed_sum(*self.terms, sign) if len(self.terms) == 2 else self.terms[0]

    def add(self, sign, value):
        self.terms = [self.get(-sign), (sign, value)]


class _Transposed:
    def __init__(self, slp, dry=False):
        ops, self.results = slp
        self.dry, self.adj = dry, {}
        self.split = {new: (a, b, sg) for new, a, b, sg in ops}
        self.pending = {}
        for v in [v for _, v in self.results] + [v for _, a, b, _ in ops for v in (a, b)]:
            self.pending[v] = self.pending.get(v, 0) + 1

    def put(self, v, sign, val):
        if v not in self.adj:
            self.adj[v] = _Sum(sign, val)
        elif not self.dry:
            self.adj[v].add(sign, val)
        self.pending[v] -= 1
        if self.pending[v] == 0 and v in self.split:
            a, b, sg = self.split[v]
            s, val = self.adj.pop(v).get(1)
            self.put(a, s, val)
            self.put(b, s * sg, val)

    def feed(self, t, val, sign=1):
        s, v = self.results[t]
        self.put(v, s * sign, val)


_FORM_SIGN = (1, -1, 1)
_SCHEME = _HK((0, 0, 1, 1, 2), (((0, 1), 2), ((2, 3), 0)))
_NAMES = list(_SCHEME.names)
_R = len(_NAMES)
_LHS_SLP = _slp([_SCHEME.lhs[p] for p in _NAMES])
_LHS_SIGN = dict(zip(_NAMES, _slp_signs(_LHS_SLP, {(i, s): _FORM_SIGN[s] for i in range(5) for s in range(3)})))
_W_FULL = _SCHEME.weights([(i, j) for i in range(5) for j in range(5)])
_W_K4 = _SCHEME.weights([(i, j) for i in range(4) for j in range(4)])
_NAMES_K4 = [p for p in _NAMES if p in _W_K4]
_D4 = _SCHEME.idx[4][4], _SCHEME.idx[4][5]
_LHS_SLP_K4 = _slp([_SCHEME.lhs[p] for p in _NAMES_K4])
assert [_LHS_SIGN[p] for p in _NAMES_K4] == _slp_signs(
    _LHS_SLP_K4, {(i, s): _FORM_SIGN[s] for i in range(4) for s in range(3)})


def _n2_products():
    res = []
    for i, j in ((0, 2), (1, 3)):
        w = _SCHEME.weights([(i, i), (i, j), (j, i), (j, j)])
        col = {i: 0, j: 1}
        for p in _NAMES:
            if p in w:
                res.append((p, {(col[c], s): v for (c, s), v in _SCHEME.out[p].items()},
                            {(a, col[b]): v for (a, b), v in w[p].items()}))
    for c in range(2):
        res.append((_D4[0], {(c, 1): 1}, {(4, c): 1}))
        res.append((_D4[1], {(c, 0): 1}, {(4, c): -1}))
    forms = []
    for _, out, _ in res:
        if out not in forms:
            forms.append(out)
    merged = [(f, [(p, w) for p, out, w in res if out == f]) for f in forms]
    one, two, three = ([m for m in merged if len(m[1]) == n] for n in (1, 2, 3))
    return two[:1] + [three[0], one[0], three[1], one[1]] + two[1:]


def _groups():
    vec = {}
    for p in _NAMES:
        vec[p] = {}
        for (j, form), c in _SCHEME.out[p].items():
            for half, v in (((1, 1),), ((0, 1),), ((0, -1), (1, -1)))[form]:
                _acc(vec[p], (j, half), c * v)

    def relation(s, a, b):
        for ca in (1, -1):
            for cb in (1, -1):
                d = dict(vec[s])
                for p, c in ((a, ca), (b, cb)):
                    for k, v in vec[p].items():
                        _acc(d, k, -c * v)
                if not d:
                    return ca, cb

    def match(sums, free):
        if not sums:
            return []
        s = sums[0]
        pair = _NAMES[_NAMES.index(s) - 2:_NAMES.index(s)]
        for a in free:
            for b, c in (pair, pair[::-1]):
                if relation(s, a, b):
                    rest = match(sums[1:], [p for p in free if p != a])
                    if rest is not None:
                        return [(s, a, b, c) + relation(s, a, b)] + rest
    return match([p for p in _NAMES if p[0] == "S"], [p for p in _NAMES if p[0].isdigit()])


_N2 = _n2_products()
_GROUPS = _groups()
_KEPT = [p for g in _GROUPS for p in g[1:4]]


class _Weights:
    def __init__(self, w, lhs_sign, order, move_sign=True, in_place=True):
        w = {p: {k: lhs_sign[p] * c for k, c in d.items()} for p, d in w.items()}
        self.sign = {p: next(iter(d.values())) if len(d) == 1 and move_sign else 1 for p, d in w.items()}
        self.single = {p: next(iter(d)) for p, d in w.items() if len(d) == 1 and in_place}
        self.summed = [p for p in lhs_sign if p in w and p not in self.single]
        self.terms = [len(w[p]) for p in self.summed]
        self.slp = _slp([{k: c * self.sign[p] for k, c in w[p].items()} for p in self.summed])
        self.used = sorted({k for p in self.summed for k in w[p]})
        self.order = order
        assert sorted(order) == list(range(len(self.summed)))


_V_FULL = _Weights(_W_FULL, _LHS_SIGN, (11, 25, 24, 12, 14, 16, 5, 4, 0, 13, 17, 1, 20, 22, 8, 9, 18, 23, 2, 3, 15,
                                        19, 7, 6, 10, 21))
_V_K4 = _Weights(_W_K4, _LHS_SIGN, (8, 11, 1, 18, 15, 10, 0, 19, 9, 4, 14, 5, 12, 13, 16, 6, 7, 2, 17, 3))
_V_ALL = _Weights(_W_FULL, _LHS_SIGN, (11, 36, 10, 39, 12, 16, 0, 14, 5, 1, 34, 13, 29, 17, 4, 24, 30, 18, 9, 37, 8,
                                       23, 33, 28, 3, 35, 38, 2, 25, 15, 21, 7, 20, 27, 19, 22, 31, 26, 6, 32),
                  in_place=False)
_V_N2 = _Weights({(n, p): w for n, (_, parts) in enumerate(_N2) for p, w in parts},
                 {(n, p): _LHS_SIGN[p] for n, (_, parts) in enumerate(_N2) for p, _ in parts},
                 (8, 6, 14, 10, 16, 9, 2, 0, 4, 5, 1, 13, 3, 12, 15, 17, 11, 7), move_sign=False, in_place=False)
assert all(_V_K4.sign[p] == _V_FULL.sign[p] for p in _NAMES_K4) and all(_V_FULL.sign[p] == 1 for p in _D4)


class _Outputs:
    def __init__(self, outs, signs):
        self.slp, self.sign = _slp(outs), signs
        self.ncol = 1 + max(j for out in outs for j, _ in out)
        self.order, rest = [], list(range(len(outs)))
        while rest:
            self.order.append(min(rest, key=lambda t: self._live(self.order + [t])))
            rest.remove(self.order[-1])

    def _live(self, seq):
        tr = _Transposed(self.slp, dry=True)
        for t in seq:
            tr.feed(t, None)
        todo = [[tr.pending.get((j, s), 0) for s in range(3)] for j in range(5)]
        return len(tr.adj) - sum(not any(n) for n in todo), sum(n ** 0.5 for col in todo for n in col)


_O_ALL = _Outputs([_SCHEME.out[p] for p in _NAMES], [_V_FULL.sign[p] for p in _NAMES])
_O_KEPT = _Outputs([_SCHEME.out[p] for p in _KEPT], [_V_FULL.sign[p] for p in _KEPT])
_O_N2 = _Outputs([f for f, _ in _N2], [1] * len(_N2))


def _lhs_sums(slp, a1, a2):
    env = {}
    for i, (x, y) in enumerate(zip(a1, a2)):
        env[i, 0], env[i, 1], env[i, 2] = (1, x), (-1, y), (1, lax.sub(y, x))
    for new, a, b, sg in slp[0]:
        env[new] = _signed_sum(env[a], (sg * env[b][0], env[b][1]))
    return [env[v][1] for _, v in slp[1]]


def _columns(acc, ncol):
    c1, c2 = [], []
    for j in range(ncol):
        s2, v2 = acc[j, 2].get(1)
        for form, dst in ((1, c1), (0, c2)):
            s, v = _signed_sum(acc[j, form].get(s2), (-s2, v2))
            dst.append(v if s > 0 else lax.neg(v))
    return c1, c2


def _lo(v):
    return lax.slice_in_dim(v, 0, v.shape[0] // 2, axis=0)


def _hi(v):
    return lax.slice_in_dim(v, v.shape[0] // 2, v.shape[0], axis=0)


def _cat(*vs):
    return lax.concatenate(vs, 0)


def _pack(v):
    return lax.bitcast_convert_type(pltpu.pack_elementwise([_lo(v), _hi(v)], packed_dtype=BF16), U32)


def _unpack(w):
    return _cat(*[pltpu.unpack_elementwise(w, index=i, packed_dtype=BF16, unpacked_dtype=F32) for i in range(2)])


def _cmul(ar, ai, br, bi):
    return lax.sub(lax.mul(ar, br), lax.mul(ai, bi)), lax.add(lax.mul(ar, bi), lax.mul(ai, br))


def _cmad(ar, ai, br, bi, cr, ci):
    tr, ti = _cmul(ar, ai, br, bi)
    return lax.add(tr, cr), lax.add(ti, ci)


def _gelu2(g):
    k = 0.7978845608028654
    return lax.add(g, lax.mul(g, lax.tanh(lax.mul(g, k + (k * 0.044715) * lax.mul(g, g)))))


def _silu_half(d):
    z = 0.25 * d
    return lax.add(z, lax.mul(z, lax.tanh(z)))


_LS = (17, 17, 17, 13)
_NB, _LM = len(_LS), max(_LS)
_CHUNK = 20
_FIRST = (4, 3, 1)

_nt = lambda i, j: (LANE * j, LANE * i)
_nn = lambda i, j: (LANE * i, LANE * j)
_TABLES = dict(b0=(_V_FULL, "bre", 0, _nt), b1=(_V_FULL, "bim", 0, _nt),
               c0=(_V_ALL, "cre", 0, _nt), c1=(_V_ALL, "cim", 0, _nt),
               g0=(_V_FULL, "wg", 0, _nt), u0=(_V_FULL, "wu", 0, _nt),
               g1=(_V_FULL, "wg", 5 * LANE, _nt), u1=(_V_FULL, "wu", 5 * LANE, _nt),
               r0=(_V_FULL, "wr", 0, _nt), r1=(_V_N2, "wr", 5 * LANE, _nt),
               d0=(_V_FULL, "wd", 0, _nn), d1=(_V_FULL, "wd", 5 * LANE, _nn), d2=(_V_K4, "wd", 10 * LANE, _nn))

_PER_POSITION = dict(stage=30, stats=38, ln=95, project=130, states=195, act=175, act_rest=120, finish=165,
                     skip=75, column=35)
_ONCE = dict(starts=300, out=1, coefs=500, r1=300, d2=500, c0=1500, c1=1500)
_PAUSE = dict(states=300, finish=300, act_rest=300, project=300, ln=200, bim=800, wr=1500, x1=1, wgu=1, rest=1)
_WINDOW = dict(act=13, column=13)


def _products(key):
    if key[0] == "b":
        stage = lambda p: 2 if len(_W_FULL[p]) > 2 else p not in _V_FULL.single or _V_FULL.single[p][0] not in _FIRST
        return _NAMES if key[2] == 3 else sorted((p for p in _NAMES if stage(p) == key[2]),
                                                 key=lambda p: len(_W_FULL[p]))
    if key[0] == "d":
        return [p for p in _products(("D",)) if min(j for j, _ in _SCHEME.out[p]) == key[2]]
    return sorted(_NAMES, key=lambda p: p in _W_K4) if key[0] == "D" else _NAMES


def _n_tiles(key):
    if key[0] in "Dd":
        return sum(2 + (p in _W_K4) + 4 * (p in _D4) for p in _products(key))
    if key[0] == "r":
        return _R if key[2] else len(_V_N2.summed) + 2
    return dict(R=_R + len(_V_N2.summed), b=len(_products(key))).get(key[0], 2 * _R)


def _plan():
    R, B, C, D = (lambda b, k=k: (k, b) for k in "RBCD")
    G = lambda b, g: ("G", b, g)
    during = lambda first, last, *tasks: [(t, first, last) for t in tasks]
    prep = lambda names: [("prep", n) for n in names.split()]
    norm = lambda b: [("stage", b), ("stats", b, 0), ("stats", b, 1), ("ln", b)]
    b0, b1, b2, b3 = (("b", 0, n) for n in range(4))
    r0, r1 = ("r", 0, 0), ("r", 0, 1)

    steps = []
    for n in range(4):
        steps += [("wait", "x0", n), ("run", "moments", n)]
    steps += [("run", "ln", 0), ("wait", "bre", 0), b0, ("wait", "bre", 1), ("run", "prep", "b0", 0), b1,
              ("run", "prep", "b0", 1), b2, b3, r0, r1, B(1), G(0, 0), G(0, 1), R(1), D(0)]
    tasks = (during(b2, b2, ("wait", "bim"), *prep("b1")) + during(b3, b3, ("coefs",), ("wait", "wr"), *prep("r1"))
             + during(r0, r0, *prep("r0")) + during(r0, r1, ("wait", "x1"), *norm(1))
             + during(r1, G(0, 0), ("project", 0)) + during(B(1), B(1), ("wait", "wgu"), *prep("g0 u0"))
             + during(B(1), G(0, 0), *prep("g1 u1")) + during(B(1), D(0), ("starts", 0))
             + during(B(1), G(0, 1), ("act_rest", 0))
             + during(G(0, 1), R(1), ("act", 0, 0), ("wait", "rest"), *prep("d0 d1 d2"))
             + during(R(1), R(1), ("act", 0, 1)) + during(R(1), D(0), *prep("c0 c1"), ("states", 0)))
    for b in range(1, _NB):
        more = b + 1 < _NB
        extra = B(b + 1) if more else C(b)
        down = [R(b + 1), D(b)] if more else [("d", b, c) for c in range(5)]
        steps += [C(b - 1), G(b, 0), G(b, 1), extra] + down
        second = during(R(b), G(b, 1), *norm(2)) if b == 1 else []
        tasks += second[:2] + during(R(b), C(b - 1), ("project", b)) + second[2:]
        tasks += during(C(b - 1), G(b, 1), ("act_rest", b), ("starts", b))
        if not more:
            tasks += during(C(b - 1), G(b, 1), ("states", b))
        tasks += during(G(b, 0), down[0] if more else extra, ("finish", b - 1), ("out", b - 1))
        tasks += during(G(b, 1), extra, ("act", b, 0)) + during(extra, down[0] if more else extra, ("act", b, 1))
        if b + 2 < _NB:
            tasks += during(down[0], G(b + 1, 1), *norm(b + 2))
        if more:
            tasks += during(C(b - 1), D(b), ("states", b))
        else:
            tasks += during(down[0], down[0], ("skip", b))
            tasks += [(("column", b, c), down[c + 1], down[-1]) for c in range(4)]
            steps += [("run", "column", b, 4)]
    return steps, [u for t in tasks for u in [(("pause", t[0][0]),) + t[1:]] * (t[0][0] in _PAUSE) + [t]]


def _spread(cycles, work, lo, hi):
    def run(load, p0, p1, u):
        ends, idle = [], []
        for p in range(p0, p1):
            left = load * cycles[p]
            while u < hi[p] and left > 0:
                need = (int(u) + 1 - u) * work[int(u)][p]
                u, left = (int(u) + 1, left - need) if need <= left else (u + left / work[int(u)][p], 0)
            ends.append(u)
            idle.append(left > 0)
        return ends, idle

    def solve(p0, p1, u, last):
        if p0 == p1:
            return []
        need = lo[p0:p1 - 1] + [max(lo[p1 - 1], last)]
        a, b = 0.0, 8.0
        for _ in range(40):
            m = (a + b) / 2
            a, b = (a, m) if all(e >= n for e, n in zip(run(m, p0, p1, u)[0], need)) else (m, b)
        j = next((p0 + k for k, (e, n) in enumerate(zip(run(a, p0, p1, u)[0], need)) if e < n), p1 - 1)
        ends, idle = run(b, p0, j + 1, u)
        i = max([p0 + k + 1 for k in range(j - p0) if idle[k]], default=p0)
        ends[-1] = max(need[j - p0], u)
        return solve(p0, i, u, hi[i - 1]) + ends[i - p0:] + solve(j + 1, p1, ends[-1], last)

    return solve(0, len(cycles), 0.0, 0)


class _Schedule:
    def __init__(self):
        self.steps, self.tasks = _plan()
        self.phases = phases = [s for s in self.steps if s[0] not in ("wait", "run")]
        self.work = [[self._cycles(t, p) for p in phases] for t, _, _ in self.tasks]
        self.slots = [_LS[p[1]] * max(_n_tiles(p) / 4 - 1, 1.0) for p in phases]
        hi = [next((n for n, t in enumerate(self.tasks) if phases.index(t[1]) > i), len(self.tasks))
              for i in range(len(phases))]
        self.lo = [max([n + 1 for n, t in enumerate(self.tasks) if phases.index(t[2]) <= i], default=0)
                   for i in range(len(phases))]
        self.target = [0.0] + _spread([16 * n for n in self.slots], self.work, self.lo, hi)
        self.sets, busy = {}, []
        for i, p in enumerate(phases):
            k = self.products(p)
            if k not in self.sets:
                reader = (dict(B="project", R="act_rest", G="act", C="finish")[k[0]],) + k[1:]
                end = max((phases.index(t[2]) for t in self.tasks if t[0] == reader), default=len(phases))
                self.sets[k] = next((n for n, e in enumerate(busy) if e < i), len(busy))
                busy[self.sets[k]:self.sets[k] + 1] = [end]
        self.n_sets = len(busy)

    @staticmethod
    def products(key):
        return key if key[0] == "G" else (dict(b="B", r="R", D="C", d="C").get(key[0], key[0]), key[1])

    @staticmethod
    def _cycles(t, phase):
        if t[0] in ("pause", "wait"):
            return _PAUSE[t[1]]
        if t[0] in _PER_POSITION:
            return _LS[t[1]] * (170 if t[0] == "states" and phase[0] in "CDd" else _PER_POSITION[t[0]])
        return _ONCE.get(t[t[0] == "prep"], 680)

    def progress(self, i, x):
        u0, u1 = self.target[i], self.target[i + 1]
        knots = [u0] + list(range(int(u0) + 1, int(np.ceil(u1)))) + [u1]
        t = np.cumsum([0.0] + [(b - a) * self.work[int(a)][i] for a, b in zip(knots, knots[1:]) if b > a])
        return float(np.interp(x * t[-1], t, knots[:len(t)])) if x < 1 else u1


class _Buf:
    def __init__(self, ref, z):
        flat = len(ref.shape) == 2
        n = 32 // ref.dtype.itemsize if flat else 1
        end = ref.shape[0] - n
        self.ref, self.ready, self.copied = ref, False, False
        self.view = ref.at[pl.ds(pl.multiple_of(n * z, n) if flat else z, end)]
        self.spare, self.zeros = ((pl.ds(end - k * n, n), pl.ds(0, LANE)) if flat else (end - k, pl.ds(0, 8))
                                  for k in (1, 2))

    def fence(self, v):
        if self.ref.dtype == BF16:
            v = pltpu.bitcast(v, BF16)
        elif self.ref.dtype != v.dtype:
            v = lax.bitcast_convert_type(v, self.ref.dtype)
        self.view[self.spare] = v

    def done(self):
        if not self.ready:
            self.ref[self.zeros] = jnp.zeros((32 // self.ref.dtype.itemsize, LANE), self.ref.dtype)
            self.ready = True
        if self.copied:
            self.fence(jnp.zeros((8, LANE), F32))
        v = (self.ref if self.copied else self.view)[self.zeros]
        self.copied = False
        return pltpu.bitcast(v, U32) if v.dtype == BF16 else lax.bitcast_convert_type(v, U32)


def _scratch(plan, S, D, F):
    NL = D // LANE
    slots = lambda n, rows, dtype: pltpu.VMEM((n + 3, rows, LANE), dtype)
    rows = lambda n: [pltpu.VMEM((32 * L * n + 24, LANE), F32) for L in _LS]
    buf = dict(
        raw=dict({k: [pltpu.VMEM((n + 48, LANE), BF16)] * NL for k, n in dict(
            bre=D, bim=D, cre=D, cim=D, wg=2 * D, wu=2 * D, wr=2 * (F - 2 * D), wd=F + -F % LANE).items()},
            x=pltpu.VMEM((S + 48, D), BF16)),
        v={k: slots(len(t[0].summed), LANE // 2, U32) for k, t in _TABLES.items()},
        xf=[[v] * NL for v in rows(1)], s0=rows(1), s1=rows(1), of=rows(NL)[:-1], oc=rows(1)[-1:] * NL,
        xl=[slots(_R, 8 * _LM, U32)] * 2, hl=[slots(2 * _R, 8 * _LM, U32)] * 2,
        dl=slots(2 * _R + len(_NAMES_K4) + 8, 8 * _LM, U32),
        u=[[slots(4 * NL, 8, F32)] * _LM] * 2, e=[slots(6, 16, F32)] * NL,
        coef=slots(4 + 2 * _LM + 8 * len(set(_LS)), 8, F32),
    )
    for n in range(plan.n_sets):
        most = [max(_R if k[0] == "C" or k == ("B", 0) and half else len(_KEPT) for k, m in plan.sets.items() if m == n)
                for half in range(2)]
        buf["p%d" % n] = [[[[slots(_CHUNK - 1, 8, F32)] * -(-m // _CHUNK) for m in most]] * 2] * _LM
    return dict(buf=buf, vec=[pltpu.VMEM((D,), BF16)] * 4,
                sem=[pltpu.SemaphoreType.DMA((11,)), pltpu.SemaphoreType.DMA, pltpu.SemaphoreType.REGULAR])


def _kernel(plan, x_hbm, lre_hbm, lim_hbm, bre_hbm, bim_hbm, cre_hbm, cim_hbm, ldt_hbm, dsk_hbm,
            wg_hbm, wu_hbm, wd_hbm, o_hbm, sc):
    in_sem, out_sem, idle_sem = sc["sem"]
    S, D = x_hbm.shape
    F = wd_hbm.shape[0]
    NL = D // LANE
    T0 = [32 * sum(_LS[:b]) for b in range(_NB)]

    z = jnp.clip(pl.semaphore_read(idle_sem), 0, 1)
    bufs = jax.tree.map(lambda ref: _Buf(ref, z), sc["buf"])
    raw = bufs["raw"]
    xl, hl, dl = bufs["xl"], bufs["hl"], bufs["dl"]
    xf, sb, of = bufs["xf"], (bufs["s0"], bufs["s1"]), bufs["of"]
    ub, eb, cf = bufs["u"], bufs["e"], bufs["coef"]

    def products(key):
        return bufs["p%d" % plan.sets[plan.products(key)]]

    copies = {}

    def copy(name, src, dst):
        copies.setdefault(name, [])
        copies[name].append(pltpu.make_async_copy(src, dst, in_sem.at[list(copies).index(name)]))

    def copy_x(name, r0, n):
        copy(name, x_hbm.at[pl.ds(r0, n)], raw["x"].ref.at[pl.ds(r0, n)])

    def copy_strips(name, src, r0, n, dst, d0=0, strips=range(NL)):
        for c in strips:
            copy(name, src.at[pl.ds(r0, n), pl.ds(LANE * c, LANE)], raw[dst][c].ref.at[pl.ds(d0, n)])

    pieces = [32 * (_LS[0] - _LS[0] * (4 - n) // 4) for n in range(5)]
    for n in range(4):
        copy_x(("x0", n), pieces[n], pieces[n + 1] - pieces[n])
    copy_strips(("bre", 0), bre_hbm, 0, D, "bre", 0, _FIRST)
    copy_strips(("bre", 1), bre_hbm, 0, D, "bre", 0, [c for c in range(NL) if c not in _FIRST])
    copy_strips(("bim",), bim_hbm, 0, D, "bim")
    for src, dst in zip((lre_hbm, lim_hbm, ldt_hbm, dsk_hbm), sc["vec"]):
        copy(("bim",), src, dst)
    n = F - 2 * D
    copy_strips(("wr",), wg_hbm, 2 * D, n, "wr")
    copy_strips(("wr",), wu_hbm, F - n % LANE, n % LANE, "wr", n)
    copy_strips(("wr",), wu_hbm, 2 * D, n - n % LANE, "wr", n + n % LANE)
    copy_x(("x1",), T0[1], 32 * _LS[1])
    copy_strips(("wgu",), wg_hbm, 0, 2 * D, "wg")
    copy_strips(("wgu",), wu_hbm, 0, 2 * D, "wu")
    copy_strips(("rest",), wd_hbm, 0, F, "wd")
    copy_strips(("rest",), cre_hbm, 0, D, "cre")
    copy_strips(("rest",), cim_hbm, 0, D, "cim")
    copy_x(("rest",), T0[2], S - T0[2])
    for strip in raw["wd"]:
        strip.ref[pl.ds(F, -F % LANE), :] = jnp.zeros((-F % LANE, LANE), BF16)
    out_copies = []

    def copy_out(b, c, src, n):
        T = 32 * _LS[b]
        src.copied = True
        out_copies.append(pltpu.make_async_copy(
            src.ref.at[pl.ds(n * T, T)], o_hbm.at[pl.ds(T0[b], T), pl.ds(LANE * c, LANE)], out_sem))
        out_copies[-1].start()


    high_powers = {L: 4 + 2 * _LM + 8 * n for n, L in enumerate(sorted(set(_LS)))}

    def t_coefs():
        yield 1
        yield None, 1
        lre, lim, ldt, dsk = (_cat(*[v[:, LANE * c:LANE * c + LANE] for c in range(NL)])
                              for v in (r[...].astype(F32).reshape(1, D) for r in sc["vec"]))
        dt = jnp.exp(ldt).astype(BF16).astype(F32)
        zr, zi = dt * lre, dt * lim
        mag = jnp.exp(zr)
        ar, ai = mag * jnp.cos(zi), mag * jnp.sin(zi)
        nr, ni = ar - 1.0, ai
        big = jnp.abs(lre) >= jnp.abs(lim)
        rat = jnp.where(big, lim / lre, lre / lim)
        den = jnp.where(big, lre + lim * rat, lre * rat + lim)
        qr = 2.0 * jnp.where(big, nr + ni * rat, nr * rat + ni) / den
        qi = 2.0 * jnp.where(big, ni - nr * rat, ni * rat - nr) / den
        powers = [(ar, ai)]
        for n in range(2, _LM + 1):
            powers.append(_cmul(*powers[n // 2 - 1], *powers[n - n // 2 - 1]))
        consts = [dsk, qr, qi, -qi] + [v for p in powers for v in p]
        for L in high_powers:
            p = powers[L - 1]
            for _ in range(4):
                p = _cmul(*p, *p)
                consts += p
        for n, v in enumerate(consts):
            cf.ref[n, pl.ds(0, NL), :] = v
        yield cf, -5

    def coef(n, c, reps=1):
        return jnp.broadcast_to(cf.ref[n, pl.ds(c, 1), :], (8 * reps, LANE))

    def power(n, c, reps=1):
        slot = 2 + 2 * n if n <= _LM else next(
            s + 2 * k for L, s in high_powers.items() for k in range(4) if n == L << k + 1)
        return coef(slot, c, reps), coef(slot + 1, c, reps)

    def tile_rows(src, row0, corner, i, j, r0=0, n=LANE):
        row, col = corner(i, j)
        return raw[src][col // LANE].ref[pl.ds(row0 + row + r0, n), :]

    def t_prep(name, long_sums=None):
        tab, src, row0, corner = _TABLES[name]
        dest = bufs["v"][name]
        ops, results = tab.slp
        parts = {new: (a, b, sg) for new, a, b, sg in ops}
        inner = [v for _, a, b, _ in ops for v in (a, b)]
        want = {v: s for s, v in results if v not in inner}
        seq = []

        def need(v):
            if v not in seq:
                for u in parts.get(v, ())[:2]:
                    need(u)
                seq.append(v)
        for n in tab.order:
            if long_sums in (None, tab.terms[n] > 2):
                need(results[n][1])
                seq.append(n)
        tiles = [v for v in seq if v in tab.used]
        yield 8 * len(tiles)
        for r0 in range(0, LANE, 16):
            env = {}
            for v in seq:
                if v in parts:
                    a, b, sg = parts[v]
                    env[v] = _signed_sum(env[a], (sg * env[b][0], env[b][1]), want.get(v, 1))
                elif v in tiles:
                    if tiles.index(v) % 9 == 0:
                        for m in ("cre", "cim") if name[0] == "c" else (src,):
                            yield raw[m][corner(*v)[1] // LANE], 0
                        yield None, len(tiles[tiles.index(v):][:9])
                    load = lambda src: _unpack(pltpu.bitcast(tile_rows(src, row0, corner, *v, r0, 16), U32))
                    if name[0] == "c":
                        re, im = (1, 2) if name == "c0" else (3, 1)
                        env[v] = 1, lax.sub(lax.mul(load("cre"), coef(re, v[0], 2)),
                                            lax.mul(load("cim"), coef(im, v[0], 2)))
                    else:
                        env[v] = 1, load(src)
                else:
                    s, val = env[results[v][1]]
                    dest.ref[v, pl.ds(r0 // 2, 8), :] = _pack(val if s * results[v][0] > 0 else lax.neg(val))
            yield dest, -2

    def weight(name, p):
        tab = _TABLES[name][0]
        if p in tab.single:
            return tile_rows(*_TABLES[name][1:], *tab.single[p])
        return pltpu.bitcast(bufs["v"][name].ref[tab.summed.index(p)], BF16)

    def gather_weight(outs):
        return 2.6 * len(outs.order) + 5 * -(-len(outs.order) // _CHUNK)

    def gather(key, q, v, half, outs):
        chunks = products(key)[q][v][half]
        tr = _Transposed(outs.slp)
        for m, r in enumerate(outs.order):
            if m % _CHUNK == 0:
                yield chunks[m // _CHUNK], 5 + 2.6 * min(_CHUNK, len(outs.order) - m)
            tr.feed(r, chunks[m // _CHUNK].ref[m % _CHUNK], outs.sign[r])
        return _columns(tr.adj, outs.ncol)

    def scatter(slp, names, a1, a2, buf, q, first, weight, bursts=None):
        vals = _lhs_sums(slp, a1, a2)
        last = [max(2, *(i for i, _ in _SCHEME.lhs[p])) for p in names]
        order = sorted(range(len(vals)), key=lambda n: last[n])
        if bursts:
            groups = [order[len(order) * i // bursts:len(order) * (i + 1) // bursts] for i in range(bursts)]
        else:
            groups = [[n for n in order if last[n] == i] for i in (2, 3, 4)]
        for group in groups:
            if bursts and bursts > 1:
                yield buf, 0
            for n in group:
                buf.ref[first + n, pl.ds(8 * q, 8), :] = _pack(vals[n])
            if not bursts or group is groups[-1]:
                yield buf, -1
            yield None, weight / len(groups)

    def in_rows(b, q, h):
        return [pl.ds((h + 2 * t) * _LS[b] + q, 8, stride=4 * _LS[b]) for t in range(2)]

    def out_rows(b, q, v, h, c=0):
        return pl.ds((32 * c + 8 * (2 * h + v)) * _LS[b] + q, 8, stride=_LS[b])

    def load_in(buf, b, q, h):
        return _cat(*[buf.ref[s, :] for s in in_rows(b, q, h)])

    def load_x(r0, c):
        return raw["x"].ref[pl.ds(r0, 32), pl.ds(LANE * c, LANE)].astype(F32)

    def row_mean(tiles):
        tot = jnp.sum(functools.reduce(lax.add, tiles), axis=-1, keepdims=True) * (1.0 / D)
        return jnp.broadcast_to(tot, tiles[0].shape)

    def t_stage(b):
        yield _LS[b]
        for r0 in range(0, 32 * _LS[b], 32):
            yield raw["x"], 1
            for c in range(NL):
                xf[b][c].ref[pl.ds(r0, 32), :] = load_x(T0[b] + r0, c)
            for dest in xf[b]:
                yield dest, -1

    def t_stats(b, n):
        yield 140 * _LS[b]
        for q in range(_LS[b]):
            for h in range(2):
                if n:
                    yield sb[0][b], 1
                xv = []
                for c in range(NL):
                    yield xf[b][c], 0
                    xv.append(load_in(xf[b][c], b, q, h))
                yield None, 70 - n
                if n:
                    mean = load_in(sb[0][b], b, q, h)
                    xv = [lax.mul(d, d) for d in (lax.sub(v, mean) for v in xv)]
                v = lax.rsqrt(row_mean(xv) + 1e-5) if n else row_mean(xv)
                for s, part in zip(in_rows(b, q, h), (_lo(v), _hi(v))):
                    sb[n][b].ref[s, :] = part
            yield sb[n][b], -2

    def t_moments(n):
        yield 0
        for r0 in range(pieces[n], pieces[n + 1], 32):
            xv = [load_x(r0, c) for c in range(NL)]
            mean = row_mean(xv)
            var = row_mean([lax.mul(d, d) for d in (lax.sub(v, mean) for v in xv)])
            for buf, v in zip(xf[0] + [sb[0][0], sb[1][0]], xv + [mean, lax.rsqrt(var + 1e-5)]):
                buf.ref[pl.ds(r0, 32), :] = v
                yield buf, -1

    def t_ln(b):
        yield 575 * _LS[b]
        for q in range(_LS[b]):
            yield sb[0][b], 2
            yield sb[1][b], 3
            stats = [[load_in(sb[n][b], b, q, h) for n in range(2)] for h in range(2)]
            halves = [[], []]
            for c in range(NL):
                yield None, (25, 25, 85, 115, 140)[c]
                for h, (mean, rstd) in enumerate(stats):
                    halves[h].append(lax.mul(lax.sub(load_in(xf[b][c], b, q, h), mean), rstd))
            yield from scatter(_LHS_SLP, _NAMES, *halves, xl[b % 2], q, 0, 180)

    def state(part, h, c):
        return (2 * part + h) * NL + c

    def load_state(q, n):
        return _cat(*[ub[v][q].ref[n] for v in range(2)])

    def t_project(b):
        real = _O_KEPT if b else _O_ALL
        yield 2 * (gather_weight(real) + gather_weight(_O_KEPT) + 120) * _LS[b]
        for q in range(_LS[b]):
            for v in range(2):
                ur = yield from gather(("B", b), q, v, 1, real)
                ui = yield from gather(("B", b), q, v, 0, _O_KEPT)
                yield None, 100
                for c in range(NL):
                    a = power(1, c) if q else None
                    for h in range(2):
                        e = ur[h][c], ui[h][c]
                        if q:
                            e = _cmad(*a, *(ub[v][q - 1].ref[state(t, h, c)] for t in range(2)), *e)
                        for t in range(2):
                            ub[v][q].ref[state(t, h, c)] = e[t]
                yield ub[v][q], -2
                yield None, 20

    def t_starts(b):
        L = _LS[b]
        row = lax.broadcasted_iota(jnp.int32, (16, LANE), 0)
        yield 149 * NL
        for c in range(NL):
            yield ub[0][L - 1], 4
            yield ub[1][L - 1], 5
            yield eb[c], 0
            even, odd = ([load_state(L - 1, state(t, h, c)) for t in range(2)] for h in range(2))
            f = _cmad(*power(L, c, 2), *even, *odd)
            carry = [eb[c].ref[4 + t] for t in range(2)] if b else [0.0, 0.0]
            if b:
                f = [lax.add(v, jnp.where(row == 0, w, 0.0)) for v, w in zip(f, _cmul(*power(2 * L, c, 2), *carry))]
            for n in (1, 2, 4, 8):
                f = [jnp.where(row >= n, w, v)
                     for v, w in zip(f, _cmad(*power(2 * n * L, c, 2), *[pltpu.roll(v, n, 0) for v in f], *f))]
            first = [jnp.where(row == 0, w, pltpu.roll(v, 1, 0)) for v, w in zip(f, carry)]
            for h, init in enumerate((first, _cmad(*power(L, c, 2), *first, *even))):
                for t in range(2):
                    eb[c].ref[2 * t + h] = init[t]
            for t in range(2):
                eb[c].ref[4 + t] = jnp.broadcast_to(f[t][15:16], (16, LANE))
            yield None, 140
            yield eb[c], -4

    def t_states(b):
        yield 1480 * _LS[b]
        for q in range(_LS[b]):
            for part in range(2):
                tiles = []
                for c in range(NL):
                    yield eb[c], 1
                    for v in range(2):
                        yield ub[v][q], 0
                    yield None, (39, 39, 94, 119, 144)[c]
                    pr, pi = power(q + 1, c, 2)
                    hs = []
                    for h in range(2):
                        t = lax.mul(pr, eb[c].ref[2 * part + h]), lax.mul(pi, eb[c].ref[2 * (1 - part) + h])
                        hs.append(lax.add(load_state(q, state(part, h, c)), lax.add(*t) if part else lax.sub(*t)))
                    tiles.append((_cat(*map(_lo, hs)), _cat(*map(_hi, hs))))
                yield from scatter(_LHS_SLP, _NAMES, *zip(*tiles), hl[b % 2], q, part * _R, 300, 2)

    K4 = 2 * _R
    K4D = K4 + len(_NAMES_K4)

    def t_act(b, g):
        yield (4 * gather_weight(_O_KEPT) + 250) * _LS[b]
        for q in range(_LS[b]):
            hidden = [[], []]
            for v in range(2):
                gate = yield from gather(("G", b, g), q, v, 0, _O_KEPT)
                for c in range(NL):
                    yield None, 5
                    for h in range(2):
                        gate[h][c] = _gelu2(gate[h][c])
                up = yield from gather(("G", b, g), q, v, 1, _O_KEPT)
                for c in range(NL):
                    hidden[v].append(_cat(*[lax.mul(gate[h][c], up[h][c]) for h in range(2)]))
            yield from scatter(_LHS_SLP, _NAMES, *hidden, dl, q, g * _R, 200, 5)

    def t_act_rest(b):
        lane = lax.broadcasted_iota(jnp.int32, (8, LANE), 1)
        yield (2 * gather_weight(_O_KEPT) + 2 * gather_weight(_O_N2) + 140) * _LS[b]
        for q in range(_LS[b]):
            hidden = [[], []]
            for v in range(2):
                ta = yield from gather(("R", b), q, v, 0, _O_KEPT)
                for c in range(4):
                    yield None, 5
                    for h in range(2):
                        a = _gelu2(ta[h][c])
                        if c == 3:
                            a = jnp.where(lane < LANE // 2, lax.mul(a, pltpu.roll(ta[h][c], LANE // 2, 1)), 0.0)
                        ta[h][c] = a
                tb = yield from gather(("R", b), q, v, 1, _O_N2)
                for c in range(4):
                    hidden[v].append(_cat(*[lax.mul(ta[h][c], (ta[h] + tb[h])[4 + c]) if c < 3 else ta[h][c]
                                            for h in range(2)]))
            for h in range(2):
                for i in range(4):
                    dl.ref[K4D + 4 * h + i, pl.ds(8 * q, 8), :] = _pack(hidden[h][i])
            yield from scatter(_LHS_SLP_K4, _NAMES_K4, *hidden, dl, q, K4, 100, 1)

    def ssm_output(b, q, v, emit):
        y = yield from gather(("C", b), q, v, 0, _O_ALL)
        yield sb[0][b], 2
        yield sb[1][b], 3
        stats = [[sb[n][b].ref[out_rows(b, q, v, h), :] for n in range(2)] for h in range(2)]
        for c in range(NL):
            yield xf[b][c], 27
            for h, (mean, rstd) in enumerate(stats):
                x = xf[b][c].ref[out_rows(b, q, v, h), :]
                emit(h, c, x, lax.add(y[h][c], lax.mul(lax.mul(lax.sub(x, mean), rstd), coef(0, c))))

    def t_finish(b):
        yield 2 * (2 * gather_weight(_O_ALL) + 195) * _LS[b]
        for q in range(_LS[b]):
            for v in range(2):
                g = yield from gather(("C", b), q, v, 1, _O_ALL)
                for c in range(NL):
                    yield None, 11
                    for h in range(2):
                        g[h][c] = _silu_half(g[h][c])

                def emit(h, c, x, s):
                    of[b].ref[out_rows(b, q, v, h, c), :] = lax.add(x, lax.mul(s, g[h][c]))
                yield from ssm_output(b, q, v, emit)
                yield of[b], -1

    def t_out(b):
        yield 1
        yield None, 1
        for c in range(NL):
            copy_out(b, c, of[b], c)
        yield of[b], -3

    def t_skip(b):
        yield 2 * (gather_weight(_O_ALL) + 140) * _LS[b]
        for q in range(_LS[b]):
            for v in range(2):
                def emit(h, c, x, s):
                    ub[v][q].ref[state(0, h, c)] = s
                yield from ssm_output(b, q, v, emit)
                yield ub[v][q], -1

    def t_column(b, c):
        dest = bufs["oc"][c]
        terms = sorted((s, m, sign * _O_ALL.sign[r]) for m, r in enumerate(_O_ALL.order)
                       for (j, s), sign in _SCHEME.out[_NAMES[r]].items() if j == c)
        yield 6 * _LS[b] + 1
        for q in range(_LS[b]):
            chunks = [products(("C", b))[q][v][1] for v in range(2)]
            for n in sorted({m // _CHUNK for _, m, _ in terms}):
                for v in range(2):
                    yield chunks[v][n], 0
            yield None, 3
            acc = {}
            for s, m, sign in terms:
                val = _cat(*[chunks[v][m // _CHUNK].ref[m % _CHUNK] for v in range(2)])
                if (0, s) in acc:
                    acc[0, s].add(sign, val)
                else:
                    acc[0, s] = _Sum(sign, val)
            yield None, 1
            g = [_silu_half(d[0]) for d in _columns(acc, 1)]
            for v in range(2):
                yield ub[v][q], 1
            for h in range(2):
                res = lax.mul(load_state(q, state(0, h, c)), g[h])
                for v, part in enumerate((_lo(res), _hi(res))):
                    dest.ref[out_rows(b, q, v, h), :] = lax.add(xf[b][c].ref[out_rows(b, q, v, h), :], part)
            yield dest, -1
        yield None, 1
        copy_out(b, c, dest, 0)
        yield dest, -1

    tasks = dict(coefs=t_coefs, prep=t_prep, stage=t_stage, stats=t_stats, moments=t_moments, ln=t_ln,
                 project=t_project, starts=t_starts, states=t_states, act=t_act, act_rest=t_act_rest,
                 finish=t_finish, out=t_out, skip=t_skip, column=t_column)

    def dots(key, issued):
        kind, b = key[0], key[1]
        w = lambda *a: functools.partial(weight, *a)
        keep = lambda place: lambda vs: [(place, vs[0])]
        everywhere = range(_LS[b])
        res = []

        def halves(buf, dims, group, keep):
            (lhs, rhs, _), = group
            n = (_LS[b] + 1) // 2
            return buf, dims, [(lhs, rhs, everywhere[:n]), (lhs, rhs, everywhere[n:])], lambda vs: keep([_cat(*vs)])

        def grouped(name, half):
            for n, (s, a, bb, c, ca, cb) in enumerate(_GROUPS):
                def fold(vs, first=3 * n, signs=(ca * _V_FULL.sign[s] * _V_FULL.sign[a],
                                                 cb * _V_FULL.sign[s] * _V_FULL.sign[bb])):
                    sums = [(lax.add if sg > 0 else lax.sub)(v, vs[1]) for sg, v in zip(signs, vs[2:])]
                    return [((half, _O_KEPT.order.index(r)), v) for r, v in enumerate(sums + vs[:1], first)]
                res.append((xl[b % 2], NT, [([_NAMES.index(p)], [w(name, p)], everywhere) for p in (c, s, a, bb)], fold))

        if kind == "B":
            grouped("b0", 1)
            grouped("b1", 0)
        elif kind == "b" and key[2] == 3:
            grouped("b1", 0)
        elif kind == "G":
            grouped("g%d" % key[2], 0)
            grouped("u%d" % key[2], 1)
        elif kind == "r" and key[2]:
            grouped("r0", 0)
        elif kind in "Rr":
            rest = [(xl[b % 2], NT, [([_NAMES.index(p) for p, _ in parts], [w("r1", (n, p)) for p, _ in parts],
                                     everywhere)], keep((1, _O_N2.order.index(n))))
                    for n, (_, parts) in enumerate(_N2)]
            if kind == "R":
                grouped("r0", 0)
                res = rest[1:] + res + rest[:1]
            else:
                res = [halves(*rest[0])] + rest[1:]
        else:
            for p in _products(key):
                r = _NAMES.index(p)
                place = _O_ALL.order.index(r)
                if kind == "b":
                    res.append((xl[b % 2], NT, [([r], [w("b0", p)], everywhere)], keep((1, place))))
                elif kind == "C":
                    res.append((hl[b % 2], NT, [([r, _R + r], [w("c0", p), w("c1", p)], everywhere)], keep((0, place))))
                else:
                    lhs, rhs = [r, _R + r], [w("d0", p), w("d1", p)]
                    if p in _W_K4:
                        lhs.append(K4 + _NAMES_K4.index(p))
                        rhs.append(w("d2", p))
                    if p in _D4:
                        lhs += [K4D + 4 * _D4.index(p) + i for i in range(4)]
                        rhs += [functools.partial(tile_rows, *_TABLES["d2"][1:], i, 4) for i in range(4)]
                    cuts = [i for i in range(len(lhs) + 1) if i in (0, len(lhs)) or (issued + i) % 4 == 0]
                    issued += len(lhs)
                    for i, j in zip(cuts, cuts[1:]):
                        res.append((dl, NN, [(lhs[i:j], rhs[i:j], everywhere)], keep((1 + (i > 0), place))))
        if key == plan.phases[-1]:
            res[-1] = halves(*res[-1])
        return res

    def stream():
        for n, (t, _, _) in enumerate(plan.tasks):
            if t[0] not in ("wait", "pause"):
                task = tasks[t[0]](*t[1:])
                done, total = 0.0, next(task)
                for buf, cost in task:
                    if cost >= 0:
                        yield buf, n + done / total, None
                        done += cost
                    else:
                        yield buf, None, -cost * _WINDOW.get(t[0], 17)
                assert abs(done - total) < 1e-6 * total

    waits = [(n, t[1:]) for n, (t, _, _) in enumerate(plan.tasks) if t[0] == "wait"]
    work = stream()
    item = next(work)
    issued, current = 0, (-1, {})
    due = {}

    def operand(buf, slot, where, rnd):
        nonlocal current
        zeros = dict(current[1]) if rnd == current[0] else {}
        for k in [k for k in due if k[0] <= rnd]:
            zeros.setdefault(min(max(k[1], where[0]), where[-1]), []).extend(due.pop(k))
        zeros = {q: [functools.reduce(lax.bitwise_or, zs)] for q, zs in zeros.items() if q in where}
        current = rnd, zeros
        if not zeros:
            return buf.ref[slot, pl.ds(8 * where[0], 8 * len(where)), :]
        rows = [buf.ref[slot, pl.ds(8 * q, 8), :] for q in where]
        for q, (v,) in zeros.items():
            rows[q - where[0]] = lax.bitwise_or(rows[q - where[0]], v)
        return _cat(*rows)

    def run_phase(key):
        nonlocal issued, item
        L, i = _LS[key[1]], plan.phases.index(key)
        dest = products(key)
        first = issued // 4
        released = first - 1
        for buf, dims, group, keep in dots(key, issued):
            vs = []
            for lhs, rhs, where in group:
                a = [operand(buf, slot, where, (issued + n) // 4) for n, slot in enumerate(lhs)]
                a = a[0] if len(a) == 1 else lax.concatenate(a, 1)
                w = [load() for load in rhs]
                w = w[0] if len(w) == 1 else lax.concatenate(w, 1 if dims is NT else 0)
                vs.append(lax.dot_general(pltpu.bitcast(a, BF16), w, dims, preferred_element_type=F32))
                issued += len(rhs)
            rnd = (issued - 1) // 4
            kept = keep(vs)
            mark = kept[1 % len(kept)][1]
            for q in range(L):
                for (half, slot), val in kept:
                    for v in range(2):
                        chunk = dest[q][v][min(half, 1)][slot // _CHUNK]
                        rows = lax.slice_in_dim(val, 16 * q + 8 * v, 16 * q + 8 * v + 8, axis=0)
                        chunk.ref[slot % _CHUNK] = lax.add(chunk.view[slot % _CHUNK], rows) if half > 1 else rows
                fenced = []
                goal = min([plan.progress(i, ((rnd - first) * L + q + 1) / plan.slots[i]) - 1e-6]
                           + [n for n, _ in waits])
                while rnd > released and item is not None and (item[1] is None or item[1] < goal):
                    if item[1] is None:
                        late = max(L, q + item[2])
                        due.setdefault((rnd + late // L, late % L), []).append(item[0].done())
                    elif item[0] is not None and item[0] not in fenced:
                        fenced.append(item[0])
                        item[0].fence(lax.slice_in_dim(mark, 16 * q, 16 * q + 8, axis=0))
                    item = next(work, None)
            released = rnd
            reached = plan.progress(i, (rnd - first + 1) * L / plan.slots[i])
            while waits and waits[0][0] + 1 <= reached + 1e-6 and issued % 4 == 0:
                for cp in copies[waits.pop(0)[1]]:
                    cp.wait()
        assert item is None or item[1] >= plan.lo[i] - 1e-6
        assert not waits or waits[0][0] >= plan.lo[i]

    for cp in sum(copies.values(), []):
        cp.start()
    for step in plan.steps:
        if step[0] == "wait":
            for cp in copies[step[1:]]:
                cp.wait()
        elif step[0] == "run":
            task, written = tasks[step[1]](*step[2:]), []
            next(task)
            for buf, cost in task:
                if cost < 0 and buf not in written:
                    written.append(buf)
            for buf in written:
                buf.fence(jnp.zeros((8, LANE), F32))
        else:
            run_phase(step)
    assert item is None and not waits
    for cp in out_copies:
        cp.wait()


@jax.jit
def pallas_recurrent_scan__ssm_conv_s5__geglu_ffn__prompt_kernel(
    A_x, A_Lambda_re, A_Lambda_im, A_B_re, A_B_im, A_C_re, A_C_im, A_log_dt, A_Dskip,
    B_x, B_w_gate, B_w_up, B_w_down,
):
    del B_x
    batch, S, D = A_x.shape
    F = B_w_down.shape[0]
    assert (batch, S, D, F) == (1, 32 * sum(_LS), 5 * LANE, 13 * LANE + LANE // 2)
    plan = _Schedule()
    out = pl.pallas_call(
        functools.partial(_kernel, plan),
        in_specs=[pl.BlockSpec(memory_space=pl.ANY)] * 12,
        out_specs=pl.BlockSpec(memory_space=pl.ANY),
        out_shape=jax.ShapeDtypeStruct((S, D), F32),
        scratch_shapes=[_scratch(plan, S, D, F)],
        compiler_params=pltpu.CompilerParams(vmem_limit_bytes=126 * 2**20),
    )(A_x.reshape(S, D), A_Lambda_re, A_Lambda_im, A_B_re, A_B_im, A_C_re, A_C_im, A_log_dt, A_Dskip,
      B_w_gate.T, B_w_up.T, B_w_down)
    return out.reshape(batch, S, D)
```

```python
import functools

import numpy as np
import jax
import jax.numpy as jnp
from jax import lax
import jax.experimental.pallas as pl
import jax.experimental.pallas.tpu as pltpu

F32 = jnp.float32
BF16 = jnp.bfloat16
U32 = jnp.uint32
LANE = 128
NT = (((1,), (1,)), ((), ()))
NN = (((1,), (0,)), ((), ()))


def _acc(d, k, c):
    d[k] = d.get(k, 0) + c
    if d[k] == 0:
        del d[k]


class _HK:
    def __init__(self, methods, via):
        self.names, self.lhs, self.out = [], {}, {}
        n = len(methods)
        self.idx = [self._index(str(i), {i: 1}, {i: 1}, m) for i, m in enumerate(methods)]
        self.y, virt = {}, {}
        for i in range(n):
            self.y[i, i] = {self.idx[i][4]: 1, self.idx[i][5]: -1}
        for i in range(n):
            for j in range(n):
                if (methods[i] + 1) % 3 == methods[j]:
                    self.y[i, j], self.y[j, i], v = self._pair(self.idx[i], self.idx[j])
                    virt[i, j] = (v, 1)
                    virt[j, i] = (v, -1)
        for (i, j), l in via:
            v, sg = virt[j, l]
            if (methods[i] + 1) % 3 == v[3]:
                yiv, yvi, _ = self._pair(self.idx[i], v)
            else:
                yvi, yiv, _ = self._pair(v, self.idx[i])
            d = dict(yiv)
            for k, c in self.y[i, l].items():
                _acc(d, k, -c)
            self.y[i, j] = d
            d = {k: sg * c for k, c in yvi.items()}
            for k, c in self.y[l, i].items():
                _acc(d, k, c)
            self.y[j, i] = d
        assert len(self.y) == n * n

    def _prod(self, name, lhs, out):
        self.names.append(name)
        self.lhs[name], self.out[name] = lhs, out

    def _index(self, name, a, c, m):
        m1, m2 = (m + 1) % 3, (m + 2) % 3
        d1, d2 = name + ".1", name + ".2"
        self._prod(d1, {(i, m1): v for i, v in a.items()}, {(j, m2): v for j, v in c.items()})
        self._prod(d2, {(i, m2): v for i, v in a.items()}, {(j, m1): v for j, v in c.items()})
        return (name, a, c, m, d1, d2)

    def _pair(self, I, J):
        s = I[3]
        s1 = (s + 1) % 3
        assert s1 == J[3]
        a, c, lhs, out = dict(I[1]), dict(I[2]), {}, {}
        for k, v in J[1].items():
            _acc(a, k, -v)
        for k, v in J[2].items():
            _acc(c, k, v)
        V = self._index("(%s-%s)" % (I[0], J[0]), a, c, (s + 2) % 3)
        for k, v in I[1].items():
            _acc(lhs, (k, s1), v)
        for k, v in J[1].items():
            _acc(lhs, (k, s), v)
        for k, v in I[2].items():
            _acc(out, (k, s1), v)
        for k, v in J[2].items():
            _acc(out, (k, s), -v)
        sn = "S(%s,%s)" % (I[0], J[0])
        self._prod(sn, lhs, out)
        return ({sn: 1, V[4]: 1, I[5]: 1, J[5]: -1}, {sn: 1, V[5]: 1, I[4]: 1, J[4]: -1}, V)

    def weights(self, entries):
        w = {}
        for ij in entries:
            for p, c in self.y[ij].items():
                _acc(w.setdefault(p, {}), ij, c)
        return {p: d for p, d in w.items() if d}


def _slp(targets):
    ts = [dict(t) for t in targets]
    ops = []
    while any(len(t) > 1 for t in ts):
        cnt = {}
        for t in ts:
            ks = sorted(t, key=repr)
            for x in range(len(ks)):
                for y in range(x + 1, len(ks)):
                    key = (ks[x], ks[y], t[ks[x]] * t[ks[y]])
                    cnt[key] = cnt.get(key, 0) + 1
        a, b, sg = max(cnt, key=lambda k: cnt[k])
        new = ("t", len(ops))
        ops.append((new, a, b, sg))
        for t in ts:
            if a in t and b in t and t[a] * t[b] == sg:
                t[new] = t.pop(a)
                del t[b]
    return ops, [next(iter(t.items()))[::-1] for t in ts]


def _signed_sum(p, q, sign=1):
    (sp, vp), (sq, vq) = p, q
    if sp == sq:
        return sp, lax.add(vp, vq)
    return sign, (lax.sub(vp, vq) if sp == sign else lax.sub(vq, vp))


def _slp_signs(slp, signs):
    ops, results = slp
    signs = dict(signs)
    for new, a, b, sg in ops:
        signs[new] = signs[a] if signs[a] == sg * signs[b] else 1
    return [s * signs[v] for s, v in results]


class _Sum:
    def __init__(self, sign, value):
        self.terms = [(sign, value)]

    def get(self, sign):
        return _signed_sum(*self.terms, sign) if len(self.terms) == 2 else self.terms[0]

    def add(self, sign, value):
        self.terms = [self.get(-sign), (sign, value)]


class _Transposed:
    def __init__(self, slp, dry=False):
        ops, self.results = slp
        self.dry, self.adj = dry, {}
        self.split = {new: (a, b, sg) for new, a, b, sg in ops}
        self.pending = {}
        for v in [v for _, v in self.results] + [v for _, a, b, _ in ops for v in (a, b)]:
            self.pending[v] = self.pending.get(v, 0) + 1

    def put(self, v, sign, val):
        if v not in self.adj:
            self.adj[v] = _Sum(sign, val)
        elif not self.dry:
            self.adj[v].add(sign, val)
        self.pending[v] -= 1
        if self.pending[v] == 0 and v in self.split:
            a, b, sg = self.split[v]
            s, val = self.adj.pop(v).get(1)
            self.put(a, s, val)
            self.put(b, s * sg, val)

    def feed(self, t, val, sign=1):
        s, v = self.results[t]
        self.put(v, s * sign, val)


_FORM_SIGN = (1, -1, 1)
_SCHEME = _HK((0, 0, 1, 1, 2), (((0, 1), 2), ((2, 3), 0)))
_NAMES = list(_SCHEME.names)
_R = len(_NAMES)
_LHS_SLP = _slp([_SCHEME.lhs[p] for p in _NAMES])
_LHS_SIGN = dict(zip(_NAMES, _slp_signs(_LHS_SLP, {(i, s): _FORM_SIGN[s] for i in range(5) for s in range(3)})))
_W_FULL = _SCHEME.weights([(i, j) for i in range(5) for j in range(5)])
_W_K4 = _SCHEME.weights([(i, j) for i in range(4) for j in range(4)])
_NAMES_K4 = [p for p in _NAMES if p in _W_K4]
_D4 = _SCHEME.idx[4][4], _SCHEME.idx[4][5]
_LHS_SLP_K4 = _slp([_SCHEME.lhs[p] for p in _NAMES_K4])
assert [_LHS_SIGN[p] for p in _NAMES_K4] == _slp_signs(
    _LHS_SLP_K4, {(i, s): _FORM_SIGN[s] for i in range(4) for s in range(3)})


def _n2_products():
    res = []
    for i, j in ((0, 2), (1, 3)):
        w = _SCHEME.weights([(i, i), (i, j), (j, i), (j, j)])
        col = {i: 0, j: 1}
        for p in _NAMES:
            if p in w:
                res.append((p, {(col[c], s): v for (c, s), v in _SCHEME.out[p].items()},
                            {(a, col[b]): v for (a, b), v in w[p].items()}))
    for c in range(2):
        res.append((_D4[0], {(c, 1): 1}, {(4, c): 1}))
        res.append((_D4[1], {(c, 0): 1}, {(4, c): -1}))
    forms = []
    for _, out, _ in res:
        if out not in forms:
            forms.append(out)
    merged = [(f, [(p, w) for p, out, w in res if out == f]) for f in forms]
    one, two, three = ([m for m in merged if len(m[1]) == n] for n in (1, 2, 3))
    return two[:1] + [three[0], one[0], three[1], one[1]] + two[1:]


def _groups():
    vec = {}
    for p in _NAMES:
        vec[p] = {}
        for (j, form), c in _SCHEME.out[p].items():
            for half, v in (((1, 1),), ((0, 1),), ((0, -1), (1, -1)))[form]:
                _acc(vec[p], (j, half), c * v)

    def relation(s, a, b):
        for ca in (1, -1):
            for cb in (1, -1):
                d = dict(vec[s])
                for p, c in ((a, ca), (b, cb)):
                    for k, v in vec[p].items():
                        _acc(d, k, -c * v)
                if not d:
                    return ca, cb

    def match(sums, free):
        if not sums:
            return []
        s = sums[0]
        pair = _NAMES[_NAMES.index(s) - 2:_NAMES.index(s)]
        for a in free:
            for b, c in (pair, pair[::-1]):
                if relation(s, a, b):
                    rest = match(sums[1:], [p for p in free if p != a])
                    if rest is not None:
                        return [(s, a, b, c) + relation(s, a, b)] + rest
    return match([p for p in _NAMES if p[0] == "S"], [p for p in _NAMES if p[0].isdigit()])


_N2 = _n2_products()
_GROUPS = _groups()
_KEPT = [p for g in _GROUPS for p in g[1:4]]


class _Weights:
    def __init__(self, w, lhs_sign, order, move_sign=True, in_place=True):
        w = {p: {k: lhs_sign[p] * c for k, c in d.items()} for p, d in w.items()}
        self.sign = {p: next(iter(d.values())) if len(d) == 1 and move_sign else 1 for p, d in w.items()}
        self.single = {p: next(iter(d)) for p, d in w.items() if len(d) == 1 and in_place}
        self.summed = [p for p in lhs_sign if p in w and p not in self.single]
        self.terms = [len(w[p]) for p in self.summed]
        self.slp = _slp([{k: c * self.sign[p] for k, c in w[p].items()} for p in self.summed])
        self.used = sorted({k for p in self.summed for k in w[p]})
        self.order = order
        assert sorted(order) == list(range(len(self.summed)))


_V_FULL = _Weights(_W_FULL, _LHS_SIGN, (11, 25, 24, 12, 14, 16, 5, 4, 0, 13, 17, 1, 20, 22, 8, 9, 18, 23, 2, 3, 15,
                                        19, 7, 6, 10, 21))
_V_K4 = _Weights(_W_K4, _LHS_SIGN, (8, 11, 1, 18, 15, 10, 0, 19, 9, 4, 14, 5, 12, 13, 16, 6, 7, 2, 17, 3))
_V_ALL = _Weights(_W_FULL, _LHS_SIGN, (11, 36, 10, 39, 12, 16, 0, 14, 5, 1, 34, 13, 29, 17, 4, 24, 30, 18, 9, 37, 8,
                                       23, 33, 28, 3, 35, 38, 2, 25, 15, 21, 7, 20, 27, 19, 22, 31, 26, 6, 32),
                  in_place=False)
_V_N2 = _Weights({(n, p): w for n, (_, parts) in enumerate(_N2) for p, w in parts},
                 {(n, p): _LHS_SIGN[p] for n, (_, parts) in enumerate(_N2) for p, _ in parts},
                 (8, 6, 14, 10, 16, 9, 2, 0, 4, 5, 1, 13, 3, 12, 15, 17, 11, 7), move_sign=False, in_place=False)
assert all(_V_K4.sign[p] == _V_FULL.sign[p] for p in _NAMES_K4) and all(_V_FULL.sign[p] == 1 for p in _D4)


class _Outputs:
    def __init__(self, outs, signs):
        self.slp, self.sign = _slp(outs), signs
        self.ncol = 1 + max(j for out in outs for j, _ in out)
        self.order, rest = [], list(range(len(outs)))
        while rest:
            self.order.append(min(rest, key=lambda t: self._live(self.order + [t])))
            rest.remove(self.order[-1])

    def _live(self, seq):
        tr = _Transposed(self.slp, dry=True)
        for t in seq:
            tr.feed(t, None)
        todo = [[tr.pending.get((j, s), 0) for s in range(3)] for j in range(5)]
        return len(tr.adj) - sum(not any(n) for n in todo), sum(n ** 0.5 for col in todo for n in col)


_O_ALL = _Outputs([_SCHEME.out[p] for p in _NAMES], [_V_FULL.sign[p] for p in _NAMES])
_O_KEPT = _Outputs([_SCHEME.out[p] for p in _KEPT], [_V_FULL.sign[p] for p in _KEPT])
_O_N2 = _Outputs([f for f, _ in _N2], [1] * len(_N2))


def _lhs_sums(slp, a1, a2):
    env = {}
    for i, (x, y) in enumerate(zip(a1, a2)):
        env[i, 0], env[i, 1], env[i, 2] = (1, x), (-1, y), (1, lax.sub(y, x))
    for new, a, b, sg in slp[0]:
        env[new] = _signed_sum(env[a], (sg * env[b][0], env[b][1]))
    return [env[v][1] for _, v in slp[1]]


def _columns(acc, ncol):
    c1, c2 = [], []
    for j in range(ncol):
        s2, v2 = acc[j, 2].get(1)
        for form, dst in ((1, c1), (0, c2)):
            s, v = _signed_sum(acc[j, form].get(s2), (-s2, v2))
            dst.append(v if s > 0 else lax.neg(v))
    return c1, c2


def _lo(v):
    return lax.slice_in_dim(v, 0, v.shape[0] // 2, axis=0)


def _hi(v):
    return lax.slice_in_dim(v, v.shape[0] // 2, v.shape[0], axis=0)


def _cat(*vs):
    return lax.concatenate(vs, 0)


def _pack(v):
    return lax.bitcast_convert_type(pltpu.pack_elementwise([_lo(v), _hi(v)], packed_dtype=BF16), U32)


def _unpack(w):
    return _cat(*[pltpu.unpack_elementwise(w, index=i, packed_dtype=BF16, unpacked_dtype=F32) for i in range(2)])


def _cmul(ar, ai, br, bi):
    return lax.sub(lax.mul(ar, br), lax.mul(ai, bi)), lax.add(lax.mul(ar, bi), lax.mul(ai, br))


def _cmad(ar, ai, br, bi, cr, ci):
    tr, ti = _cmul(ar, ai, br, bi)
    return lax.add(tr, cr), lax.add(ti, ci)


def _gelu2(g):
    k = 0.7978845608028654
    return lax.add(g, lax.mul(g, lax.tanh(lax.mul(g, k + (k * 0.044715) * lax.mul(g, g)))))


def _silu_half(d):
    z = 0.25 * d
    return lax.add(z, lax.mul(z, lax.tanh(z)))


_LS = (17, 17, 17, 13)
_NB, _LM = len(_LS), max(_LS)
_CHUNK = 20
_FIRST = (4, 3, 1)

_nt = lambda i, j: (LANE * j, LANE * i)
_nn = lambda i, j: (LANE * i, LANE * j)
_TABLES = dict(b0=(_V_FULL, "bre", 0, _nt), b1=(_V_FULL, "bim", 0, _nt),
               c0=(_V_ALL, "cre", 0, _nt), c1=(_V_ALL, "cim", 0, _nt),
               g0=(_V_FULL, "wg", 0, _nt), u0=(_V_FULL, "wu", 0, _nt),
               g1=(_V_FULL, "wg", 5 * LANE, _nt), u1=(_V_FULL, "wu", 5 * LANE, _nt),
               r0=(_V_FULL, "wr", 0, _nt), r1=(_V_N2, "wr", 5 * LANE, _nt),
               d0=(_V_FULL, "wd", 0, _nn), d1=(_V_FULL, "wd", 5 * LANE, _nn), d2=(_V_K4, "wd", 10 * LANE, _nn))

_PER_POSITION = dict(stage=30, stats=38, ln=95, project=130, states=195, act=175, act_rest=120, finish=165,
                     skip=75, column=35)
_ONCE = dict(starts=300, out=1, coefs=500, r1=300, u1=800, d2=500, c0=1800, c1=1500)
_PAUSE = dict(states=300, finish=300, act_rest=300, project=300, ln=200, bim=800, wr=1500, x1=1, wgu=1, rest=1)
_WINDOW = dict(act=14, column=13, states=15, finish=18)
_TUNING = {
    ("b", 0, 2): (-1.5, 0, 0.25, 1, "csab", 0, {}),
    ("b", 0, 3): (-0.25, 0, 1, 1, "acbs", 0, {}),
    ("r", 0, 0): (0, 1, 0.25, 1, "csab", -300, {8: 0.88}),
    ("r", 0, 1): (0, 3, 0.5, 1, "csab", 0, {11: 1.1}),
    ("B", 1): (0.25, 0, 1, 1, "csab", 60, {}),
    ("G", 0, 0): (0, 3, 1, 2, "csab", 0, {17: 0.9, 18: 1.25}),
    ("G", 0, 1): (-0.5, 0, 0.5, 1, "csab", 0, {26: 0.9}),
    ("R", 1): (1.75, 0, 1, 1, "csab", 0, {}),
    ("D", 0): (0.5, 1, 0.5, 0, "csab", 0, {29: 0.81}),
    ("G", 1, 0): (0, 1, 1.5, 2, "cbsa", 0, {}),
    ("G", 1, 1): (0, 1, 1, 1, "bacs", 0, {41: 0.9}),
    ("B", 2): (0, 0, 2, 2, "csab", -60, {46: 0.8}),
    ("R", 2): (0, -1, 1, 1, "cbas", 0, {47: 1.6}),
    ("D", 1): (-0.5, 0, 2, 2, "csab", 300, {}),
    ("C", 1): (0.25, 1, 0.75, 1, "csab", 0, {56: 1.6}),
    ("G", 2, 0): (0, 0, 1.75, 2, "csab", 0, {}),
    ("G", 2, 1): (0.5, -2, 2, 2, "csab", 0, {}),
    ("B", 3): (0.5, -2, 0.5, 1, "csab", 0, {}),
    ("R", 3): (-0.5, 0, 1, 1, "sabc", 0, {}),
    ("D", 2): (0.5, 0, 1, 0, "csab", 0, {}),
    ("C", 2): (0, 2, 1.5, 0, "csab", 0, {}),
    ("G", 3, 0): (0.5, 0, 1, 1, "bcas", 0, {}),
    ("d", 3, 0): (-0.25, 0, 1, 1, "csab", 0, {}),
    ("d", 3, 1): (0, 2, 1, 2, "csab", 0, {}),
    ("d", 3, 2): (-2, 0, 0.25, 1, "csab", 0, {}),
    ("d", 3, 3): (0.75, 1, 0.25, 1, "csab", 0, {}),
    ("d", 3, 4): (0, 0, 0.5, 1, "csab", 0, {}),
}
_UNTUNED = (0, 0, 1, 1, "csab", 0, {})


def _products(key):
    if key[0] == "b":
        stage = lambda p: 2 if len(_W_FULL[p]) > 2 else p not in _V_FULL.single or _V_FULL.single[p][0] not in _FIRST
        return _NAMES if key[2] == 3 else sorted((p for p in _NAMES if stage(p) == key[2]),
                                                 key=lambda p: len(_W_FULL[p]))
    if key[0] == "d":
        return [p for p in _products(("D",)) if min(j for j, _ in _SCHEME.out[p]) == key[2]]
    return sorted(_NAMES, key=lambda p: p in _W_K4) if key[0] == "D" else _NAMES


def _n_tiles(key):
    if key[0] in "Dd":
        return sum(2 + (p in _W_K4) + 4 * (p in _D4) for p in _products(key))
    if key[0] == "r":
        return _R if key[2] else len(_V_N2.summed) + 2
    return dict(R=_R + len(_V_N2.summed), b=len(_products(key))).get(key[0], 2 * _R)


def _plan():
    R, B, C, D = (lambda b, k=k: (k, b) for k in "RBCD")
    G = lambda b, g: ("G", b, g)
    during = lambda first, last, *tasks: [(t, first, last) for t in tasks]
    prep = lambda names: [("prep", n) for n in names.split()]
    norm = lambda b: [("stage", b), ("stats", b, 0), ("stats", b, 1), ("ln", b)]
    b0, b1, b2, b3 = (("b", 0, n) for n in range(4))
    r0, r1 = ("r", 0, 0), ("r", 0, 1)

    steps = []
    for n in range(4):
        steps += [("wait", "x0", n), ("run", "moments", n)]
    steps += [("run", "ln", 0), ("wait", "bre", 0), b0, ("wait", "bre", 1), ("run", "prep", "b0", 0), b1,
              ("run", "prep", "b0", 1), b2, b3, r0, r1, B(1), G(0, 0), G(0, 1), R(1), D(0)]
    tasks = (during(b2, b2, ("wait", "bim"), *prep("b1")) + during(b3, b3, ("coefs",), ("wait", "wr"), *prep("r1"))
             + during(r0, r0, *prep("r0")) + during(r0, r1, ("wait", "x1"), *norm(1))
             + during(r1, G(0, 0), ("project", 0)) + during(B(1), B(1), ("wait", "wgu"), *prep("g0 u0"))
             + during(B(1), G(0, 0), *prep("g1 u1")) + during(B(1), D(0), ("starts", 0))
             + during(B(1), G(0, 1), ("act_rest", 0))
             + during(G(0, 1), R(1), ("act", 0, 0), ("wait", "rest"), *prep("d0 d1 d2"))
             + during(R(1), R(1), ("act", 0, 1)) + during(R(1), D(0), *prep("c0 c1"), ("states", 0)))
    for b in range(1, _NB):
        more = b + 1 < _NB
        extra = B(b + 1) if more else C(b)
        down = [R(b + 1), D(b)] if more else [("d", b, c) for c in range(5)]
        steps += [C(b - 1), G(b, 0), G(b, 1), extra] + down
        second = during(R(b), G(b, 1), *norm(2)) if b == 1 else []
        tasks += second[:2] + during(R(b), C(b - 1), ("project", b)) + second[2:]
        tasks += during(C(b - 1), G(b, 1), ("act_rest", b), ("starts", b))
        if not more:
            tasks += during(C(b - 1), G(b, 1), ("states", b))
        tasks += during(G(b, 0), down[0] if more else extra, ("finish", b - 1), ("out", b - 1))
        tasks += during(G(b, 1), extra, ("act", b, 0)) + during(extra, down[0] if more else extra, ("act", b, 1))
        if b + 2 < _NB:
            tasks += during(down[0], G(b + 1, 1), *norm(b + 2))
        if more:
            tasks += during(C(b - 1), D(b), ("states", b))
        else:
            tasks += during(down[0], down[0], ("skip", b))
            tasks += [(("column", b, c), down[c + 1], down[-1]) for c in range(4)]
            steps += [("run", "column", b, 4)]
    return steps, [u for t in tasks for u in [(("pause", t[0][0]),) + t[1:]] * (t[0][0] in _PAUSE) + [t]]


def _spread(cycles, work, lo, hi):
    def run(load, p0, p1, u):
        ends, idle = [], []
        for p in range(p0, p1):
            left = load * cycles[p]
            while u < hi[p] and left > 0:
                need = (int(u) + 1 - u) * work[int(u)][p]
                u, left = (int(u) + 1, left - need) if need <= left else (u + left / work[int(u)][p], 0)
            ends.append(u)
            idle.append(left > 0)
        return ends, idle

    def solve(p0, p1, u, last):
        if p0 == p1:
            return []
        need = lo[p0:p1 - 1] + [max(lo[p1 - 1], last)]
        a, b = 0.0, 8.0
        for _ in range(40):
            m = (a + b) / 2
            a, b = (a, m) if all(e >= n for e, n in zip(run(m, p0, p1, u)[0], need)) else (m, b)
        j = next((p0 + k for k, (e, n) in enumerate(zip(run(a, p0, p1, u)[0], need)) if e < n), p1 - 1)
        ends, idle = run(b, p0, j + 1, u)
        i = max([p0 + k + 1 for k in range(j - p0) if idle[k]], default=p0)
        ends[-1] = max(need[j - p0], u)
        return solve(p0, i, u, hi[i - 1]) + ends[i - p0:] + solve(j + 1, p1, ends[-1], last)

    return solve(0, len(cycles), 0.0, 0)


class _Schedule:
    def __init__(self):
        self.steps, self.tasks = _plan()
        self.phases = phases = [s for s in self.steps if s[0] not in ("wait", "run")]
        self.work = [[self._cycles(t, p) for p in phases] for t, _, _ in self.tasks]
        cycles = [16 * _LS[p[1]] * max(_n_tiles(p) / 4 - 1, 1.0) for p in phases]
        hi = [next((n for n, t in enumerate(self.tasks) if phases.index(t[1]) > i), len(self.tasks))
              for i in range(len(phases))]
        self.lo = [max([n + 1 for n, t in enumerate(self.tasks) if phases.index(t[2]) <= i], default=0)
                   for i in range(len(phases))]
        self.target = [0.0] + _spread(cycles, self.work, self.lo, hi)
        for i, p in enumerate(phases):
            *_, shift, shares = _TUNING.get(p, _UNTUNED)
            u = self.target[i + 1]
            u += shift / max(self.work[min(int(u), len(self.tasks) - 1)][i], 1000)
            self.target[i + 1] = min(max(u, self.lo[i], self.target[i]), hi[i])
            for n, share in shares.items():
                self.work[n][i] *= share
        self.sets, busy = {}, []
        for i, p in enumerate(phases):
            k = self.products(p)
            if k not in self.sets:
                reader = (dict(B="project", R="act_rest", G="act", C="finish")[k[0]],) + k[1:]
                end = max((phases.index(t[2]) for t in self.tasks if t[0] == reader), default=len(phases))
                self.sets[k] = next((n for n, e in enumerate(busy) if e < i), len(busy))
                busy[self.sets[k]:self.sets[k] + 1] = [end]
        self.n_sets = len(busy)

    @staticmethod
    def products(key):
        return key if key[0] == "G" else (dict(b="B", r="R", D="C", d="C").get(key[0], key[0]), key[1])

    @staticmethod
    def _cycles(t, phase):
        if t[0] in ("pause", "wait"):
            return _PAUSE[t[1]]
        if t[0] in _PER_POSITION:
            return _LS[t[1]] * (170 if t[0] == "states" and phase[0] in "CDd" else _PER_POSITION[t[0]])
        return _ONCE.get(t[t[0] == "prep"], 680)

    def progress(self, i, x):
        u0, u1 = self.target[i], self.target[i + 1]
        knots = [u0] + list(range(int(u0) + 1, int(np.ceil(u1)))) + [u1]
        t = np.cumsum([0.0] + [(b - a) * self.work[int(a)][i] for a, b in zip(knots, knots[1:]) if b > a])
        return float(np.interp(x * t[-1], t, knots[:len(t)])) if x < 1 else u1


class _Buf:
    def __init__(self, ref, z):
        flat = len(ref.shape) == 2
        n = 32 // ref.dtype.itemsize if flat else 1
        end = ref.shape[0] - n
        self.ref, self.ready, self.copied = ref, False, False
        self.view = ref.at[pl.ds(pl.multiple_of(n * z, n) if flat else z, end)]
        self.spare, self.zeros = ((pl.ds(end - k * n, n), pl.ds(0, LANE)) if flat else (end - k, pl.ds(0, 8))
                                  for k in (1, 2))

    def fence(self, v):
        if self.ref.dtype == BF16:
            v = pltpu.bitcast(v, BF16)
        elif self.ref.dtype != v.dtype:
            v = lax.bitcast_convert_type(v, self.ref.dtype)
        self.view[self.spare] = v

    def done(self):
        if not self.ready:
            for rows in (self.zeros, self.spare):
                self.ref[rows] = jnp.zeros((32 // self.ref.dtype.itemsize, LANE), self.ref.dtype)
            self.ready = True
        if self.copied:
            self.fence(jnp.zeros((8, LANE), F32))
        v = (self.ref if self.copied else self.view)[self.zeros]
        self.copied = False
        return pltpu.bitcast(v, U32) if v.dtype == BF16 else lax.bitcast_convert_type(v, U32)


def _scratch(plan, S, D, F):
    NL = D // LANE
    slots = lambda n, rows, dtype: pltpu.VMEM((n + 3, rows, LANE), dtype)
    rows = lambda n: [pltpu.VMEM((32 * L * n + 24, LANE), F32) for L in _LS]
    buf = dict(
        raw=dict({k: [pltpu.VMEM((n + 48, LANE), BF16)] * NL for k, n in dict(
            bre=D, bim=D, cre=D, cim=D, wg=2 * D, wu=2 * D, wr=2 * (F - 2 * D), wd=F + -F % LANE).items()},
            x=pltpu.VMEM((S + 48, D), BF16)),
        v={k: slots(len(t[0].summed), LANE // 2, U32) for k, t in _TABLES.items()},
        xf=[[v] * NL for v in rows(1)], s0=rows(1), s1=rows(1), of=rows(NL)[:-1], oc=rows(1)[-1:] * NL,
        xl=[slots(_R, 8 * _LM, U32)] * 2, hl=[slots(2 * _R, 8 * _LM, U32)] * 2,
        dl=slots(2 * _R + len(_NAMES_K4) + 8, 8 * _LM, U32),
        u=[[slots(4 * NL, 8, F32)] * _LM] * 2, e=[slots(6, 16, F32)] * NL,
        coef=slots(4 + 2 * _LM + 8 * len(set(_LS)), 8, F32),
    )
    for n in range(plan.n_sets):
        most = [max(_R if k[0] == "C" or k == ("B", 0) and half else len(_KEPT) for k, m in plan.sets.items() if m == n)
                for half in range(2)]
        buf["p%d" % n] = [[[[slots(_CHUNK - 1, 8, F32)] * -(-m // _CHUNK) for m in most]] * 2] * _LM
    return dict(buf=buf, vec=[pltpu.VMEM((D,), BF16)] * 4,
                sem=[pltpu.SemaphoreType.DMA((11,)), pltpu.SemaphoreType.DMA, pltpu.SemaphoreType.REGULAR])


def _kernel(plan, x_hbm, lre_hbm, lim_hbm, bre_hbm, bim_hbm, cre_hbm, cim_hbm, ldt_hbm, dsk_hbm,
            wg_hbm, wu_hbm, wd_hbm, o_hbm, sc):
    in_sem, out_sem, idle_sem = sc["sem"]
    S, D = x_hbm.shape
    F = wd_hbm.shape[0]
    NL = D // LANE
    T0 = [32 * sum(_LS[:b]) for b in range(_NB)]

    z = jnp.clip(pl.semaphore_read(idle_sem), 0, 1)
    bufs = jax.tree.map(lambda ref: _Buf(ref, z), sc["buf"])
    raw = bufs["raw"]
    xl, hl, dl = bufs["xl"], bufs["hl"], bufs["dl"]
    xf, sb, of = bufs["xf"], (bufs["s0"], bufs["s1"]), bufs["of"]
    ub, eb, cf = bufs["u"], bufs["e"], bufs["coef"]

    def products(key):
        return bufs["p%d" % plan.sets[plan.products(key)]]

    copies = {}

    def copy(name, src, dst):
        copies.setdefault(name, [])
        copies[name].append(pltpu.make_async_copy(src, dst, in_sem.at[list(copies).index(name)]))

    def copy_x(name, r0, n):
        copy(name, x_hbm.at[pl.ds(r0, n)], raw["x"].ref.at[pl.ds(r0, n)])

    def copy_strips(name, src, r0, n, dst, d0=0, strips=range(NL)):
        for c in strips:
            copy(name, src.at[pl.ds(r0, n), pl.ds(LANE * c, LANE)], raw[dst][c].ref.at[pl.ds(d0, n)])

    pieces = [32 * (_LS[0] - _LS[0] * (4 - n) // 4) for n in range(5)]
    for n in range(4):
        copy_x(("x0", n), pieces[n], pieces[n + 1] - pieces[n])
    copy_strips(("bre", 0), bre_hbm, 0, D, "bre", 0, _FIRST)
    copy_strips(("bre", 1), bre_hbm, 0, D, "bre", 0, [c for c in range(NL) if c not in _FIRST])
    copy_strips(("bim",), bim_hbm, 0, D, "bim")
    for src, dst in zip((lre_hbm, lim_hbm, ldt_hbm, dsk_hbm), sc["vec"]):
        copy(("bim",), src, dst)
    n = F - 2 * D
    copy_strips(("wr",), wg_hbm, 2 * D, n, "wr")
    copy_strips(("wr",), wu_hbm, F - n % LANE, n % LANE, "wr", n)
    copy_strips(("wr",), wu_hbm, 2 * D, n - n % LANE, "wr", n + n % LANE)
    copy_x(("x1",), T0[1], 32 * _LS[1])
    copy_strips(("wgu",), wg_hbm, 0, 2 * D, "wg")
    copy_strips(("wgu",), wu_hbm, 0, 2 * D, "wu")
    copy_strips(("rest",), wd_hbm, 0, F, "wd")
    copy_strips(("rest",), cre_hbm, 0, D, "cre")
    copy_strips(("rest",), cim_hbm, 0, D, "cim")
    copy_x(("rest",), T0[2], S - T0[2])
    for strip in raw["wd"]:
        strip.ref[pl.ds(F, -F % LANE), :] = jnp.zeros((-F % LANE, LANE), BF16)
    out_copies = []

    def copy_out(b, c, src, n):
        T = 32 * _LS[b]
        src.copied = True
        out_copies.append(pltpu.make_async_copy(
            src.ref.at[pl.ds(n * T, T)], o_hbm.at[pl.ds(T0[b], T), pl.ds(LANE * c, LANE)], out_sem))
        out_copies[-1].start()


    high_powers = {L: 4 + 2 * _LM + 8 * n for n, L in enumerate(sorted(set(_LS)))}

    def t_coefs():
        yield 1
        yield None, 1
        lre, lim, ldt, dsk = (_cat(*[v[:, LANE * c:LANE * c + LANE] for c in range(NL)])
                              for v in (r[...].astype(F32).reshape(1, D) for r in sc["vec"]))
        dt = jnp.exp(ldt).astype(BF16).astype(F32)
        zr, zi = dt * lre, dt * lim
        mag = jnp.exp(zr)
        ar, ai = mag * jnp.cos(zi), mag * jnp.sin(zi)
        nr, ni = ar - 1.0, ai
        big = jnp.abs(lre) >= jnp.abs(lim)
        rat = jnp.where(big, lim / lre, lre / lim)
        den = jnp.where(big, lre + lim * rat, lre * rat + lim)
        qr = 2.0 * jnp.where(big, nr + ni * rat, nr * rat + ni) / den
        qi = 2.0 * jnp.where(big, ni - nr * rat, ni * rat - nr) / den
        powers = [(ar, ai)]
        for n in range(2, _LM + 1):
            powers.append(_cmul(*powers[n // 2 - 1], *powers[n - n // 2 - 1]))
        consts = [dsk, qr, qi, -qi] + [v for p in powers for v in p]
        for L in high_powers:
            p = powers[L - 1]
            for _ in range(4):
                p = _cmul(*p, *p)
                consts += p
        for n, v in enumerate(consts):
            cf.ref[n, pl.ds(0, NL), :] = v
        yield cf, -5

    def coef(n, c, reps=1):
        return jnp.broadcast_to(cf.ref[n, pl.ds(c, 1), :], (8 * reps, LANE))

    def power(n, c, reps=1):
        slot = 2 + 2 * n if n <= _LM else next(
            s + 2 * k for L, s in high_powers.items() for k in range(4) if n == L << k + 1)
        return coef(slot, c, reps), coef(slot + 1, c, reps)

    def tile_rows(src, row0, corner, i, j, r0=0, n=LANE):
        row, col = corner(i, j)
        return raw[src][col // LANE].ref[pl.ds(row0 + row + r0, n), :]

    def t_prep(name, long_sums=None):
        tab, src, row0, corner = _TABLES[name]
        dest = bufs["v"][name]
        ops, results = tab.slp
        parts = {new: (a, b, sg) for new, a, b, sg in ops}
        inner = [v for _, a, b, _ in ops for v in (a, b)]
        want = {v: s for s, v in results if v not in inner}
        seq = []

        def need(v):
            if v not in seq:
                for u in parts.get(v, ())[:2]:
                    need(u)
                seq.append(v)
        for n in tab.order:
            if long_sums in (None, tab.terms[n] > 2):
                need(results[n][1])
                seq.append(n)
        tiles = [v for v in seq if v in tab.used]
        yield 8 * len(tiles)
        for r0 in range(0, LANE, 16):
            env = {}
            for v in seq:
                if v in parts:
                    a, b, sg = parts[v]
                    env[v] = _signed_sum(env[a], (sg * env[b][0], env[b][1]), want.get(v, 1))
                elif v in tiles:
                    if tiles.index(v) % 9 == 0:
                        for m in ("cre", "cim") if name[0] == "c" else (src,):
                            yield raw[m][corner(*v)[1] // LANE], 0
                        yield None, len(tiles[tiles.index(v):][:9])
                    load = lambda src: _unpack(pltpu.bitcast(tile_rows(src, row0, corner, *v, r0, 16), U32))
                    if name[0] == "c":
                        re, im = (1, 2) if name == "c0" else (3, 1)
                        env[v] = 1, lax.sub(lax.mul(load("cre"), coef(re, v[0], 2)),
                                            lax.mul(load("cim"), coef(im, v[0], 2)))
                    else:
                        env[v] = 1, load(src)
                else:
                    s, val = env[results[v][1]]
                    dest.ref[v, pl.ds(r0 // 2, 8), :] = _pack(val if s * results[v][0] > 0 else lax.neg(val))
            yield dest, -2

    def weight(name, p):
        tab = _TABLES[name][0]
        if p in tab.single:
            return tile_rows(*_TABLES[name][1:], *tab.single[p])
        return pltpu.bitcast(bufs["v"][name].ref[tab.summed.index(p)], BF16)

    def gather_weight(outs):
        return 2.6 * len(outs.order) + 5 * -(-len(outs.order) // _CHUNK)

    def gather(key, q, v, half, outs):
        chunks = products(key)[q][v][half]
        tr = _Transposed(outs.slp)
        for m, r in enumerate(outs.order):
            if m % _CHUNK == 0:
                yield chunks[m // _CHUNK], 5 + 2.6 * min(_CHUNK, len(outs.order) - m)
            tr.feed(r, chunks[m // _CHUNK].ref[m % _CHUNK], outs.sign[r])
        return _columns(tr.adj, outs.ncol)

    def scatter(slp, names, a1, a2, buf, q, first, weight, bursts=None):
        vals = _lhs_sums(slp, a1, a2)
        last = [max(2, *(i for i, _ in _SCHEME.lhs[p])) for p in names]
        order = sorted(range(len(vals)), key=lambda n: last[n])
        if bursts:
            groups = [order[len(order) * i // bursts:len(order) * (i + 1) // bursts] for i in range(bursts)]
        else:
            groups = [[n for n in order if last[n] == i] for i in (2, 3, 4)]
        for group in groups:
            if bursts and bursts > 1:
                yield buf, 0
            for n in group:
                buf.ref[first + n, pl.ds(8 * q, 8), :] = _pack(vals[n])
            if not bursts or group is groups[-1]:
                yield buf, -1
            yield None, weight / len(groups)

    def in_rows(b, q, h):
        return [pl.ds((h + 2 * t) * _LS[b] + q, 8, stride=4 * _LS[b]) for t in range(2)]

    def out_rows(b, q, v, h, c=0):
        return pl.ds((32 * c + 8 * (2 * h + v)) * _LS[b] + q, 8, stride=_LS[b])

    def load_in(buf, b, q, h):
        return _cat(*[buf.ref[s, :] for s in in_rows(b, q, h)])

    def load_x(r0, c):
        return raw["x"].ref[pl.ds(r0, 32), pl.ds(LANE * c, LANE)].astype(F32)

    def row_mean(tiles):
        tot = jnp.sum(functools.reduce(lax.add, tiles), axis=-1, keepdims=True) * (1.0 / D)
        return jnp.broadcast_to(tot, tiles[0].shape)

    def t_stage(b):
        yield _LS[b]
        for r0 in range(0, 32 * _LS[b], 32):
            yield raw["x"], 1
            for c in range(NL):
                xf[b][c].ref[pl.ds(r0, 32), :] = load_x(T0[b] + r0, c)
            for dest in xf[b]:
                yield dest, -1

    def t_stats(b, n):
        yield 140 * _LS[b]
        for q in range(_LS[b]):
            for h in range(2):
                if n:
                    yield sb[0][b], 1
                xv = []
                for c in range(NL):
                    yield xf[b][c], 0
                    xv.append(load_in(xf[b][c], b, q, h))
                yield None, 70 - n
                if n:
                    mean = load_in(sb[0][b], b, q, h)
                    xv = [lax.mul(d, d) for d in (lax.sub(v, mean) for v in xv)]
                v = lax.rsqrt(row_mean(xv) + 1e-5) if n else row_mean(xv)
                for s, part in zip(in_rows(b, q, h), (_lo(v), _hi(v))):
                    sb[n][b].ref[s, :] = part
            yield sb[n][b], -2

    def t_moments(n):
        yield 0
        for r0 in range(pieces[n], pieces[n + 1], 32):
            xv = [load_x(r0, c) for c in range(NL)]
            mean = row_mean(xv)
            var = row_mean([lax.mul(d, d) for d in (lax.sub(v, mean) for v in xv)])
            for buf, v in zip(xf[0] + [sb[0][0], sb[1][0]], xv + [mean, lax.rsqrt(var + 1e-5)]):
                buf.ref[pl.ds(r0, 32), :] = v
                yield buf, -1

    def t_ln(b):
        yield 575 * _LS[b]
        for q in range(_LS[b]):
            yield sb[0][b], 2
            yield sb[1][b], 3
            stats = [[load_in(sb[n][b], b, q, h) for n in range(2)] for h in range(2)]
            halves = [[], []]
            for c in range(NL):
                yield None, (25, 25, 85, 115, 140)[c]
                for h, (mean, rstd) in enumerate(stats):
                    halves[h].append(lax.mul(lax.sub(load_in(xf[b][c], b, q, h), mean), rstd))
            yield from scatter(_LHS_SLP, _NAMES, *halves, xl[b % 2], q, 0, 180)

    def state(part, h, c):
        return (2 * part + h) * NL + c

    def load_state(q, n):
        return _cat(*[ub[v][q].ref[n] for v in range(2)])

    def t_project(b):
        real = _O_KEPT if b else _O_ALL
        yield 2 * (gather_weight(real) + gather_weight(_O_KEPT) + 120) * _LS[b]
        for q in range(_LS[b]):
            for v in range(2):
                ur = yield from gather(("B", b), q, v, 1, real)
                ui = yield from gather(("B", b), q, v, 0, _O_KEPT)
                yield None, 100
                for c in range(NL):
                    a = power(1, c) if q else None
                    for h in range(2):
                        e = ur[h][c], ui[h][c]
                        if q:
                            e = _cmad(*a, *(ub[v][q - 1].ref[state(t, h, c)] for t in range(2)), *e)
                        for t in range(2):
                            ub[v][q].ref[state(t, h, c)] = e[t]
                yield ub[v][q], -2
                yield None, 20

    def t_starts(b):
        L = _LS[b]
        row = lax.broadcasted_iota(jnp.int32, (16, LANE), 0)
        yield 149 * NL
        for c in range(NL):
            yield ub[0][L - 1], 4
            yield ub[1][L - 1], 5
            yield eb[c], 0
            even, odd = ([load_state(L - 1, state(t, h, c)) for t in range(2)] for h in range(2))
            f = _cmad(*power(L, c, 2), *even, *odd)
            carry = [eb[c].ref[4 + t] for t in range(2)] if b else [0.0, 0.0]
            if b:
                f = [lax.add(v, jnp.where(row == 0, w, 0.0)) for v, w in zip(f, _cmul(*power(2 * L, c, 2), *carry))]
            for n in (1, 2, 4, 8):
                f = [jnp.where(row >= n, w, v)
                     for v, w in zip(f, _cmad(*power(2 * n * L, c, 2), *[pltpu.roll(v, n, 0) for v in f], *f))]
            first = [jnp.where(row == 0, w, pltpu.roll(v, 1, 0)) for v, w in zip(f, carry)]
            for h, init in enumerate((first, _cmad(*power(L, c, 2), *first, *even))):
                for t in range(2):
                    eb[c].ref[2 * t + h] = init[t]
            for t in range(2):
                eb[c].ref[4 + t] = jnp.broadcast_to(f[t][15:16], (16, LANE))
            yield None, 140
            yield eb[c], -4

    def t_states(b):
        yield 1480 * _LS[b]
        for q in range(_LS[b]):
            for part in range(2):
                tiles = []
                for c in range(NL):
                    yield eb[c], 1
                    for v in range(2):
                        yield ub[v][q], 0
                    yield None, (39, 39, 94, 119, 144)[c]
                    pr, pi = power(q + 1, c, 2)
                    hs = []
                    for h in range(2):
                        t = lax.mul(pr, eb[c].ref[2 * part + h]), lax.mul(pi, eb[c].ref[2 * (1 - part) + h])
                        hs.append(lax.add(load_state(q, state(part, h, c)), lax.add(*t) if part else lax.sub(*t)))
                    tiles.append((_cat(*map(_lo, hs)), _cat(*map(_hi, hs))))
                yield from scatter(_LHS_SLP, _NAMES, *zip(*tiles), hl[b % 2], q, part * _R, 300, 2)

    K4 = 2 * _R
    K4D = K4 + len(_NAMES_K4)

    def t_act(b, g):
        yield (4 * gather_weight(_O_KEPT) + 250) * _LS[b]
        for q in range(_LS[b]):
            hidden = [[], []]
            for v in range(2):
                gate = yield from gather(("G", b, g), q, v, 0, _O_KEPT)
                for c in range(NL):
                    yield None, 5
                    for h in range(2):
                        gate[h][c] = _gelu2(gate[h][c])
                up = yield from gather(("G", b, g), q, v, 1, _O_KEPT)
                for c in range(NL):
                    hidden[v].append(_cat(*[lax.mul(gate[h][c], up[h][c]) for h in range(2)]))
            yield from scatter(_LHS_SLP, _NAMES, *hidden, dl, q, g * _R, 200, 5)

    def t_act_rest(b):
        lane = lax.broadcasted_iota(jnp.int32, (8, LANE), 1)
        yield (2 * gather_weight(_O_KEPT) + 2 * gather_weight(_O_N2) + 140) * _LS[b]
        for q in range(_LS[b]):
            hidden = [[], []]
            for v in range(2):
                ta = yield from gather(("R", b), q, v, 0, _O_KEPT)
                for c in range(4):
                    yield None, 5
                    for h in range(2):
                        a = _gelu2(ta[h][c])
                        if c == 3:
                            a = jnp.where(lane < LANE // 2, lax.mul(a, pltpu.roll(ta[h][c], LANE // 2, 1)), 0.0)
                        ta[h][c] = a
                tb = yield from gather(("R", b), q, v, 1, _O_N2)
                for c in range(4):
                    hidden[v].append(_cat(*[lax.mul(ta[h][c], (ta[h] + tb[h])[4 + c]) if c < 3 else ta[h][c]
                                            for h in range(2)]))
            for h in range(2):
                for i in range(4):
                    dl.ref[K4D + 4 * h + i, pl.ds(8 * q, 8), :] = _pack(hidden[h][i])
            yield from scatter(_LHS_SLP_K4, _NAMES_K4, *hidden, dl, q, K4, 100, 1)

    def ssm_output(b, q, v, emit):
        y = yield from gather(("C", b), q, v, 0, _O_ALL)
        yield sb[0][b], 2
        yield sb[1][b], 3
        stats = [[sb[n][b].ref[out_rows(b, q, v, h), :] for n in range(2)] for h in range(2)]
        for c in range(NL):
            yield xf[b][c], 27
            for h, (mean, rstd) in enumerate(stats):
                x = xf[b][c].ref[out_rows(b, q, v, h), :]
                emit(h, c, x, lax.add(y[h][c], lax.mul(lax.mul(lax.sub(x, mean), rstd), coef(0, c))))

    def t_finish(b):
        yield 2 * (2 * gather_weight(_O_ALL) + 195) * _LS[b]
        for q in range(_LS[b]):
            for v in range(2):
                g = yield from gather(("C", b), q, v, 1, _O_ALL)
                for c in range(NL):
                    yield None, 11
                    for h in range(2):
                        g[h][c] = _silu_half(g[h][c])

                def emit(h, c, x, s):
                    of[b].ref[out_rows(b, q, v, h, c), :] = lax.add(x, lax.mul(s, g[h][c]))
                yield from ssm_output(b, q, v, emit)
                yield of[b], -1

    def t_out(b):
        yield 1
        yield None, 1
        for c in range(NL):
            copy_out(b, c, of[b], c)
        yield of[b], -3

    def t_skip(b):
        yield 2 * (gather_weight(_O_ALL) + 140) * _LS[b]
        for q in range(_LS[b]):
            for v in range(2):
                def emit(h, c, x, s):
                    ub[v][q].ref[state(0, h, c)] = s
                yield from ssm_output(b, q, v, emit)
                yield ub[v][q], -1

    def t_column(b, c):
        dest = bufs["oc"][c]
        terms = sorted((s, m, sign * _O_ALL.sign[r]) for m, r in enumerate(_O_ALL.order)
                       for (j, s), sign in _SCHEME.out[_NAMES[r]].items() if j == c)
        yield 6 * _LS[b] + 1
        for q in range(_LS[b]):
            chunks = [products(("C", b))[q][v][1] for v in range(2)]
            for n in sorted({m // _CHUNK for _, m, _ in terms}):
                for v in range(2):
                    yield chunks[v][n], 0
            yield None, 3
            acc = {}
            for s, m, sign in terms:
                val = _cat(*[chunks[v][m // _CHUNK].ref[m % _CHUNK] for v in range(2)])
                if (0, s) in acc:
                    acc[0, s].add(sign, val)
                else:
                    acc[0, s] = _Sum(sign, val)
            yield None, 1
            g = [_silu_half(d[0]) for d in _columns(acc, 1)]
            for v in range(2):
                yield ub[v][q], 1
            for h in range(2):
                res = lax.mul(load_state(q, state(0, h, c)), g[h])
                for v, part in enumerate((_lo(res), _hi(res))):
                    dest.ref[out_rows(b, q, v, h), :] = lax.add(xf[b][c].ref[out_rows(b, q, v, h), :], part)
            yield dest, -1
        yield None, 1
        copy_out(b, c, dest, 0)
        yield dest, -1

    tasks = dict(coefs=t_coefs, prep=t_prep, stage=t_stage, stats=t_stats, moments=t_moments, ln=t_ln,
                 project=t_project, starts=t_starts, states=t_states, act=t_act, act_rest=t_act_rest,
                 finish=t_finish, out=t_out, skip=t_skip, column=t_column)

    def dots(key, issued, order):
        kind, b = key[0], key[1]
        w = lambda *a: functools.partial(weight, *a)
        keep = lambda place: lambda vs: [(place, vs[0])]
        everywhere = range(_LS[b])
        res = []

        def halves(buf, dims, group, keep):
            (lhs, rhs, _), = group
            n = (_LS[b] + 1) // 2
            return buf, dims, [(lhs, rhs, everywhere[:n]), (lhs, rhs, everywhere[n:])], lambda vs: keep([_cat(*vs)])

        def grouped(name, half):
            for n, (s, a, bb, c, ca, cb) in enumerate(_GROUPS):
                def fold(vs, first=3 * n, signs=(ca * _V_FULL.sign[s] * _V_FULL.sign[a],
                                                 cb * _V_FULL.sign[s] * _V_FULL.sign[bb])):
                    vs = [vs[order.index(k)] for k in "sabc"]
                    sums = [(lax.add if sg > 0 else lax.sub)(v, vs[0]) for sg, v in zip(signs, vs[1:3])]
                    return [((half, _O_KEPT.order.index(r)), v) for r, v in enumerate(sums + vs[3:], first)]
                res.append((xl[b % 2], NT, [([_NAMES.index(p)], [w(name, p)], everywhere)
                                            for p in (dict(s=s, a=a, b=bb, c=c)[k] for k in order)], fold))

        if kind == "B":
            grouped("b0", 1)
            grouped("b1", 0)
        elif kind == "b" and key[2] == 3:
            grouped("b1", 0)
        elif kind == "G":
            grouped("g%d" % key[2], 0)
            grouped("u%d" % key[2], 1)
        elif kind == "r" and key[2]:
            grouped("r0", 0)
        elif kind in "Rr":
            rest = [(xl[b % 2], NT, [([_NAMES.index(p) for p, _ in parts], [w("r1", (n, p)) for p, _ in parts],
                                     everywhere)], keep((1, _O_N2.order.index(n))))
                    for n, (_, parts) in enumerate(_N2)]
            if kind == "R":
                grouped("r0", 0)
                res = rest[1:] + res + rest[:1]
            else:
                res = [halves(*rest[0])] + rest[1:]
        else:
            for p in _products(key):
                r = _NAMES.index(p)
                place = _O_ALL.order.index(r)
                if kind == "b":
                    res.append((xl[b % 2], NT, [([r], [w("b0", p)], everywhere)], keep((1, place))))
                elif kind == "C":
                    res.append((hl[b % 2], NT, [([r, _R + r], [w("c0", p), w("c1", p)], everywhere)], keep((0, place))))
                else:
                    lhs, rhs = [r, _R + r], [w("d0", p), w("d1", p)]
                    if p in _W_K4:
                        lhs.append(K4 + _NAMES_K4.index(p))
                        rhs.append(w("d2", p))
                    if p in _D4:
                        lhs += [K4D + 4 * _D4.index(p) + i for i in range(4)]
                        rhs += [functools.partial(tile_rows, *_TABLES["d2"][1:], i, 4) for i in range(4)]
                    cuts = [i for i in range(len(lhs) + 1) if i in (0, len(lhs)) or (issued + i) % 4 == 0]
                    issued += len(lhs)
                    for i, j in zip(cuts, cuts[1:]):
                        res.append((dl, NN, [(lhs[i:j], rhs[i:j], everywhere)], keep((1 + (i > 0), place))))
        if key == plan.phases[-1]:
            res[-1] = halves(*res[-1])
        return res

    def stream():
        for n, (t, _, _) in enumerate(plan.tasks):
            if t[0] not in ("wait", "pause"):
                task = tasks[t[0]](*t[1:])
                done, total = 0.0, next(task)
                for buf, cost in task:
                    if cost >= 0:
                        yield buf, n + done / total, None
                        done += cost
                    else:
                        yield buf, None, -cost * _WINDOW.get(t[0], 17)
                assert abs(done - total) < 1e-6 * total

    waits = [(n, t[1:]) for n, (t, _, _) in enumerate(plan.tasks) if t[0] == "wait"]
    work = stream()
    item = next(work)
    issued, current = 0, (-1, {})
    due = {}

    def operand(buf, slot, where, rnd):
        nonlocal current
        zeros = dict(current[1]) if rnd == current[0] else {}
        for k in [k for k in due if k[0] <= rnd]:
            zeros.setdefault(min(max(k[1], where[0]), where[-1]), []).extend(due.pop(k))
        zeros = {q: [functools.reduce(lax.bitwise_or, zs)] for q, zs in zeros.items() if q in where}
        current = rnd, zeros
        if not zeros:
            return buf.ref[slot, pl.ds(8 * where[0], 8 * len(where)), :]
        rows = [buf.ref[slot, pl.ds(8 * q, 8), :] for q in where]
        for q, (v,) in zeros.items():
            rows[q - where[0]] = lax.bitwise_or(rows[q - where[0]], v)
        return _cat(*rows)

    def run_phase(key):
        nonlocal issued, item
        L, i = _LS[key[1]], plan.phases.index(key)
        dest = products(key)
        first = issued // 4
        released = first - 1
        lead, slack, quiet, which, order = _TUNING.get(key, _UNTUNED)[:5]
        slots = L * max(_n_tiles(key) / 4 - quiet, 1.0)
        for buf, dims, group, keep in dots(key, issued, order):
            vs = []
            for lhs, rhs, where in group:
                a = [operand(buf, slot, where, (issued + n) // 4) for n, slot in enumerate(lhs)]
                a = a[0] if len(a) == 1 else lax.concatenate(a, 1)
                w = [load() for load in rhs]
                w = w[0] if len(w) == 1 else lax.concatenate(w, 1 if dims is NT else 0)
                vs.append(lax.dot_general(pltpu.bitcast(a, BF16), w, dims, preferred_element_type=F32))
                issued += len(rhs)
            rnd = (issued - 1) // 4
            kept = keep(vs)
            mark = kept[which % len(kept)][1]
            for q in range(L):
                for (half, slot), val in kept:
                    for v in range(2):
                        chunk = dest[q][v][min(half, 1)][slot // _CHUNK]
                        rows = lax.slice_in_dim(val, 16 * q + 8 * v, 16 * q + 8 * v + 8, axis=0)
                        chunk.ref[slot % _CHUNK] = lax.add(chunk.ref[slot % _CHUNK], rows) if half > 1 else rows
                fenced = []
                goal = min([plan.progress(i, max((rnd - first) * L + q + 1 + lead, 0) / slots) - 1e-6]
                           + [n for n, _ in waits])
                while rnd > released and item is not None and (item[1] is None or item[1] < goal):
                    if item[1] is None:
                        late = max(L, q + item[2] + slack)
                        due.setdefault((rnd + late // L, late % L), []).append(item[0].done())
                    elif item[0] is not None and item[0] not in fenced:
                        fenced.append(item[0])
                        item[0].fence(lax.slice_in_dim(mark, 16 * q, 16 * q + 8, axis=0))
                    item = next(work, None)
            released = rnd
            reached = plan.progress(i, (rnd - first + 1) * L / slots)
            while waits and waits[0][0] + 1 <= reached + 1e-6 and issued % 4 == 0:
                for cp in copies[waits.pop(0)[1]]:
                    cp.wait()
        assert item is None or item[1] >= plan.lo[i] - 1e-6
        assert not waits or waits[0][0] >= plan.lo[i]

    for cp in sum(copies.values(), []):
        cp.start()
    for step in plan.steps:
        if step[0] == "wait":
            for cp in copies[step[1:]]:
                cp.wait()
        elif step[0] == "run":
            task, written = tasks[step[1]](*step[2:]), []
            next(task)
            for buf, cost in task:
                if cost < 0 and buf not in written:
                    written.append(buf)
            for buf in written:
                buf.fence(jnp.zeros((8, LANE), F32))
        else:
            run_phase(step)
    assert item is None and not waits
    for cp in out_copies:
        cp.wait()


@jax.jit
def pallas_recurrent_scan__ssm_conv_s5__geglu_ffn__prompt_kernel(
    A_x, A_Lambda_re, A_Lambda_im, A_B_re, A_B_im, A_C_re, A_C_im, A_log_dt, A_Dskip,
    B_x, B_w_gate, B_w_up, B_w_down,
):
    del B_x
    batch, S, D = A_x.shape
    F = B_w_down.shape[0]
    assert (batch, S, D, F) == (1, 32 * sum(_LS), 5 * LANE, 13 * LANE + LANE // 2)
    plan = _Schedule()
    out = pl.pallas_call(
        functools.partial(_kernel, plan),
        in_specs=[pl.BlockSpec(memory_space=pl.ANY)] * 12,
        out_specs=pl.BlockSpec(memory_space=pl.ANY),
        out_shape=jax.ShapeDtypeStruct((S, D), F32),
        scratch_shapes=[_scratch(plan, S, D, F)],
        compiler_params=pltpu.CompilerParams(vmem_limit_bytes=126 * 2**20),
    )(A_x.reshape(S, D), A_Lambda_re, A_Lambda_im, A_B_re, A_B_im, A_C_re, A_C_im, A_log_dt, A_Dskip,
      B_w_gate.T, B_w_up.T, B_w_down)
    return out.reshape(batch, S, D)
```
